```python
import jax
import jax.numpy as jnp

def _softmax(x, axis=-1):
    return jax.nn.softmax(x, axis=axis)
def _gelu(x):
    return jax.nn.gelu(x, approximate=True)
def _silu(x):
    return jax.nn.silu(x)
def _sigmoid(x):
    return jax.nn.sigmoid(x)
def _layernorm(x, axis=-1, eps=1e-5):
    m = jnp.mean(x, axis=axis, keepdims=True)
    v = jnp.var(x, axis=axis, keepdims=True)
    return (x - m) / jnp.sqrt(v + eps)
def _scatter_add(tgt, idx, src, axis=0):
    return tgt.at[idx].add(src)
def _segment_sum(src, seg, n):
    return jax.ops.segment_sum(src, seg, n)
class _Rng:
    def __init__(self, key):
        self._k = key
    def _next(self):
        self._k, sub = jax.random.split(self._k)
        return sub
    def normal(self, shape):
        return jax.random.normal(self._next(), shape, dtype=jnp.bfloat16)
    def randint(self, lo, hi, shape):
        return jax.random.randint(self._next(), shape, lo, hi, dtype=jnp.int32)
    def uniform(self, shape, lo=0.0, hi=1.0):
        return jax.random.uniform(self._next(), shape, jnp.bfloat16, lo, hi)
    def permutation(self, n):
        return jax.random.permutation(self._next(), n)


kernel_name = 'standalone__self_sup_conv_stem_wavlm__speech'

def setup_inputs():
    _rng = _Rng(jax.random.key(int.from_bytes(__import__("os").urandom(4), "little")))
    _w = (lambda a: (lambda t: t.astype(jnp.bfloat16) if jnp.issubdtype(t.dtype, jnp.floating) else t)(jnp.asarray(a)))
    B, T, D, K = 2, 16000, 512, 31
    scale = (K * D) ** -0.5
    return {
        "x": _w((lambda *s: _rng.normal(s) * 0.05)(B, T, D)),
        "w": _w((lambda *s: _rng.normal(s) * 0.05)(K, D, D) * scale),
        "gn_gamma": _w((lambda *s: _rng.normal(s) * 0.05)(D) * 0.1 + 1.0),
        "gn_beta": _w((lambda *s: _rng.normal(s) * 0.05)(D) * 0.1),
    }

def reference(x, w, gn_gamma, gn_beta):
    B, T, D = x.shape
    K = w.shape[0]
    s = 2
    L = (T - K) // s + 1
    h = jnp.einsum('blc,cd->bld', x[:, 0:s * L:s, :], w[0])
    for i in range(1, K):
        h = h + jnp.einsum('blc,cd->bld', x[:, i:i + s * L:s, :], w[i])
    mu = jnp.einsum('bld->bd', h)[:, None, :] / L
    var = jnp.einsum('bld->bd', (h - mu) ** 2)[:, None, :] / L
    h = (h - mu) / jnp.sqrt(var + 1e-5)
    h = h * gn_gamma[None, None, :] + gn_beta[None, None, :]
    return _gelu(h)
```

```python
import math
import random
import numpy as np
import jax, jax.numpy as jnp
from jax import lax
from jax.experimental import pallas as pl
from jax.experimental.pallas import tpu as pltpu


class Net:
    def __init__(self):
        self.nodes = []
        self.cse = {}

    def _mk(self, key):
        if key in self.cse:
            return self.cse[key]
        self.nodes.append(key)
        self.cse[key] = len(self.nodes) - 1
        return self.cse[key]

    def inp(self, i):
        return (self._mk(('in', i)), 1)

    def neg(self, x):
        return None if x is None else (x[0], -x[1])

    def add(self, x, y):
        if x is None:
            return y
        if y is None:
            return x
        (a, sa), (b, sb) = x, y
        if a == b:
            if sa == sb:
                return self.mul(x, 2.0)
            return None
        if sa == sb:
            if a > b:
                a, b = b, a
            return (self._mk(('add', a, b)), sa)
        if a > b:
            a, b, sa = b, a, sb
        return (self._mk(('sub', a, b)), sa)

    def sub(self, x, y):
        return self.add(x, self.neg(y))

    def mul(self, x, c):
        if x is None or abs(c) < 1e-12:
            return None
        a, s = x
        if c < 0:
            c, s = -c, -s
        if abs(c - 1.0) < 1e-12:
            return (a, s)
        c = float(np.float64(round(c, 14)))
        return (self._mk(('mul', a, c)), s)

    def cadd(self, x, y):
        return (self.add(x[0], y[0]), self.add(x[1], y[1]))

    def csub(self, x, y):
        return (self.sub(x[0], y[0]), self.sub(x[1], y[1]))

    def cmulc(self, x, c, s):
        a, b = x
        if abs(s) < 1e-12:
            return (self.mul(a, c), self.mul(b, c))
        if abs(c) < 1e-12:
            return (self.mul(b, -s), self.mul(a, s))
        if abs(abs(c) - abs(s)) < 1e-12:
            sg = 1.0 if s * c > 0 else -1.0
            re = self.sub(a, self.mul(b, sg))
            im = self.add(b, self.mul(a, sg))
            return (self.mul(re, c), self.mul(im, c))
        re = self.sub(self.mul(a, c), self.mul(b, s))
        im = self.add(self.mul(a, s), self.mul(b, c))
        return (re, im)


def w(k, n):
    ang = -2.0 * math.pi * (k % n) / n
    return math.cos(ang), math.sin(ang)


def cfft(net, z):
    n = len(z)
    if n == 1:
        return [z[0]]
    if n == 2:
        return [net.cadd(z[0], z[1]), net.csub(z[0], z[1])]
    if n % 4 == 0:
        h, q = n // 2, n // 4
        e = [net.cadd(z[t], z[t + h]) for t in range(h)]
        o = [net.csub(z[t], z[t + h]) for t in range(h)]
        z1, z3 = [], []
        for t in range(q):
            a, b = o[t], o[t + q]
            mib = (b[1], net.neg(b[0]))
            p = net.cadd(a, mib)
            m = net.csub(a, mib)
            z1.append(net.cmulc(p, *w(t, n)))
            z3.append(net.cmulc(m, *w(3 * t, n)))
        E = cfft(net, e)
        Z1 = cfft(net, z1)
        Z3 = cfft(net, z3)
        out = [None] * n
        for k in range(h):
            out[2 * k] = E[k]
        for k in range(q):
            out[4 * k + 1] = Z1[k]
            out[4 * k + 3] = Z3[k]
        return out
    if n % 2 == 0:
        m = n // 2
        out = [None] * n
        rows = []
        for t2 in range(m):
            a = z[(2 * t2) % n]
            b = z[(m + 2 * t2) % n]
            rows.append((net.cadd(a, b), net.csub(a, b)))
        for k1 in range(2):
            Z = cfft(net, [rows[t2][k1] for t2 in range(m)])
            for k2 in range(m):
                for k in range(n):
                    if k % 2 == k1 and k % m == k2:
                        out[k] = Z[k2]
        return out
    if n % 3 == 0 and n > 3:
        raise NotImplementedError
    out = []
    p = {t: net.cadd(z[t], z[n - t]) for t in range(1, (n + 1) // 2)}
    q = {t: net.csub(z[t], z[n - t]) for t in range(1, (n + 1) // 2)}
    s = z[0]
    for t in p:
        s = net.cadd(s, p[t])
    out = [None] * n
    out[0] = s
    for k in range(1, (n + 1) // 2):
        A = z[0]
        B = (None, None)
        for t in p:
            c, sn = w(k * t, n)
            A = net.cadd(A, (net.mul(p[t][0], c), net.mul(p[t][1], c)))
            B = net.cadd(B, (net.mul(q[t][1], -sn), net.mul(q[t][0], sn)))
        out[k] = net.cadd(A, B)
        out[n - k] = net.csub(A, B)
    return out


def cfft_pfa(net, z, n1, n2):
    n = n1 * n2
    out = [None] * n
    cols = [cfft_any(net, [z[(n2 * t1 + n1 * t2) % n] for t2 in range(n2)]) for t1 in range(n1)]
    for k2 in range(n2):
        Z = cfft_any(net, [cols[t1][k2] for t1 in range(n1)])
        for k1 in range(n1):
            for k in range(n):
                if k % n1 == k1 and k % n2 == k2:
                    out[k] = Z[k1]
    return out


def cfft5(net, z):
    c1, c2 = math.cos(2 * math.pi / 5), math.cos(4 * math.pi / 5)
    s1, s2 = math.sin(2 * math.pi / 5), math.sin(4 * math.pi / 5)
    t1 = net.cadd(z[1], z[4]); t2 = net.cadd(z[2], z[3])
    t3 = net.csub(z[1], z[4]); t4 = net.csub(z[2], z[3])
    t5 = net.cadd(t1, t2)
    def rm(x, c):
        return (net.mul(x[0], c), net.mul(x[1], c))
    m1 = rm(t5, (c1 + c2) / 2 - 1.0)
    m2 = rm(net.csub(t1, t2), (c1 - c2) / 2)
    y0 = net.cadd(z[0], t5)
    a = net.cadd(y0, m1)
    a1 = net.cadd(a, m2); a2 = net.csub(a, m2)
    m3 = rm(net.cadd(t3, t4), s2)
    m4 = rm(t3, s1 - s2)
    m5 = rm(t4, s1 + s2)
    b1 = net.cadd(m3, m4)
    b2 = net.csub(m3, m5)
    def mi(x):
        return (x[1], net.neg(x[0]))
    return [y0, net.cadd(a1, mi(b1)), net.cadd(a2, mi(b2)), net.csub(a2, mi(b2)), net.csub(a1, mi(b1))]


def rfft5(net, x):
    c1, c2 = math.cos(2 * math.pi / 5), math.cos(4 * math.pi / 5)
    s1, s2 = math.sin(2 * math.pi / 5), math.sin(4 * math.pi / 5)
    t1 = net.add(x[1], x[4]); t2 = net.add(x[2], x[3])
    t3 = net.sub(x[1], x[4]); t4 = net.sub(x[2], x[3])
    t5 = net.add(t1, t2)
    m1 = net.mul(t5, (c1 + c2) / 2 - 1.0)
    m2 = net.mul(net.sub(t1, t2), (c1 - c2) / 2)
    y0 = net.add(x[0], t5)
    a = net.add(y0, m1)
    a1 = net.add(a, m2); a2 = net.sub(a, m2)
    m3 = net.mul(net.add(t3, t4), s2)
    m4 = net.mul(t3, s1 - s2)
    m5 = net.mul(t4, s1 + s2)
    b1 = net.add(m3, m4); b2 = net.sub(m3, m5)
    return [(y0, None), (a1, net.neg(b1)), (a2, net.neg(b2))]


def cfft_any(net, z):
    n = len(z)
    if n == 5:
        return cfft5(net, z)
    if n == 12:
        return cfft_pfa(net, z, 3, 4)
    if n == 10:
        return cfft_pfa(net, z, 5, 2)
    if n == 20:
        return cfft_pfa(net, z, 5, 4)
    if n == 6:
        return cfft_pfa(net, z, 3, 2)
    if n == 14:
        return cfft_pfa(net, z, 7, 2)
    if n == 15:
        return cfft_pfa(net, z, 5, 3)
    return cfft(net, z)


def rfft_pfa(net, x, n1, n2):
    n = n1 * n2
    inner = [rfft(net, [x[(n2 * t1 + n1 * t2) % n] for t1 in range(n1)]) for t2 in range(n2)]
    out = [None] * (n // 2 + 1)
    for k1 in range(n1 // 2 + 1):
        col = [inner[t2][k1] for t2 in range(n2)]
        if all(c[1] is None for c in col):
            Z = rfft(net, [c[0] for c in col])
            Z = Z + [(Z[n2 - k2][0], net.neg(Z[n2 - k2][1])) for k2 in range(len(Z), n2)]
        else:
            Z = cfft_any(net, col)
        for k2 in range(n2):
            k = [k for k in range(n) if k % n1 == k1 and k % n2 == k2][0]
            if k <= n // 2:
                if out[k] is None:
                    out[k] = Z[k2]
            else:
                if out[n - k] is None:
                    out[n - k] = (Z[k2][0], net.neg(Z[k2][1]))
    return out


PFA = {40: (8, 5), 20: (4, 5), 24: (8, 3), 48: (16, 3), 12: (4, 3), 56: (8, 7), 10: (2, 5), 6: (2, 3), 60: (4, 15), 15: (3, 5), 44: (4, 11), 36: (4, 9)}
USE_PFA = True


def rfft(net, x):
    n = len(x)
    if USE_PFA and n in PFA:
        return rfft_pfa(net, x, *PFA[n])
    if n == 1:
        return [(x[0], None)]
    if n == 2:
        return [(net.add(x[0], x[1]), None), (net.sub(x[0], x[1]), None)]
    if n % 4 == 0:
        h, q = n // 2, n // 4
        e = [net.add(x[t], x[t + h]) for t in range(h)]
        o = [net.sub(x[t], x[t + h]) for t in range(h)]
        z = [net.cmulc((o[t], net.neg(o[t + q])), *w(t, n)) for t in range(q)]
        E = rfft(net, e)
        Z = cfft_any(net, z)
        out = [None] * (h + 1)
        for k in range(len(E)):
            out[2 * k] = E[k]
        for k in range(q):
            f = 4 * k + 1
            if f <= h:
                out[f] = Z[k]
            else:
                out[n - f] = (Z[k][0], net.neg(Z[k][1]))
        return out
    if n % 2 == 0:
        m = n // 2
        e = [net.add(x[t], x[t + m]) for t in range(m)]
        o = [net.sub(x[t], x[t + m]) for t in range(m)]
        E = rfft(net, e)
        op = [o[t] if t % 2 == 0 else net.neg(o[t]) for t in range(m)]
        O = rfft(net, op)
        out = [None] * (m + 1)
        for k in range(len(E)):
            out[2 * k] = E[k]
        for f in range(1, m + 1, 2):
            j = ((f - m) // 2) % m
            if j <= m // 2:
                out[f] = O[j]
            else:
                out[f] = (O[m - j][0], net.neg(O[m - j][1]))
        return out
    if n == 5:
        return rfft5(net, x)
    p = {t: net.add(x[t], x[n - t]) for t in range(1, (n + 1) // 2)}
    q = {t: net.sub(x[t], x[n - t]) for t in range(1, (n + 1) // 2)}
    s = x[0]
    for t in p:
        s = net.add(s, p[t])
    out = [(s, None)]
    for k in range(1, (n + 1) // 2):
        A = x[0]
        B = None
        for t in p:
            c, sn = w(k * t, n)
            A = net.add(A, net.mul(p[t], c))
            B = net.add(B, net.mul(q[t], sn))
        out.append((A, B))
    return out


class Prog:
    def __init__(self, net, outputs):
        order = []
        seen = set()

        def visit(n):
            if n in seen:
                return
            seen.add(n)
            k = net.nodes[n]
            if k[0] in ('add', 'sub'):
                visit(k[1]); visit(k[2])
            elif k[0] == 'mul':
                visit(k[1])
            order.append(n)
        for o in outputs:
            if o is not None:
                visit(o[0])
        self.net = net
        self.order = order
        self.outputs = outputs

    def count(self):
        c = {'add': 0, 'sub': 0, 'mul': 0, 'in': 0}
        for n in self.order:
            c[self.net.nodes[n][0]] += 1
        return c

    def run(self, load, emit=None):
        vals = {}
        for n in self.order:
            k = self.net.nodes[n]
            if k[0] == 'in':
                vals[n] = load(k[1])
            elif k[0] == 'add':
                vals[n] = vals[k[1]] + vals[k[2]]
            elif k[0] == 'sub':
                vals[n] = vals[k[1]] - vals[k[2]]
            else:
                vals[n] = vals[k[1]] * k[2]
        return [None if o is None else vals[o[0]] for o in self.outputs]

    @property
    def signs(self):
        return [0 if o is None else o[1] for o in self.outputs]

    def matrix(self, n_in, signed=True):
        eye = np.eye(n_in)
        res = self.run(lambda i: eye[i])
        rows = []
        for r, s in zip(res, self.signs):
            rows.append(np.zeros(n_in) if r is None else (r * s if signed else r))
        return np.stack(rows)


def transpose(net, outputs, wanted_inputs):
    prog = Prog(net, outputs)
    live = set(prog.order)
    consumers = {n: [] for n in prog.order}
    for n in prog.order:
        k = net.nodes[n]
        if k[0] == 'add':
            consumers[k[1]].append((n, 1.0)); consumers[k[2]].append((n, 1.0))
        elif k[0] == 'sub':
            consumers[k[1]].append((n, 1.0)); consumers[k[2]].append((n, -1.0))
        elif k[0] == 'mul':
            consumers[k[1]].append((n, k[2]))
    outmap = {}
    for r, o in enumerate(outputs):
        if o is not None:
            outmap.setdefault(o[0], []).append((r, o[1]))
    tn = Net()
    memo = {}

    def adj(n):
        if n in memo:
            return memo[n]
        acc = None
        for r, s in outmap.get(n, []):
            v = tn.inp(r)
            acc = tn.add(acc, v if s > 0 else tn.neg(v))
        for c, coef in consumers[n]:
            acc = tn.add(acc, tn.mul(adj(c), coef))
        memo[n] = acc
        return acc
    outs = []
    for i in wanted_inputs:
        key = ('in', i)
        if key in net.cse and net.cse[key] in live:
            outs.append(adj(net.cse[key]))
        else:
            outs.append(None)
    return tn, outs


def build(N, taps, scale=True):
    hop = N - taps + 1
    na = Net()
    U = rfft(na, [na.inp(t) for t in range(N)])
    a_out = [U[0][0], U[N // 2][0]]
    bins = list(range(1, N // 2))
    for k in bins:
        a, b = U[k]
        a_out += [na.add(a, b), a, b]
    nc = Net()
    V = rfft(nc, [nc.inp(t) for t in range(N)])
    c_out = [V[0][0], V[N // 2][0]]
    for k in bins:
        al, be = V[k]
        c_out += [nc.add(al, be), be, nc.neg(al)]
    tn, c_res = transpose(nc, c_out, list(range(hop)))
    nb = Net()
    Wf = rfft(nb, [nb.inp(t) if t < taps else None for t in range(N)])
    s0 = 1.0 / N if scale else 0.5
    b_out = [nb.mul(Wf[0][0], s0), nb.mul(Wf[N // 2][0], s0)]
    for k in bins:
        c = Wf[k][0]
        d = nb.neg(Wf[k][1])
        sc = 2.0 / N if scale else 1.0
        b_out += [nb.mul(c, sc), nb.mul(nb.sub(d, c), sc), nb.mul(nb.add(c, d), sc)]
    return dict(N=N, hop=hop, taps=taps, na=na, a_out=a_out, nb=nb, b_out=b_out, tn=tn, c_res=c_res, bins=bins)


def max_live(net, order, outputs, out_at_once=True):
    uses = {n: 0 for n in order}
    for n in order:
        k = net.nodes[n]
        for a in ([k[1], k[2]] if k[0] in ('add', 'sub') else [k[1]] if k[0] == 'mul' else []):
            uses[a] += 1
    live = set(); peak = 0; tot = 0
    rem = dict(uses)
    for n in order:
        k = net.nodes[n]
        live.add(n)
        peak = max(peak, len(live))
        for a in set([k[1], k[2]] if k[0] in ('add', 'sub') else [k[1]] if k[0] == 'mul' else []):
            rem[a] -= (1 if k[0] == 'mul' or k[1] != k[2] else 2)
            if rem[a] == 0:
                live.discard(a)
        if rem[n] == 0:
            live.discard(n)
        tot += len(live)
    return peak, tot / len(order)


def min_live_order(net, outputs, seed=0, tries=200):
    base = Prog(net, outputs).order
    nodes = set(base)
    def operands(n):
        k = net.nodes[n]
        return [k[1], k[2]] if k[0] in ('add', 'sub') else [k[1]] if k[0] == 'mul' else []
    consumers = {n: [] for n in base}
    for n in base:
        for a in set(operands(n)):
            consumers[a].append(n)
    best = (max_live(net, base, outputs), base)
    rnd = random.Random(seed)
    pos = {n: i for i, n in enumerate(base)}
    for it in range(tries):
        done = set(); order = []
        live = set()
        remc = {n: len(consumers[n]) for n in base}
        isin = {n: net.nodes[n][0] == 'in' for n in base}
        def ready(n):
            return n not in done and not isin[n] and all((a in done) or isin[a] for a in operands(n))
        noise = rnd.random() * 1.5
        work = [n for n in base if not isin[n]]
        left = set(work)
        while left:
            cands = [n for n in left if ready(n)]
            def score(n):
                ops = set(operands(n))
                newloads = sum(1 for a in ops if a not in done)
                kills = sum(1 for a in ops if remc[a] == 1)
                born = 0 if remc[n] == 0 else 1
                return (newloads + born - kills) + noise * rnd.random() + 1e-4 * pos[n]
            n = min(cands, key=score)
            for a in sorted(set(operands(n)), key=lambda a: pos[a]):
                if a not in done:
                    done.add(a); order.append(a)
                remc[a] -= 1
            done.add(n); order.append(n); left.discard(n)
        ml = max_live(net, order, outputs)
        if ml < best[0]:
            best = (ml, order)
    return best


def solve_signs(G, iters=200000, seed=0):
    rnd = random.Random(seed)
    nets = {'A': (G['na'], G['a_out']), 'B': (G['nb'], G['b_out']), 'C': (G['tn'], G['c_res'])}
    order = {k: Prog(*v).order for k, v in nets.items()}
    R = len(G['a_out'])
    sig = {}
    for k in 'ABC':
        for n in order[k]:
            sig[(k, n)] = 1
    fixed = set()
    for k in 'AB':
        for n in order[k]:
            if nets[k][0].nodes[n][0] == 'in':
                fixed.add((k, n))
    for o in G['c_res']:
        sig[('C', o[0])] = o[1]; fixed.add(('C', o[0]))
    cin = {}
    for n in order['C']:
        nd = G['tn'].nodes[n]
        if nd[0] == 'in':
            cin[nd[1]] = n; fixed.add(('C', n))
    def cin_sign(r):
        a, b = G['a_out'][r], G['b_out'][r]
        return (sig[('A', a[0])] * a[1]) * (sig[('B', b[0])] * b[1])
    outmap = {}
    for r in range(R):
        outmap.setdefault(('A', G['a_out'][r][0]), []).append(r)
        outmap.setdefault(('B', G['b_out'][r][0]), []).append(r)
    def refresh():
        for r, n in cin.items():
            sig[('C', n)] = cin_sign(r)
    clauses = []
    for k in 'ABC':
        net = nets[k][0]
        for n in order[k]:
            nd = net.nodes[n]
            if nd[0] in ('add', 'sub'):
                clauses.append((k, n, nd[1], nd[2], 1 if nd[0] == 'add' else -1))
    occ = {}
    for ci, (k, n, a, b, cb) in enumerate(clauses):
        for v in (n, a, b):
            occ.setdefault((k, v), []).append(ci)
    def viol(ci):
        k, n, a, b, cb = clauses[ci]
        return sig[(k, n)] * sig[(k, a)] < 0 and sig[(k, n)] * cb * sig[(k, b)] < 0
    def flip(v):
        sig[v] = -sig[v]
        for r in outmap.get(v, []):
            if r in cin:
                sig[('C', cin[r])] = cin_sign(r)
    def affected(v):
        cs = set(occ.get(v, []))
        for r in outmap.get(v, []):
            if r in cin:
                cs.update(occ.get(('C', cin[r]), []))
        return cs
    flippers = {}
    for v, rs in outmap.items():
        for r in rs:
            if r in cin:
                flippers.setdefault(('C', cin[r]), []).append(v)
    refresh()
    bad = {ci for ci in range(len(clauses)) if viol(ci)}
    best = (len(bad), dict(sig))
    for it in range(iters):
        if not bad:
            break
        ci = rnd.choice(list(bad))
        k, n, a, b, cb = clauses[ci]
        cands = []
        for v in ((k, n), (k, a), (k, b)):
            if v in fixed:
                cands += flippers.get(v, [])
            else:
                cands.append(v)
        cands = [v for v in cands if v not in fixed]
        if not cands:
            continue
        def delta(v):
            cs = affected(v)
            before = sum(viol(c) for c in cs)
            flip(v)
            after = sum(viol(c) for c in cs)
            flip(v)
            return after - before
        if rnd.random() < 0.2:
            v = rnd.choice(cands)
        else:
            v = min(cands, key=lambda v: (delta(v), rnd.random()))
        cs = affected(v)
        flip(v)
        for c in cs:
            if viol(c): bad.add(c)
            else: bad.discard(c)
        if len(bad) < best[0]:
            best = (len(bad), dict(sig))
    nb, sg = best
    return ({n: s for (k, n), s in sg.items() if k == 'A'}, {n: s for (k, n), s in sg.items() if k == 'B'},
            {n: s for (k, n), s in sg.items() if k == 'C'}, nb)


class FixedProg:
    def __init__(self, net, outputs, sig, order=None):
        self.net, self.outputs, self.sig = net, outputs, sig
        self.order = order if order is not None else Prog(net, outputs).order
    def count(self):
        c = {'add': 0, 'sub': 0, 'mul': 0, 'in': 0}
        for n in self.order:
            c[self.net.nodes[n][0]] += 1
        return c


N, TAPS = 40, 16
G = build(N, TAPS, scale=False)
HOP = G['hop']; R = len(G['a_out'])
T, D, K = 16000, 512, 31
L = (T - K) // 2 + 1
MB = 64; NCH = -(-L // (HOP * MB))
CH = HOP * MB
XM = CH + 16
LP = NCH * CH
TM = T // 2
LAST_M = TM - (NCH - 1) * CH
HS = 2.0 / N
T2 = 1
U32, F32, BF16 = jnp.uint32, jnp.float32, jnp.bfloat16

bins = G['bins']
ev = [0, 1] + [2 + 3 * i + q for i, k in enumerate(bins) if k % 2 == 0 for q in range(3)]
od = [2 + 3 * i + q for i, k in enumerate(bins) if k % 2 == 1 for q in range(3)]
if (N // 2) % 2 == 1:
    ev.remove(1); od = [1] + od
IDX = (ev, od)
RH = (len(ev), len(od))
LOC = {}
for hf in range(2):
    for i, r in enumerate(IDX[hf]):
        LOC[r] = (hf, i)
SA, SB, SC, NBAD = solve_signs(G)
assert NBAD == 0
def mkprog(net, outs, sig):
    return FixedProg(net, outs, sig, order=min_live_order(net, outs, tries=100)[1])
PA = [mkprog(G['na'], [G['a_out'][r] for r in idx], SA) for idx in IDX]
PB = [mkprog(G['nb'], [G['b_out'][r] for r in idx], SB) for idx in IDX]
PC = mkprog(G['tn'], G['c_res'], SC)


def run_gen(prog, loads, sink):
    nsets = len(loads)
    vals = [dict() for _ in range(nsets)]
    sig = prog.sig
    outs = {}
    for r, o in enumerate(prog.outputs):
        outs.setdefault(o[0], []).append(r)
    for n in prog.order:
        k = prog.net.nodes[n]
        for s in range(nsets):
            v = vals[s]
            if k[0] == 'in':
                v[n] = loads[s](k[1])
            elif k[0] == 'mul':
                v[n] = v[k[1]] * (k[2] * sig[n] * sig[k[1]])
            else:
                a, b = k[1], k[2]
                cb = 1 if k[0] == 'add' else -1
                p, q = sig[n] * sig[a], sig[n] * cb * sig[b]
                if p > 0 and q > 0: v[n] = v[a] + v[b]
                elif p > 0: v[n] = v[a] - v[b]
                elif q > 0: v[n] = v[b] - v[a]
                else: v[n] = -(v[a] + v[b])
            yield 1
        for r in outs.get(n, []):
            yield from sink(r, [vals[s][n] for s in range(nsets)])


def drain(gen):
    for _ in gen:
        pass


def unpack(wd, hi):
    wd = (wd & jnp.uint32(0xffff0000)) if hi else (wd << 16)
    return lax.bitcast_convert_type(wd, F32)


def pack(lo, hi):
    return pltpu.pack_elementwise([lo, hi], packed_dtype=BF16)


def prog_weight(prog, nsets, per_out):
    return len(prog.order) * nsets + len(prog.outputs) * per_out


def interleave(mms, gens_weights):
    total = sum(w for _, w in gens_weights)
    def allops():
        for g, _ in gens_weights:
            yield from g
    gen = allops()
    e = 0; done = False
    for i, mm in enumerate(mms):
        mm()
        tgt = (i + 1) * total // len(mms)
        while not done and e < tgt:
            try:
                e += next(gen)
            except StopIteration:
                done = True
    for _ in gen:
        pass


def merge(lists):
    lists = [l for l in lists if l]
    out = []
    pos = [0] * len(lists)
    tot = sum(len(l) for l in lists)
    for _ in range(tot):
        i = min((i for i in range(len(lists)) if pos[i] < len(lists[i])), key=lambda i: (pos[i] + 0.5) / len(lists[i]))
        out.append(lists[i][pos[i]]); pos[i] += 1
    return out


C0 = math.sqrt(2.0 / math.pi)
def gelu_half(zh):
    u = zh * (zh * zh * (8.0 * C0 * 0.044715) + 2.0 * C0)
    return zh * jnp.tanh(u) + zh


def kernel(x_hbm, w_hbm, gam_ref, bet_ref, out_hbm,
           xb0, xb1, xb2, xb3, we, wo, xe, xo, ye, yo, h0, h1, h2, h3, st, nrm, xsem, wsem, osem):
    xb = (xb0, xb1, xb2, xb3)
    wh = (we, wo); xh = (xe, xo); yy = (ye, yo)
    hh = (h0, h1, h2, h3)
    x32 = x_hbm.bitcast(U32)
    w32 = w_hbm.bitcast(F32)
    o32 = out_hbm.bitcast(F32)
    LASTJ = 2 * NCH - 1

    def x_copy(j, c, full):
        b = j // NCH
        cj = j % NCH
        rows = XM if full else LAST_M
        return pltpu.make_async_copy(
            x32.at[b, pl.ds(pl.multiple_of(cj * CH, 8), rows), pl.ds(c * 128, 128)],
            xb[c].at[pl.ds(0, rows), :], xsem.at[c])

    def x_start(j):
        cj = j % NCH
        @pl.when(cj < NCH - 1)
        def _():
            for c in range(4):
                x_copy(j, c, True).start()
        @pl.when(cj == NCH - 1)
        def _():
            for c in range(4):
                x_copy(j, c, False).start()
                xb[c][pl.ds(LAST_M, XM - LAST_M), :] = jnp.zeros((XM - LAST_M, 128), U32)

    def x_wait(j, cs=range(4)):
        cj = j % NCH
        @pl.when(cj < NCH - 1)
        def _():
            for c in cs:
                x_copy(j, c, True).wait()
        @pl.when(cj == NCH - 1)
        def _():
            for c in cs:
                x_copy(j, c, False).wait()

    WQ = 4
    def w_copy(n, q):
        dst = hh[n].at[1, pl.ds(0, K * 256), :].reshape(K, 256, 128)
        r = 256 // WQ
        return pltpu.make_async_copy(w32.at[:, pl.ds(q * r, r), pl.ds(n * 128, 128)], dst.at[:, pl.ds(q * r, r), :], wsem.at[n, q])

    def o_copy(n, r0, rows, k):
        return pltpu.make_async_copy(hh[n].at[0, pl.ds(r0, rows), :], o32.at[pl.ds(r0, rows), n, 0, :], osem.at[n, k])

    def a_piece(g, c, p, half):
        dyn = not isinstance(g, int)
        base = pl.multiple_of(g * (16 * HOP), 8) if dyn else g * (16 * HOP)
        row = pl.multiple_of(g * 8, 8) if dyn else g * 8
        xw = xb[c].at[pl.ds(base, 16 * HOP + 16), :]
        def mkload(o):
            return lambda t: unpack(xw[pl.ds(t + o * HOP, 8, stride=2 * HOP), :], p)
        def sink(i, vs):
            xh[half][i, pl.ds(row, 8), p * 512 + c * 128:p * 512 + (c + 1) * 128] = pack(vs[0], vs[1])
            yield 1
        return run_gen(PA[half], [mkload(0), mkload(1)], sink), prog_weight(PA[half], 2, 1)

    def a_pieces(half):
        return [a_piece(g, c, p, half) for c in range(4) for g in range(MB // 16) for p in range(2)]

    def w_piece(n, g, p, half):
        dyn = not isinstance(g, int)
        row = pl.multiple_of(g * 8, 8) if dyn else g * 8
        cache = {}
        def word(j):
            if j not in cache:
                cache[j] = lax.bitcast_convert_type(hh[n][1, pl.ds((2 * j + p) * 256 + row, 8), :], U32)
            return cache[j]
        def mkload(hi):
            def load(j):
                if 2 * j + p >= K:
                    return jnp.zeros((8, 128), F32)
                return unpack(word(j), hi)
            return load
        def sink(i, vs):
            wh[half][n, i, pl.ds(p * 256 + row, 8), :] = pack(vs[0], vs[1])
            yield 1
        return run_gen(PB[half], [mkload(0), mkload(1)], sink), prog_weight(PB[half], 2, 1)

    def c_pieces(j, n):
        valid = j >= 0
        b = jnp.where(valid, j // NCH, 0)
        cj = jnp.where(valid, j % NCH, NCH - 1)
        slot = jnp.where(valid, b, 2)
        state = {}
        def col(g):
            if g == 0:
                state['c'] = st[slot, n, 2]; state['a1'] = st[slot, n, 0]; state['a2'] = st[slot, n, 1]
            base = pl.multiple_of(cj * CH + g * (8 * HOP), 8)
            hs = hh[n].at[b, pl.ds(base, 8 * HOP), :]
            def sink(t, vs):
                hs[pl.ds(t, 8, stride=HOP), :] = vs[0]
                d = vs[0] - state['c']
                state['a1'] = state['a1'] + d
                state['a2'] = state['a2'] + d * d
                yield 4
            yield from run_gen(PC, [lambda r: yy[LOC[r][0]][n, LOC[r][1], g * 8:(g + 1) * 8, :]], sink)
            if g == MB // 8 - 1:
                st[slot, n, 0] = state['a1']; st[slot, n, 1] = state['a2']
        return [(col(g), prog_weight(PC, 1, 4)) for g in range(MB // 8)]

    def set_shift(j, n):
        @pl.when(jnp.logical_and(j >= 0, j % NCH == 0))
        def _():
            st[j // NCH, n, 2] = jnp.broadcast_to(ye[n, LOC[0][1], 0:1, :], (8, 128))

    def finalize_stats(n):
        sub = lax.broadcasted_iota(jnp.int32, (8, 128), 0)
        for b in range(2):
            c = st[b, n, 2]
            r0 = (L // 8) * 8
            c1 = jnp.zeros((8, 128), F32); c2 = jnp.zeros((8, 128), F32)
            for r in range(r0, LP, 8):
                d = hh[n][b, r:r + 8, :] - c
                if r < L:
                    d = jnp.where(sub >= L - r, d, 0.0)
                c1 = c1 + d; c2 = c2 + d * d
            s1 = jnp.sum(st[b, n, 0] - c1, axis=0, keepdims=True)
            s2 = jnp.sum(st[b, n, 1] - c2, axis=0, keepdims=True)
            md = s1 * (1.0 / L)
            var = (s2 * (1.0 / L) - md * md) * (HS * HS)
            mu = c[0:1] + md
            a = (HS * lax.rsqrt(var + 1e-5)) * gam_ref[:, n * 128:(n + 1) * 128].astype(F32)
            bb = bet_ref[:, n * 128:(n + 1) * 128].astype(F32) - mu * a
            nrm[n, b, 0] = jnp.broadcast_to(0.5 * a, (8, 128))
            nrm[n, b, 1] = jnp.broadcast_to(0.5 * bb, (8, 128))

    def d_vreg(n, r, cs):
        a0, b0, a1, b1 = cs
        z0 = gelu_half(hh[n][0, pl.ds(r, 8), :] * a0 + b0)
        z1 = gelu_half(hh[n][1, pl.ds(r, 8), :] * a1 + b1)
        hh[n][0, pl.ds(r, 8), :] = lax.bitcast_convert_type(pack(z0, z1), F32)

    def d_consts(n):
        return nrm[n, 0, 0], nrm[n, 0, 1], nrm[n, 1, 0], nrm[n, 1, 1]

    def d_pieces(n):
        state = {}
        def piece(r0, r1):
            if 'cs' not in state:
                state['cs'] = d_consts(n)
            for r in range(r0, r1, 8):
                d_vreg(n, r, state['cs'])
                yield 19
        P = 200
        return [(piece(r, min(r + P, LP)), 19 * (min(r + P, LP) - r) // 8) for r in range(0, LP, P)]

    NPC = 4
    PR = -(-(-(-L // NPC)) // 8) * 8
    def d_loop(n):
        cs = d_consts(n)
        UN = 5
        for k in range(NPC):
            r0 = k * PR; r1 = min(r0 + PR, LP)
            nv = -(-(r1 - r0) // 8)
            assert nv % UN == 0, nv
            def body(i, carry):
                for u in range(UN):
                    d_vreg(n, pl.multiple_of(r0 + (i * UN + u) * 8, 8), cs)
                return carry
            lax.fori_loop(0, nv // UN, body, 0)
            o_copy(n, r0, min(r0 + PR, L) - r0, k).start()

    def o_start_all(n):
        for k in range(NPC):
            r0 = k * PR
            o_copy(n, r0, min(r0 + PR, L) - r0, k).start()

    def o_wait_all(n):
        for k in range(NPC):
            r0 = k * PR
            o_copy(n, r0, min(r0 + PR, L) - r0, k).wait()

    def mm(half, n, i):
        def f():
            lhs = pltpu.bitcast(xh[half][i], BF16)
            rhs = pltpu.bitcast(wh[half][n, i], BF16)
            yy[half][n, i] = jnp.dot(lhs, rhs, preferred_element_type=F32)
        return f

    def body(name, half, tiles, lists, sl=None):
        mms = [mm(half, n, i) for n in tiles for i in range(RH[half])]
        if sl is not None:
            mms = mms[sl]
        with jax.named_scope(name):
            interleave(mms, merge(lists))

    j0 = jnp.int32(0)
    x_start(j0)
    for q in range(WQ):
        w_copy(0, q).start()
    st[...] = jnp.zeros_like(st)

    with jax.named_scope("a0"):
        for c in range(4):
            x_wait(j0, [c])
            def a0(g, carry):
                for p in range(2):
                    drain(a_piece(g, c, p, 0)[0])
                return carry
            lax.fori_loop(0, MB // 16, a0, 0)
        for n in range(1, 4):
            for q in range(WQ):
                w_copy(n, q).start()

    with jax.named_scope("wstage"):
        def wl_factory(n):
            def wl(g, carry):
                for p in range(2):
                    for half in range(2):
                        drain(w_piece(n, g, p, half)[0])
                return carry
            return wl
        for n in range(4):
            wl = wl_factory(n)
            for q in range(WQ):
                w_copy(n, q).wait()
                lax.fori_loop(q * (32 // WQ), (q + 1) * (32 // WQ), wl, 0)

    def main(j, carry):
        @pl.when(j >= 0)
        def _():
            body("E01", 0, (0, 1), [a_pieces(1)])
        @pl.when(j + 1 <= LASTJ)
        def _():
            x_start(j + 1)
        set_shift(j - 1, 2); set_shift(j - 1, 3)
        @pl.when(j + 1 >= 1)
        def _():
            body("O01", 1, (0, 1), [c_pieces(j - 1, 2), c_pieces(j - 1, 3)])
        set_shift(j, 0); set_shift(j, 1)
        @pl.when(j + 2 >= 2)
        def _():
            body("E23", 0, (2, 3), [c_pieces(j, 0), c_pieces(j, 1)])
        @pl.when(j + 1 <= LASTJ)
        def _():
            x_wait(j + 1)
        @pl.when(j < (LASTJ if T2 else LASTJ + 1))
        def _():
            body("O23", 1, (2, 3), [a_pieces(0)])
        return carry
    lax.fori_loop(0, LASTJ + 1, main, 0)

    jl = jnp.int32(LASTJ)
    if T2:
        nm = 2 * RH[1]
        g = st[2, 0, 2, 0, 0] == st[2, 0, 2, 0, 0] + 1.0
        for k in range(2):
            finalize_stats(k)
            @pl.when(jnp.logical_not(g) if k == 0 else (g == False))
            def _():
                body("O23D", 1, (2, 3), [d_pieces(k)], sl=slice(k * nm // 2, (k + 1) * nm // 2))
            o_start_all(k)

    with jax.named_scope("tail"):
        set_shift(jl, 2); set_shift(jl, 3)
        for n in (2, 3):
            for g_, _ in c_pieces(jl, n):
                drain(g_)
        for n in range(2 if T2 else 0, 4):
            finalize_stats(n)
            d_loop(n)
        for n in range(4):
            o_wait_all(n)


@jax.jit
def pallas_standalone__self_sup_conv_stem_wavlm__speech_kernel(x, w, gn_gamma, gn_beta):
    out = pl.pallas_call(
        kernel,
        in_specs=[pl.BlockSpec(memory_space=pl.ANY), pl.BlockSpec(memory_space=pl.ANY),
                  pl.BlockSpec(memory_space=pltpu.VMEM), pl.BlockSpec(memory_space=pltpu.VMEM)],
        out_specs=pl.BlockSpec(memory_space=pl.ANY),
        out_shape=jax.ShapeDtypeStruct((L, 4, 2, 128), BF16),
        scratch_shapes=[pltpu.VMEM((XM, 128), U32)] * 4 + [
            pltpu.VMEM((4, RH[0], 512, 128), U32),
            pltpu.VMEM((4, RH[1], 512, 128), U32),
            pltpu.VMEM((RH[0], MB // 2, 1024), U32),
            pltpu.VMEM((RH[1], MB // 2, 1024), U32),
            pltpu.VMEM((4, RH[0], MB, 128), F32),
            pltpu.VMEM((4, RH[1], MB, 128), F32)] + [pltpu.VMEM((2, LP, 128), F32)] * 4 + [
            pltpu.VMEM((3, 4, 3, 8, 128), F32),
            pltpu.VMEM((4, 2, 2, 8, 128), F32),
            pltpu.SemaphoreType.DMA((4,)),
            pltpu.SemaphoreType.DMA((4, 4)),
            pltpu.SemaphoreType.DMA((4, 4)),
        ],
        compiler_params=pltpu.CompilerParams(vmem_limit_bytes=127 * 1024 * 1024),
    )(x, w, gn_gamma.reshape(1, D), gn_beta.reshape(1, D))
    return out.transpose(2, 0, 1, 3).reshape(2, L, D)
```

```python
import math
import random
import numpy as np
import jax, jax.numpy as jnp
from jax import lax
from jax.experimental import pallas as pl
from jax.experimental.pallas import tpu as pltpu


class Net:
    def __init__(self):
        self.nodes = []
        self.cse = {}

    def _mk(self, key):
        if key in self.cse:
            return self.cse[key]
        self.nodes.append(key)
        self.cse[key] = len(self.nodes) - 1
        return self.cse[key]

    def inp(self, i):
        return (self._mk(('in', i)), 1)

    def neg(self, x):
        return None if x is None else (x[0], -x[1])

    def add(self, x, y):
        if x is None:
            return y
        if y is None:
            return x
        (a, sa), (b, sb) = x, y
        if a == b:
            if sa == sb:
                return self.mul(x, 2.0)
            return None
        if sa == sb:
            if a > b:
                a, b = b, a
            return (self._mk(('add', a, b)), sa)
        if a > b:
            a, b, sa = b, a, sb
        return (self._mk(('sub', a, b)), sa)

    def sub(self, x, y):
        return self.add(x, self.neg(y))

    def mul(self, x, c):
        if x is None or abs(c) < 1e-12:
            return None
        a, s = x
        if c < 0:
            c, s = -c, -s
        if abs(c - 1.0) < 1e-12:
            return (a, s)
        c = float(np.float64(round(c, 14)))
        return (self._mk(('mul', a, c)), s)

    def cadd(self, x, y):
        return (self.add(x[0], y[0]), self.add(x[1], y[1]))

    def csub(self, x, y):
        return (self.sub(x[0], y[0]), self.sub(x[1], y[1]))

    def cmulc(self, x, c, s):
        a, b = x
        if abs(s) < 1e-12:
            return (self.mul(a, c), self.mul(b, c))
        if abs(c) < 1e-12:
            return (self.mul(b, -s), self.mul(a, s))
        if abs(abs(c) - abs(s)) < 1e-12:
            sg = 1.0 if s * c > 0 else -1.0
            re = self.sub(a, self.mul(b, sg))
            im = self.add(b, self.mul(a, sg))
            return (self.mul(re, c), self.mul(im, c))
        re = self.sub(self.mul(a, c), self.mul(b, s))
        im = self.add(self.mul(a, s), self.mul(b, c))
        return (re, im)


def w(k, n):
    ang = -2.0 * math.pi * (k % n) / n
    return math.cos(ang), math.sin(ang)


def cfft(net, z):
    n = len(z)
    if n == 1:
        return [z[0]]
    if n == 2:
        return [net.cadd(z[0], z[1]), net.csub(z[0], z[1])]
    if n % 4 == 0:
        h, q = n // 2, n // 4
        e = [net.cadd(z[t], z[t + h]) for t in range(h)]
        o = [net.csub(z[t], z[t + h]) for t in range(h)]
        z1, z3 = [], []
        for t in range(q):
            a, b = o[t], o[t + q]
            mib = (b[1], net.neg(b[0]))
            p = net.cadd(a, mib)
            m = net.csub(a, mib)
            z1.append(net.cmulc(p, *w(t, n)))
            z3.append(net.cmulc(m, *w(3 * t, n)))
        E = cfft(net, e)
        Z1 = cfft(net, z1)
        Z3 = cfft(net, z3)
        out = [None] * n
        for k in range(h):
            out[2 * k] = E[k]
        for k in range(q):
            out[4 * k + 1] = Z1[k]
            out[4 * k + 3] = Z3[k]
        return out
    if n % 2 == 0:
        m = n // 2
        out = [None] * n
        rows = []
        for t2 in range(m):
            a = z[(2 * t2) % n]
            b = z[(m + 2 * t2) % n]
            rows.append((net.cadd(a, b), net.csub(a, b)))
        for k1 in range(2):
            Z = cfft(net, [rows[t2][k1] for t2 in range(m)])
            for k2 in range(m):
                for k in range(n):
                    if k % 2 == k1 and k % m == k2:
                        out[k] = Z[k2]
        return out
    if n % 3 == 0 and n > 3:
        raise NotImplementedError
    out = []
    p = {t: net.cadd(z[t], z[n - t]) for t in range(1, (n + 1) // 2)}
    q = {t: net.csub(z[t], z[n - t]) for t in range(1, (n + 1) // 2)}
    s = z[0]
    for t in p:
        s = net.cadd(s, p[t])
    out = [None] * n
    out[0] = s
    for k in range(1, (n + 1) // 2):
        A = z[0]
        B = (None, None)
        for t in p:
            c, sn = w(k * t, n)
            A = net.cadd(A, (net.mul(p[t][0], c), net.mul(p[t][1], c)))
            B = net.cadd(B, (net.mul(q[t][1], -sn), net.mul(q[t][0], sn)))
        out[k] = net.cadd(A, B)
        out[n - k] = net.csub(A, B)
    return out


def cfft_pfa(net, z, n1, n2):
    n = n1 * n2
    out = [None] * n
    cols = [cfft_any(net, [z[(n2 * t1 + n1 * t2) % n] for t2 in range(n2)]) for t1 in range(n1)]
    for k2 in range(n2):
        Z = cfft_any(net, [cols[t1][k2] for t1 in range(n1)])
        for k1 in range(n1):
            for k in range(n):
                if k % n1 == k1 and k % n2 == k2:
                    out[k] = Z[k1]
    return out


def cfft5(net, z):
    c1, c2 = math.cos(2 * math.pi / 5), math.cos(4 * math.pi / 5)
    s1, s2 = math.sin(2 * math.pi / 5), math.sin(4 * math.pi / 5)
    t1 = net.cadd(z[1], z[4]); t2 = net.cadd(z[2], z[3])
    t3 = net.csub(z[1], z[4]); t4 = net.csub(z[2], z[3])
    t5 = net.cadd(t1, t2)
    def rm(x, c):
        return (net.mul(x[0], c), net.mul(x[1], c))
    m1 = rm(t5, (c1 + c2) / 2 - 1.0)
    m2 = rm(net.csub(t1, t2), (c1 - c2) / 2)
    y0 = net.cadd(z[0], t5)
    a = net.cadd(y0, m1)
    a1 = net.cadd(a, m2); a2 = net.csub(a, m2)
    m3 = rm(net.cadd(t3, t4), s2)
    m4 = rm(t3, s1 - s2)
    m5 = rm(t4, s1 + s2)
    b1 = net.cadd(m3, m4)
    b2 = net.csub(m3, m5)
    def mi(x):
        return (x[1], net.neg(x[0]))
    return [y0, net.cadd(a1, mi(b1)), net.cadd(a2, mi(b2)), net.csub(a2, mi(b2)), net.csub(a1, mi(b1))]


def rfft5(net, x):
    c1, c2 = math.cos(2 * math.pi / 5), math.cos(4 * math.pi / 5)
    s1, s2 = math.sin(2 * math.pi / 5), math.sin(4 * math.pi / 5)
    t1 = net.add(x[1], x[4]); t2 = net.add(x[2], x[3])
    t3 = net.sub(x[1], x[4]); t4 = net.sub(x[2], x[3])
    t5 = net.add(t1, t2)
    m1 = net.mul(t5, (c1 + c2) / 2 - 1.0)
    m2 = net.mul(net.sub(t1, t2), (c1 - c2) / 2)
    y0 = net.add(x[0], t5)
    a = net.add(y0, m1)
    a1 = net.add(a, m2); a2 = net.sub(a, m2)
    m3 = net.mul(net.add(t3, t4), s2)
    m4 = net.mul(t3, s1 - s2)
    m5 = net.mul(t4, s1 + s2)
    b1 = net.add(m3, m4); b2 = net.sub(m3, m5)
    return [(y0, None), (a1, net.neg(b1)), (a2, net.neg(b2))]


def cfft_any(net, z):
    n = len(z)
    if n == 5:
        return cfft5(net, z)
    if n == 12:
        return cfft_pfa(net, z, 3, 4)
    if n == 10:
        return cfft_pfa(net, z, 5, 2)
    if n == 20:
        return cfft_pfa(net, z, 5, 4)
    if n == 6:
        return cfft_pfa(net, z, 3, 2)
    if n == 14:
        return cfft_pfa(net, z, 7, 2)
    if n == 15:
        return cfft_pfa(net, z, 5, 3)
    return cfft(net, z)


def rfft_pfa(net, x, n1, n2):
    n = n1 * n2
    inner = [rfft(net, [x[(n2 * t1 + n1 * t2) % n] for t1 in range(n1)]) for t2 in range(n2)]
    out = [None] * (n // 2 + 1)
    for k1 in range(n1 // 2 + 1):
        col = [inner[t2][k1] for t2 in range(n2)]
        if all(c[1] is None for c in col):
            Z = rfft(net, [c[0] for c in col])
            Z = Z + [(Z[n2 - k2][0], net.neg(Z[n2 - k2][1])) for k2 in range(len(Z), n2)]
        else:
            Z = cfft_any(net, col)
        for k2 in range(n2):
            k = [k for k in range(n) if k % n1 == k1 and k % n2 == k2][0]
            if k <= n // 2:
                if out[k] is None:
                    out[k] = Z[k2]
            else:
                if out[n - k] is None:
                    out[n - k] = (Z[k2][0], net.neg(Z[k2][1]))
    return out


PFA = {40: (8, 5), 20: (4, 5), 24: (8, 3), 48: (16, 3), 12: (4, 3), 56: (8, 7), 10: (2, 5), 6: (2, 3), 60: (4, 15), 15: (3, 5), 44: (4, 11), 36: (4, 9)}
USE_PFA = True


def rfft(net, x):
    n = len(x)
    if USE_PFA and n in PFA:
        return rfft_pfa(net, x, *PFA[n])
    if n == 1:
        return [(x[0], None)]
    if n == 2:
        return [(net.add(x[0], x[1]), None), (net.sub(x[0], x[1]), None)]
    if n % 4 == 0:
        h, q = n // 2, n // 4
        e = [net.add(x[t], x[t + h]) for t in range(h)]
        o = [net.sub(x[t], x[t + h]) for t in range(h)]
        z = [net.cmulc((o[t], net.neg(o[t + q])), *w(t, n)) for t in range(q)]
        E = rfft(net, e)
        Z = cfft_any(net, z)
        out = [None] * (h + 1)
        for k in range(len(E)):
            out[2 * k] = E[k]
        for k in range(q):
            f = 4 * k + 1
            if f <= h:
                out[f] = Z[k]
            else:
                out[n - f] = (Z[k][0], net.neg(Z[k][1]))
        return out
    if n % 2 == 0:
        m = n // 2
        e = [net.add(x[t], x[t + m]) for t in range(m)]
        o = [net.sub(x[t], x[t + m]) for t in range(m)]
        E = rfft(net, e)
        op = [o[t] if t % 2 == 0 else net.neg(o[t]) for t in range(m)]
        O = rfft(net, op)
        out = [None] * (m + 1)
        for k in range(len(E)):
            out[2 * k] = E[k]
        for f in range(1, m + 1, 2):
            j = ((f - m) // 2) % m
            if j <= m // 2:
                out[f] = O[j]
            else:
                out[f] = (O[m - j][0], net.neg(O[m - j][1]))
        return out
    if n == 5:
        return rfft5(net, x)
    p = {t: net.add(x[t], x[n - t]) for t in range(1, (n + 1) // 2)}
    q = {t: net.sub(x[t], x[n - t]) for t in range(1, (n + 1) // 2)}
    s = x[0]
    for t in p:
        s = net.add(s, p[t])
    out = [(s, None)]
    for k in range(1, (n + 1) // 2):
        A = x[0]
        B = None
        for t in p:
            c, sn = w(k * t, n)
            A = net.add(A, net.mul(p[t], c))
            B = net.add(B, net.mul(q[t], sn))
        out.append((A, B))
    return out


class Prog:
    def __init__(self, net, outputs):
        order = []
        seen = set()

        def visit(n):
            if n in seen:
                return
            seen.add(n)
            k = net.nodes[n]
            if k[0] in ('add', 'sub'):
                visit(k[1]); visit(k[2])
            elif k[0] == 'mul':
                visit(k[1])
            order.append(n)
        for o in outputs:
            if o is not None:
                visit(o[0])
        self.net = net
        self.order = order
        self.outputs = outputs

    def count(self):
        c = {'add': 0, 'sub': 0, 'mul': 0, 'in': 0}
        for n in self.order:
            c[self.net.nodes[n][0]] += 1
        return c

    def run(self, load, emit=None):
        vals = {}
        for n in self.order:
            k = self.net.nodes[n]
            if k[0] == 'in':
                vals[n] = load(k[1])
            elif k[0] == 'add':
                vals[n] = vals[k[1]] + vals[k[2]]
            elif k[0] == 'sub':
                vals[n] = vals[k[1]] - vals[k[2]]
            else:
                vals[n] = vals[k[1]] * k[2]
        return [None if o is None else vals[o[0]] for o in self.outputs]

    @property
    def signs(self):
        return [0 if o is None else o[1] for o in self.outputs]

    def matrix(self, n_in, signed=True):
        eye = np.eye(n_in)
        res = self.run(lambda i: eye[i])
        rows = []
        for r, s in zip(res, self.signs):
            rows.append(np.zeros(n_in) if r is None else (r * s if signed else r))
        return np.stack(rows)


def transpose(net, outputs, wanted_inputs):
    prog = Prog(net, outputs)
    live = set(prog.order)
    consumers = {n: [] for n in prog.order}
    for n in prog.order:
        k = net.nodes[n]
        if k[0] == 'add':
            consumers[k[1]].append((n, 1.0)); consumers[k[2]].append((n, 1.0))
        elif k[0] == 'sub':
            consumers[k[1]].append((n, 1.0)); consumers[k[2]].append((n, -1.0))
        elif k[0] == 'mul':
            consumers[k[1]].append((n, k[2]))
    outmap = {}
    for r, o in enumerate(outputs):
        if o is not None:
            outmap.setdefault(o[0], []).append((r, o[1]))
    tn = Net()
    memo = {}

    def adj(n):
        if n in memo:
            return memo[n]
        acc = None
        for r, s in outmap.get(n, []):
            v = tn.inp(r)
            acc = tn.add(acc, v if s > 0 else tn.neg(v))
        for c, coef in consumers[n]:
            acc = tn.add(acc, tn.mul(adj(c), coef))
        memo[n] = acc
        return acc
    outs = []
    for i in wanted_inputs:
        key = ('in', i)
        if key in net.cse and net.cse[key] in live:
            outs.append(adj(net.cse[key]))
        else:
            outs.append(None)
    return tn, outs


def build(N, taps, scale=True, variant=0):
    hop = N - taps + 1
    na = Net()
    U = rfft(na, [na.inp(t) for t in range(N)])
    a_out = [U[0][0], U[N // 2][0]]
    bins = list(range(1, N // 2))
    for k in bins:
        a, b = U[k]
        if variant == 0:
            a_out += [na.add(a, b), a, b]
        else:
            a_out += [a, na.sub(b, a), na.add(a, b)]
    nc = Net()
    V = rfft(nc, [nc.inp(t) for t in range(N)])
    c_out = [V[0][0], V[N // 2][0]]
    for k in bins:
        al, be = V[k]
        c_out += [nc.add(al, be), be, nc.neg(al)]
    tn, c_res = transpose(nc, c_out, list(range(hop)))
    def mkb(ntaps):
        nb = Net()
        Wf = rfft(nb, [nb.inp(t) if t < ntaps else None for t in range(N)])
        s0 = 1.0 / N if scale else 0.5
        b_out = [nb.mul(Wf[0][0], s0), nb.mul(Wf[N // 2][0], s0)]
        for k in bins:
            c = Wf[k][0]
            d = nb.neg(Wf[k][1])
            sc = 2.0 / N if scale else 1.0
            if variant == 0:
                b_out += [nb.mul(c, sc), nb.mul(nb.sub(d, c), sc), nb.mul(nb.add(c, d), sc)]
            else:
                b_out += [nb.mul(nb.add(c, d), sc), nb.mul(c, sc), nb.mul(d, sc)]
        return nb, b_out
    nb, b_out = mkb(taps)
    nb1, b1_out = mkb(taps - 1)
    return dict(N=N, hop=hop, taps=taps, na=na, a_out=a_out, nb=nb, b_out=b_out, nb1=nb1, b1_out=b1_out,
                tn=tn, c_res=c_res, bins=bins)


def max_live(net, order, outputs, out_at_once=True):
    uses = {n: 0 for n in order}
    for n in order:
        k = net.nodes[n]
        for a in ([k[1], k[2]] if k[0] in ('add', 'sub') else [k[1]] if k[0] == 'mul' else []):
            uses[a] += 1
    live = set(); peak = 0; tot = 0
    rem = dict(uses)
    for n in order:
        k = net.nodes[n]
        live.add(n)
        peak = max(peak, len(live))
        for a in set([k[1], k[2]] if k[0] in ('add', 'sub') else [k[1]] if k[0] == 'mul' else []):
            rem[a] -= (1 if k[0] == 'mul' or k[1] != k[2] else 2)
            if rem[a] == 0:
                live.discard(a)
        if rem[n] == 0:
            live.discard(n)
        tot += len(live)
    return peak, tot / len(order)


def min_live_order(net, outputs, seed=0, tries=200):
    base = Prog(net, outputs).order
    nodes = set(base)
    def operands(n):
        k = net.nodes[n]
        return [k[1], k[2]] if k[0] in ('add', 'sub') else [k[1]] if k[0] == 'mul' else []
    consumers = {n: [] for n in base}
    for n in base:
        for a in set(operands(n)):
            consumers[a].append(n)
    best = (max_live(net, base, outputs), base)
    rnd = random.Random(seed)
    pos = {n: i for i, n in enumerate(base)}
    for it in range(tries):
        done = set(); order = []
        live = set()
        remc = {n: len(consumers[n]) for n in base}
        isin = {n: net.nodes[n][0] == 'in' for n in base}
        def ready(n):
            return n not in done and not isin[n] and all((a in done) or isin[a] for a in operands(n))
        noise = rnd.random() * 1.5
        work = [n for n in base if not isin[n]]
        left = set(work)
        while left:
            cands = [n for n in left if ready(n)]
            def score(n):
                ops = set(operands(n))
                newloads = sum(1 for a in ops if a not in done)
                kills = sum(1 for a in ops if remc[a] == 1)
                born = 0 if remc[n] == 0 else 1
                return (newloads + born - kills) + noise * rnd.random() + 1e-4 * pos[n]
            n = min(cands, key=score)
            for a in sorted(set(operands(n)), key=lambda a: pos[a]):
                if a not in done:
                    done.add(a); order.append(a)
                remc[a] -= 1
            done.add(n); order.append(n); left.discard(n)
        ml = max_live(net, order, outputs)
        if ml < best[0]:
            best = (ml, order)
    return best


def solve_signs(G, iters=200000, seed=0):
    rnd = random.Random(seed)
    nets = {'A': (G['na'], G['a_out']), 'B': (G['nb'], G['b_out']), 'C': (G['tn'], G['c_res'])}
    order = {k: Prog(*v).order for k, v in nets.items()}
    R = len(G['a_out'])
    sig = {}
    for k in 'ABC':
        for n in order[k]:
            sig[(k, n)] = 1
    fixed = set()
    for k in 'AB':
        for n in order[k]:
            if nets[k][0].nodes[n][0] == 'in':
                fixed.add((k, n))
    for o in G['c_res']:
        sig[('C', o[0])] = o[1]; fixed.add(('C', o[0]))
    cin = {}
    for n in order['C']:
        nd = G['tn'].nodes[n]
        if nd[0] == 'in':
            cin[nd[1]] = n; fixed.add(('C', n))
    def cin_sign(r):
        a, b = G['a_out'][r], G['b_out'][r]
        return (sig[('A', a[0])] * a[1]) * (sig[('B', b[0])] * b[1])
    outmap = {}
    for r in range(R):
        outmap.setdefault(('A', G['a_out'][r][0]), []).append(r)
        outmap.setdefault(('B', G['b_out'][r][0]), []).append(r)
    def refresh():
        for r, n in cin.items():
            sig[('C', n)] = cin_sign(r)
    clauses = []
    for k in 'ABC':
        net = nets[k][0]
        for n in order[k]:
            nd = net.nodes[n]
            if nd[0] in ('add', 'sub'):
                clauses.append((k, n, nd[1], nd[2], 1 if nd[0] == 'add' else -1))
    occ = {}
    for ci, (k, n, a, b, cb) in enumerate(clauses):
        for v in (n, a, b):
            occ.setdefault((k, v), []).append(ci)
    def viol(ci):
        k, n, a, b, cb = clauses[ci]
        return sig[(k, n)] * sig[(k, a)] < 0 and sig[(k, n)] * cb * sig[(k, b)] < 0
    def flip(v):
        sig[v] = -sig[v]
        for r in outmap.get(v, []):
            if r in cin:
                sig[('C', cin[r])] = cin_sign(r)
    def affected(v):
        cs = set(occ.get(v, []))
        for r in outmap.get(v, []):
            if r in cin:
                cs.update(occ.get(('C', cin[r]), []))
        return cs
    flippers = {}
    for v, rs in outmap.items():
        for r in rs:
            if r in cin:
                flippers.setdefault(('C', cin[r]), []).append(v)
    refresh()
    bad = {ci for ci in range(len(clauses)) if viol(ci)}
    best = (len(bad), dict(sig))
    for it in range(iters):
        if not bad:
            break
        ci = rnd.choice(list(bad))
        k, n, a, b, cb = clauses[ci]
        cands = []
        for v in ((k, n), (k, a), (k, b)):
            if v in fixed:
                cands += flippers.get(v, [])
            else:
                cands.append(v)
        cands = [v for v in cands if v not in fixed]
        if not cands:
            continue
        def delta(v):
            cs = affected(v)
            before = sum(viol(c) for c in cs)
            flip(v)
            after = sum(viol(c) for c in cs)
            flip(v)
            return after - before
        if rnd.random() < 0.2:
            v = rnd.choice(cands)
        else:
            v = min(cands, key=lambda v: (delta(v), rnd.random()))
        cs = affected(v)
        flip(v)
        for c in cs:
            if viol(c): bad.add(c)
            else: bad.discard(c)
        if len(bad) < best[0]:
            best = (len(bad), dict(sig))
    nb, sg = best
    return ({n: s for (k, n), s in sg.items() if k == 'A'}, {n: s for (k, n), s in sg.items() if k == 'B'},
            {n: s for (k, n), s in sg.items() if k == 'C'}, nb)


class FixedProg:
    def __init__(self, net, outputs, sig, order=None):
        self.net, self.outputs, self.sig = net, outputs, sig
        self.order = order if order is not None else Prog(net, outputs).order
    def count(self):
        c = {'add': 0, 'sub': 0, 'mul': 0, 'in': 0}
        for n in self.order:
            c[self.net.nodes[n][0]] += 1
        return c


N, TAPS = 40, 16
G = build(N, TAPS, scale=False, variant=1)
HOP = G['hop']; R = len(G['a_out'])
T, D, K = 16000, 512, 31
L = (T - K) // 2 + 1
MB = 64; NCH = -(-L // (HOP * MB))
CH = HOP * MB
XM = CH + 16
LP = NCH * CH
TM = T // 2
LAST_M = TM - (NCH - 1) * CH
HS = 2.0 / N
T2 = 1
U32, F32, BF16 = jnp.uint32, jnp.float32, jnp.bfloat16

bins = G['bins']
ev = [0, 1] + [2 + 3 * i + q for i, k in enumerate(bins) if k % 2 == 0 for q in range(3)]
od = [2 + 3 * i + q for i, k in enumerate(bins) if k % 2 == 1 for q in range(3)]
if (N // 2) % 2 == 1:
    ev.remove(1); od = [1] + od
IDX = (ev, od)
RH = (len(ev), len(od))
LOC = {}
for hf in range(2):
    for i, r in enumerate(IDX[hf]):
        LOC[r] = (hf, i)
SA, SB, SC, NBAD = solve_signs(G)
assert NBAD == 0
def mkprog(net, outs, sig):
    return FixedProg(net, outs, sig, order=min_live_order(net, outs, tries=100)[1])
PA = [mkprog(G['na'], [G['a_out'][r] for r in idx], SA) for idx in IDX]
PB = [mkprog(G['nb'], [G['b_out'][r] for r in idx], SB) for idx in IDX]
PC = mkprog(G['tn'], G['c_res'], SC)


def run_gen(prog, loads, sink):
    nsets = len(loads)
    vals = [dict() for _ in range(nsets)]
    sig = prog.sig
    outs = {}
    for r, o in enumerate(prog.outputs):
        outs.setdefault(o[0], []).append(r)
    for n in prog.order:
        k = prog.net.nodes[n]
        for s in range(nsets):
            v = vals[s]
            if k[0] == 'in':
                v[n] = loads[s](k[1])
            elif k[0] == 'mul':
                v[n] = v[k[1]] * (k[2] * sig[n] * sig[k[1]])
            else:
                a, b = k[1], k[2]
                cb = 1 if k[0] == 'add' else -1
                p, q = sig[n] * sig[a], sig[n] * cb * sig[b]
                if p > 0 and q > 0: v[n] = v[a] + v[b]
                elif p > 0: v[n] = v[a] - v[b]
                elif q > 0: v[n] = v[b] - v[a]
                else: v[n] = -(v[a] + v[b])
            yield 1
        for r in outs.get(n, []):
            yield from sink(r, [vals[s][n] for s in range(nsets)])


def drain(gen):
    for _ in gen:
        pass


def unpack(wd, hi):
    wd = (wd & jnp.uint32(0xffff0000)) if hi else (wd << 16)
    return lax.bitcast_convert_type(wd, F32)


def pack(lo, hi):
    return pltpu.pack_elementwise([lo, hi], packed_dtype=BF16)


def prog_weight(prog, nsets, per_out):
    return len(prog.order) * nsets + len(prog.outputs) * per_out


def interleave(mms, gens_weights):
    total = sum(w for _, w in gens_weights)
    def allops():
        for g, _ in gens_weights:
            yield from g
    gen = allops()
    e = 0; done = False
    for i, mm in enumerate(mms):
        mm()
        tgt = (i + 1) * total // len(mms)
        while not done and e < tgt:
            try:
                e += next(gen)
            except StopIteration:
                done = True
    for _ in gen:
        pass


def merge(lists):
    lists = [l for l in lists if l]
    out = []
    pos = [0] * len(lists)
    tot = sum(len(l) for l in lists)
    for _ in range(tot):
        i = min((i for i in range(len(lists)) if pos[i] < len(lists[i])), key=lambda i: (pos[i] + 0.5) / len(lists[i]))
        out.append(lists[i][pos[i]]); pos[i] += 1
    return out


C0 = math.sqrt(2.0 / math.pi)
def gelu_half(zh):
    u = zh * (zh * zh * (8.0 * C0 * 0.044715) + 2.0 * C0)
    return zh * jnp.tanh(u) + zh


def kernel(x_hbm, w_hbm, gam_ref, bet_ref, out_hbm,
           xb0, xb1, xb2, xb3, we, wo, xe, xo, ye, yo, h0, h1, h2, h3, st, nrm, gsm, xsem, wsem, osem):
    xb = (xb0, xb1, xb2, xb3)
    wh = (we, wo); xh = (xe, xo); yy = (ye, yo)
    hh = (h0, h1, h2, h3)
    x32 = x_hbm.bitcast(U32)
    w32 = w_hbm.bitcast(F32)
    o32 = out_hbm.bitcast(F32)
    LASTJ = 2 * NCH - 1

    def x_copy(j, c, full):
        b = j // NCH
        cj = j % NCH
        rows = XM if full else LAST_M
        return pltpu.make_async_copy(
            x32.at[b, pl.ds(pl.multiple_of(cj * CH, 8), rows), pl.ds(c * 128, 128)],
            xb[c].at[pl.ds(0, rows), :], xsem.at[c])

    def x_start(j):
        cj = j % NCH
        @pl.when(cj < NCH - 1)
        def _():
            for c in range(4):
                x_copy(j, c, True).start()
        @pl.when(cj == NCH - 1)
        def _():
            for c in range(4):
                x_copy(j, c, False).start()
                xb[c][pl.ds(LAST_M, XM - LAST_M), :] = jnp.zeros((XM - LAST_M, 128), U32)

    def x_wait(j, cs=range(4)):
        cj = j % NCH
        @pl.when(cj < NCH - 1)
        def _():
            for c in cs:
                x_copy(j, c, True).wait()
        @pl.when(cj == NCH - 1)
        def _():
            for c in cs:
                x_copy(j, c, False).wait()

    WQ = 4
    def w_copy(n, q):
        dst = hh[n].at[1, pl.ds(0, K * 256), :].reshape(K, 256, 128)
        r = 256 // WQ
        return pltpu.make_async_copy(w32.at[:, pl.ds(q * r, r), pl.ds(n * 128, 128)], dst.at[:, pl.ds(q * r, r), :], wsem.at[n, q])

    def o_copy(n, r0, rows, k):
        return pltpu.make_async_copy(hh[n].at[0, pl.ds(r0, rows), :], o32.at[pl.ds(r0, rows), n, 0, :], osem.at[n, k])

    def a_piece(g, c, p, half):
        dyn = not isinstance(g, int)
        base = pl.multiple_of(g * (16 * HOP), 8) if dyn else g * (16 * HOP)
        row = pl.multiple_of(g * 8, 8) if dyn else g * 8
        xw = xb[c].at[pl.ds(base, 16 * HOP + 16), :]
        def mkload(o):
            return lambda t: unpack(xw[pl.ds(t + o * HOP, 8, stride=2 * HOP), :], p)
        def sink(i, vs):
            xh[half][i, pl.ds(row, 8), p * 512 + c * 128:p * 512 + (c + 1) * 128] = pack(vs[0], vs[1])
            yield 1
        return run_gen(PA[half], [mkload(0), mkload(1)], sink), prog_weight(PA[half], 2, 1)

    def a_pieces(half):
        return [a_piece(g, c, p, half) for c in range(4) for g in range(MB // 16) for p in range(2)]

    def w_piece(n, g, p, half):
        dyn = not isinstance(g, int)
        row = pl.multiple_of(g * 8, 8) if dyn else g * 8
        cache = {}
        def word(j):
            if j not in cache:
                cache[j] = lax.bitcast_convert_type(hh[n][1, pl.ds((2 * j + p) * 256 + row, 8), :], U32)
            return cache[j]
        def mkload(hi):
            def load(j):
                if 2 * j + p >= K:
                    return jnp.zeros((8, 128), F32)
                return unpack(word(j), hi)
            return load
        def sink(i, vs):
            wh[half][n, i, pl.ds(p * 256 + row, 8), :] = pack(vs[0], vs[1])
            yield 1
        return run_gen(PB[half], [mkload(0), mkload(1)], sink), prog_weight(PB[half], 2, 1)

    def c_pieces(j, n):
        if isinstance(j, int):
            b, cj = j // NCH, j % NCH
            slot = b
        else:
            valid = j >= 0
            b = jnp.where(valid, j // NCH, 0)
            cj = jnp.where(valid, j % NCH, NCH - 1)
            slot = jnp.where(valid, b, 2)
        state = {}
        def col(g):
            if g == 0:
                state['c'] = st[slot, n, 2]; state['a1'] = st[slot, n, 0]; state['a2'] = st[slot, n, 1]
            base = cj * CH + g * (8 * HOP)
            if not isinstance(j, int):
                base = pl.multiple_of(base, 8)
            hs = hh[n].at[b, pl.ds(base, 8 * HOP), :]
            def sink(t, vs):
                hs[pl.ds(t, 8, stride=HOP), :] = vs[0]
                d = vs[0] - state['c']
                state['a1'] = state['a1'] + d
                state['a2'] = state['a2'] + d * d
                yield 4
            yield from run_gen(PC, [lambda r: yy[LOC[r][0]][n, LOC[r][1], g * 8:(g + 1) * 8, :]], sink)
            if g == MB // 8 - 1:
                st[slot, n, 0] = state['a1']; st[slot, n, 1] = state['a2']
        return [(col(g), prog_weight(PC, 1, 4)) for g in range(MB // 8)]

    def set_shift(j, n):
        @pl.when(jnp.logical_and(j >= 0, j % NCH == 0))
        def _():
            st[j // NCH, n, 2] = jnp.broadcast_to(ye[n, LOC[0][1], 0:1, :], (8, 128))

    def finalize_stats(n):
        sub = lax.broadcasted_iota(jnp.int32, (8, 128), 0)
        for b in range(2):
            c = st[b, n, 2]
            r0 = (L // 8) * 8
            c1 = jnp.zeros((8, 128), F32); c2 = jnp.zeros((8, 128), F32)
            for r in range(r0, LP, 8):
                d = hh[n][b, r:r + 8, :] - c
                if r < L:
                    d = jnp.where(sub >= L - r, d, 0.0)
                c1 = c1 + d; c2 = c2 + d * d
            s1 = jnp.sum(st[b, n, 0] - c1, axis=0, keepdims=True)
            s2 = jnp.sum(st[b, n, 1] - c2, axis=0, keepdims=True)
            md = s1 * (1.0 / L)
            var = (s2 * (1.0 / L) - md * md) * (HS * HS)
            mu = c[0:1] + md
            a = (HS * lax.rsqrt(var + 1e-5)) * gam_ref[:, n * 128:(n + 1) * 128].astype(F32)
            bb = bet_ref[:, n * 128:(n + 1) * 128].astype(F32) - mu * a
            nrm[n, b, 0] = jnp.broadcast_to(0.5 * a, (8, 128))
            nrm[n, b, 1] = jnp.broadcast_to(0.5 * bb, (8, 128))

    def d_vreg(n, r, cs):
        a0, b0, a1, b1 = cs
        z0 = gelu_half(hh[n][0, pl.ds(r, 8), :] * a0 + b0)
        z1 = gelu_half(hh[n][1, pl.ds(r, 8), :] * a1 + b1)
        hh[n][0, pl.ds(r, 8), :] = lax.bitcast_convert_type(pack(z0, z1), F32)

    def d_consts(n):
        return nrm[n, 0, 0], nrm[n, 0, 1], nrm[n, 1, 0], nrm[n, 1, 1]

    def d_pieces(n, ra=0, rb=LP):
        state = {}
        def piece(r0, r1):
            if 'cs' not in state:
                state['cs'] = d_consts(n)
            for r in range(r0, r1, 8):
                d_vreg(n, r, state['cs'])
                yield 19
        P = 200
        return [(piece(r, min(r + P, rb)), 19 * (min(r + P, rb) - r) // 8) for r in range(ra, rb, P)]

    def fin_piece(n):
        def gen():
            finalize_stats(n)
            yield 100
        return [(gen(), 100)]

    NPC = 4
    PR = -(-(-(-L // NPC)) // 8) * 8
    def d_loop(n):
        cs = d_consts(n)
        UN = 5
        for k in range(NPC):
            r0 = k * PR; r1 = min(r0 + PR, LP)
            nv = -(-(r1 - r0) // 8)
            assert nv % UN == 0, nv
            def body(i, carry):
                for u in range(UN):
                    d_vreg(n, pl.multiple_of(r0 + (i * UN + u) * 8, 8), cs)
                return carry
            lax.fori_loop(0, nv // UN, body, 0)
            o_copy(n, r0, min(r0 + PR, L) - r0, k).start()

    def o_start_all(n):
        for k in range(NPC):
            r0 = k * PR
            o_copy(n, r0, min(r0 + PR, L) - r0, k).start()

    def o_wait_all(n):
        for k in range(NPC):
            r0 = k * PR
            o_copy(n, r0, min(r0 + PR, L) - r0, k).wait()

    def mm(half, n, i):
        def f():
            lhs = pltpu.bitcast(xh[half][i], BF16)
            rhs = pltpu.bitcast(wh[half][n, i], BF16)
            yy[half][n, i] = jnp.dot(lhs, rhs, preferred_element_type=F32)
        return f

    def body(name, half, tiles, lists, sl=None):
        mms = [mm(half, n, i) for n in tiles for i in range(RH[half])]
        if sl is not None:
            mms = mms[sl]
        with jax.named_scope(name):
            interleave(mms, merge(lists))

    j0 = jnp.int32(0)
    gsm[0] = jnp.int32(0)
    x_start(j0)
    for q in range(WQ):
        w_copy(0, q).start()
    st[...] = jnp.zeros_like(st)

    with jax.named_scope("a0"):
        for c in range(4):
            x_wait(j0, [c])
            def a0(g, carry):
                for p in range(2):
                    drain(a_piece(g, c, p, 0)[0])
                return carry
            lax.fori_loop(0, MB // 16, a0, 0)
        for n in range(1, 4):
            for q in range(WQ):
                w_copy(n, q).start()

    with jax.named_scope("wstage"):
        def wl_factory(n):
            def wl(g, carry):
                for p in range(2):
                    for half in range(2):
                        drain(w_piece(n, g, p, half)[0])
                return carry
            return wl
        for n in range(4):
            wl = wl_factory(n)
            for q in range(WQ):
                w_copy(n, q).wait()
                lax.fori_loop(q * (32 // WQ), (q + 1) * (32 // WQ), wl, 0)

    def main(j, carry):
        @pl.when(j >= 0)
        def _():
            body("E01", 0, (0, 1), [a_pieces(1)])
        @pl.when(j + 1 <= LASTJ)
        def _():
            x_start(j + 1)
        set_shift(j - 1, 2); set_shift(j - 1, 3)
        @pl.when(j + 1 >= 1)
        def _():
            body("O01", 1, (0, 1), [c_pieces(j - 1, 2), c_pieces(j - 1, 3)])
        @pl.when(j < (LASTJ if T2 else LASTJ + 1))
        def _():
            set_shift(j, 0); set_shift(j, 1)
        @pl.when(j + 2 < (LASTJ if T2 else LASTJ + 1) + 2)
        def _():
            body("E23", 0, (2, 3), [c_pieces(j, 0), c_pieces(j, 1)])
        @pl.when(j + 1 <= LASTJ)
        def _():
            x_wait(j + 1)
        @pl.when(j < (LASTJ if T2 else LASTJ + 1))
        def _():
            body("O23", 1, (2, 3), [a_pieces(0)])
        return carry
    lax.fori_loop(0, LASTJ + 1, main, 0)

    jl = jnp.int32(LASTJ)
    if T2:
        gd = gsm[0]
        set_shift(jl, 0); set_shift(jl, 1)
        HR = 2 * PR
        def o_start(n, ks):
            for k in ks:
                r0 = k * PR
                o_copy(n, r0, min(r0 + PR, L) - r0, k).start()
        @pl.when(gd >= 0)
        def _():
            body("E2D", 0, (2,), [c_pieces(LASTJ, 0) + fin_piece(0) + d_pieces(0, 0, HR)])
        o_start(0, (0, 1))
        @pl.when(gd + 1 >= 1)
        def _():
            body("E3D", 0, (3,), [d_pieces(0, HR, LP) + c_pieces(LASTJ, 1) + fin_piece(1)])
        o_start(0, (2, 3))
        @pl.when(gd + 2 >= 2)
        def _():
            body("O2D", 1, (2,), [d_pieces(1, 0, HR)])
        o_start(1, (0, 1))
        @pl.when(gd + 3 >= 3)
        def _():
            body("O3D", 1, (3,), [d_pieces(1, HR, LP)])
        o_start(1, (2, 3))

    with jax.named_scope("tail"):
        set_shift(jl, 2); set_shift(jl, 3)
        for n in (2, 3):
            for g_, _ in c_pieces(jl, n):
                drain(g_)
        for n in range(2 if T2 else 0, 4):
            finalize_stats(n)
            d_loop(n)
        for n in range(4):
            o_wait_all(n)


@jax.jit
def pallas_standalone__self_sup_conv_stem_wavlm__speech_kernel(x, w, gn_gamma, gn_beta):
    out = pl.pallas_call(
        kernel,
        in_specs=[pl.BlockSpec(memory_space=pl.ANY), pl.BlockSpec(memory_space=pl.ANY),
                  pl.BlockSpec(memory_space=pltpu.VMEM), pl.BlockSpec(memory_space=pltpu.VMEM)],
        out_specs=pl.BlockSpec(memory_space=pl.ANY),
        out_shape=jax.ShapeDtypeStruct((L, 4, 2, 128), BF16),
        scratch_shapes=[pltpu.VMEM((XM, 128), U32)] * 4 + [
            pltpu.VMEM((4, RH[0], 512, 128), U32),
            pltpu.VMEM((4, RH[1], 512, 128), U32),
            pltpu.VMEM((RH[0], MB // 2, 1024), U32),
            pltpu.VMEM((RH[1], MB // 2, 1024), U32),
            pltpu.VMEM((4, RH[0], MB, 128), F32),
            pltpu.VMEM((4, RH[1], MB, 128), F32)] + [pltpu.VMEM((2, LP, 128), F32)] * 4 + [
            pltpu.VMEM((3, 4, 3, 8, 128), F32),
            pltpu.VMEM((4, 2, 2, 8, 128), F32),
            pltpu.SMEM((1,), jnp.int32),
            pltpu.SemaphoreType.DMA((4,)),
            pltpu.SemaphoreType.DMA((4, 4)),
            pltpu.SemaphoreType.DMA((4, 4)),
        ],
        compiler_params=pltpu.CompilerParams(vmem_limit_bytes=127 * 1024 * 1024),
    )(x, w, gn_gamma.reshape(1, D), gn_beta.reshape(1, D))
    return out.transpose(2, 0, 1, 3).reshape(2, L, D)
```

```python
import math
import random
import numpy as np
import jax, jax.numpy as jnp
from jax import lax
from jax.experimental import pallas as pl
from jax.experimental.pallas import tpu as pltpu


class Net:
    def __init__(self):
        self.nodes = []
        self.cse = {}

    def _mk(self, key):
        if key in self.cse:
            return self.cse[key]
        self.nodes.append(key)
        self.cse[key] = len(self.nodes) - 1
        return self.cse[key]

    def inp(self, i):
        return (self._mk(('in', i)), 1)

    def neg(self, x):
        return None if x is None else (x[0], -x[1])

    def add(self, x, y):
        if x is None:
            return y
        if y is None:
            return x
        (a, sa), (b, sb) = x, y
        if a == b:
            if sa == sb:
                return self.mul(x, 2.0)
            return None
        if sa == sb:
            if a > b:
                a, b = b, a
            return (self._mk(('add', a, b)), sa)
        if a > b:
            a, b, sa = b, a, sb
        return (self._mk(('sub', a, b)), sa)

    def sub(self, x, y):
        return self.add(x, self.neg(y))

    def mul(self, x, c):
        if x is None or abs(c) < 1e-12:
            return None
        a, s = x
        if c < 0:
            c, s = -c, -s
        if abs(c - 1.0) < 1e-12:
            return (a, s)
        c = float(np.float64(round(c, 14)))
        return (self._mk(('mul', a, c)), s)

    def cadd(self, x, y):
        return (self.add(x[0], y[0]), self.add(x[1], y[1]))

    def csub(self, x, y):
        return (self.sub(x[0], y[0]), self.sub(x[1], y[1]))

    def cmulc(self, x, c, s):
        a, b = x
        if abs(s) < 1e-12:
            return (self.mul(a, c), self.mul(b, c))
        if abs(c) < 1e-12:
            return (self.mul(b, -s), self.mul(a, s))
        if abs(abs(c) - abs(s)) < 1e-12:
            sg = 1.0 if s * c > 0 else -1.0
            re = self.sub(a, self.mul(b, sg))
            im = self.add(b, self.mul(a, sg))
            return (self.mul(re, c), self.mul(im, c))
        re = self.sub(self.mul(a, c), self.mul(b, s))
        im = self.add(self.mul(a, s), self.mul(b, c))
        return (re, im)


def w(k, n):
    ang = -2.0 * math.pi * (k % n) / n
    return math.cos(ang), math.sin(ang)


def cfft(net, z):
    n = len(z)
    if n == 1:
        return [z[0]]
    if n == 2:
        return [net.cadd(z[0], z[1]), net.csub(z[0], z[1])]
    if n % 4 == 0:
        h, q = n // 2, n // 4
        e = [net.cadd(z[t], z[t + h]) for t in range(h)]
        o = [net.csub(z[t], z[t + h]) for t in range(h)]
        z1, z3 = [], []
        for t in range(q):
            a, b = o[t], o[t + q]
            mib = (b[1], net.neg(b[0]))
            p = net.cadd(a, mib)
            m = net.csub(a, mib)
            z1.append(net.cmulc(p, *w(t, n)))
            z3.append(net.cmulc(m, *w(3 * t, n)))
        E = cfft(net, e)
        Z1 = cfft(net, z1)
        Z3 = cfft(net, z3)
        out = [None] * n
        for k in range(h):
            out[2 * k] = E[k]
        for k in range(q):
            out[4 * k + 1] = Z1[k]
            out[4 * k + 3] = Z3[k]
        return out
    if n % 2 == 0:
        m = n // 2
        out = [None] * n
        rows = []
        for t2 in range(m):
            a = z[(2 * t2) % n]
            b = z[(m + 2 * t2) % n]
            rows.append((net.cadd(a, b), net.csub(a, b)))
        for k1 in range(2):
            Z = cfft(net, [rows[t2][k1] for t2 in range(m)])
            for k2 in range(m):
                for k in range(n):
                    if k % 2 == k1 and k % m == k2:
                        out[k] = Z[k2]
        return out
    if n % 3 == 0 and n > 3:
        raise NotImplementedError
    out = []
    p = {t: net.cadd(z[t], z[n - t]) for t in range(1, (n + 1) // 2)}
    q = {t: net.csub(z[t], z[n - t]) for t in range(1, (n + 1) // 2)}
    s = z[0]
    for t in p:
        s = net.cadd(s, p[t])
    out = [None] * n
    out[0] = s
    for k in range(1, (n + 1) // 2):
        A = z[0]
        B = (None, None)
        for t in p:
            c, sn = w(k * t, n)
            A = net.cadd(A, (net.mul(p[t][0], c), net.mul(p[t][1], c)))
            B = net.cadd(B, (net.mul(q[t][1], -sn), net.mul(q[t][0], sn)))
        out[k] = net.cadd(A, B)
        out[n - k] = net.csub(A, B)
    return out


def cfft_pfa(net, z, n1, n2):
    n = n1 * n2
    out = [None] * n
    cols = [cfft_any(net, [z[(n2 * t1 + n1 * t2) % n] for t2 in range(n2)]) for t1 in range(n1)]
    for k2 in range(n2):
        Z = cfft_any(net, [cols[t1][k2] for t1 in range(n1)])
        for k1 in range(n1):
            for k in range(n):
                if k % n1 == k1 and k % n2 == k2:
                    out[k] = Z[k1]
    return out


def cfft5(net, z):
    c1, c2 = math.cos(2 * math.pi / 5), math.cos(4 * math.pi / 5)
    s1, s2 = math.sin(2 * math.pi / 5), math.sin(4 * math.pi / 5)
    t1 = net.cadd(z[1], z[4]); t2 = net.cadd(z[2], z[3])
    t3 = net.csub(z[1], z[4]); t4 = net.csub(z[2], z[3])
    t5 = net.cadd(t1, t2)
    def rm(x, c):
        return (net.mul(x[0], c), net.mul(x[1], c))
    m1 = rm(t5, (c1 + c2) / 2 - 1.0)
    m2 = rm(net.csub(t1, t2), (c1 - c2) / 2)
    y0 = net.cadd(z[0], t5)
    a = net.cadd(y0, m1)
    a1 = net.cadd(a, m2); a2 = net.csub(a, m2)
    m3 = rm(net.cadd(t3, t4), s2)
    m4 = rm(t3, s1 - s2)
    m5 = rm(t4, s1 + s2)
    b1 = net.cadd(m3, m4)
    b2 = net.csub(m3, m5)
    def mi(x):
        return (x[1], net.neg(x[0]))
    return [y0, net.cadd(a1, mi(b1)), net.cadd(a2, mi(b2)), net.csub(a2, mi(b2)), net.csub(a1, mi(b1))]


def rfft5(net, x):
    c1, c2 = math.cos(2 * math.pi / 5), math.cos(4 * math.pi / 5)
    s1, s2 = math.sin(2 * math.pi / 5), math.sin(4 * math.pi / 5)
    t1 = net.add(x[1], x[4]); t2 = net.add(x[2], x[3])
    t3 = net.sub(x[1], x[4]); t4 = net.sub(x[2], x[3])
    t5 = net.add(t1, t2)
    m1 = net.mul(t5, (c1 + c2) / 2 - 1.0)
    m2 = net.mul(net.sub(t1, t2), (c1 - c2) / 2)
    y0 = net.add(x[0], t5)
    a = net.add(y0, m1)
    a1 = net.add(a, m2); a2 = net.sub(a, m2)
    m3 = net.mul(net.add(t3, t4), s2)
    m4 = net.mul(t3, s1 - s2)
    m5 = net.mul(t4, s1 + s2)
    b1 = net.add(m3, m4); b2 = net.sub(m3, m5)
    return [(y0, None), (a1, net.neg(b1)), (a2, net.neg(b2))]


def cfft_any(net, z):
    n = len(z)
    if n == 5:
        return cfft5(net, z)
    if n == 12:
        return cfft_pfa(net, z, 3, 4)
    if n == 10:
        return cfft_pfa(net, z, 5, 2)
    if n == 20:
        return cfft_pfa(net, z, 5, 4)
    if n == 6:
        return cfft_pfa(net, z, 3, 2)
    if n == 14:
        return cfft_pfa(net, z, 7, 2)
    if n == 15:
        return cfft_pfa(net, z, 5, 3)
    return cfft(net, z)


def rfft_pfa(net, x, n1, n2):
    n = n1 * n2
    inner = [rfft(net, [x[(n2 * t1 + n1 * t2) % n] for t1 in range(n1)]) for t2 in range(n2)]
    out = [None] * (n // 2 + 1)
    for k1 in range(n1 // 2 + 1):
        col = [inner[t2][k1] for t2 in range(n2)]
        if all(c[1] is None for c in col):
            Z = rfft(net, [c[0] for c in col])
            Z = Z + [(Z[n2 - k2][0], net.neg(Z[n2 - k2][1])) for k2 in range(len(Z), n2)]
        else:
            Z = cfft_any(net, col)
        for k2 in range(n2):
            k = [k for k in range(n) if k % n1 == k1 and k % n2 == k2][0]
            if k <= n // 2:
                if out[k] is None:
                    out[k] = Z[k2]
            else:
                if out[n - k] is None:
                    out[n - k] = (Z[k2][0], net.neg(Z[k2][1]))
    return out


PFA = {40: (8, 5), 20: (4, 5), 24: (8, 3), 48: (16, 3), 12: (4, 3), 56: (8, 7), 10: (2, 5), 6: (2, 3), 60: (4, 15), 15: (3, 5), 44: (4, 11), 36: (4, 9)}
USE_PFA = True


def rfft(net, x):
    n = len(x)
    if USE_PFA and n in PFA:
        return rfft_pfa(net, x, *PFA[n])
    if n == 1:
        return [(x[0], None)]
    if n == 2:
        return [(net.add(x[0], x[1]), None), (net.sub(x[0], x[1]), None)]
    if n % 4 == 0:
        h, q = n // 2, n // 4
        e = [net.add(x[t], x[t + h]) for t in range(h)]
        o = [net.sub(x[t], x[t + h]) for t in range(h)]
        z = [net.cmulc((o[t], net.neg(o[t + q])), *w(t, n)) for t in range(q)]
        E = rfft(net, e)
        Z = cfft_any(net, z)
        out = [None] * (h + 1)
        for k in range(len(E)):
            out[2 * k] = E[k]
        for k in range(q):
            f = 4 * k + 1
            if f <= h:
                out[f] = Z[k]
            else:
                out[n - f] = (Z[k][0], net.neg(Z[k][1]))
        return out
    if n % 2 == 0:
        m = n // 2
        e = [net.add(x[t], x[t + m]) for t in range(m)]
        o = [net.sub(x[t], x[t + m]) for t in range(m)]
        E = rfft(net, e)
        op = [o[t] if t % 2 == 0 else net.neg(o[t]) for t in range(m)]
        O = rfft(net, op)
        out = [None] * (m + 1)
        for k in range(len(E)):
            out[2 * k] = E[k]
        for f in range(1, m + 1, 2):
            j = ((f - m) // 2) % m
            if j <= m // 2:
                out[f] = O[j]
            else:
                out[f] = (O[m - j][0], net.neg(O[m - j][1]))
        return out
    if n == 5:
        return rfft5(net, x)
    p = {t: net.add(x[t], x[n - t]) for t in range(1, (n + 1) // 2)}
    q = {t: net.sub(x[t], x[n - t]) for t in range(1, (n + 1) // 2)}
    s = x[0]
    for t in p:
        s = net.add(s, p[t])
    out = [(s, None)]
    for k in range(1, (n + 1) // 2):
        A = x[0]
        B = None
        for t in p:
            c, sn = w(k * t, n)
            A = net.add(A, net.mul(p[t], c))
            B = net.add(B, net.mul(q[t], sn))
        out.append((A, B))
    return out


class Prog:
    def __init__(self, net, outputs):
        order = []
        seen = set()

        def visit(n):
            if n in seen:
                return
            seen.add(n)
            k = net.nodes[n]
            if k[0] in ('add', 'sub'):
                visit(k[1]); visit(k[2])
            elif k[0] == 'mul':
                visit(k[1])
            order.append(n)
        for o in outputs:
            if o is not None:
                visit(o[0])
        self.net = net
        self.order = order
        self.outputs = outputs

    def count(self):
        c = {'add': 0, 'sub': 0, 'mul': 0, 'in': 0}
        for n in self.order:
            c[self.net.nodes[n][0]] += 1
        return c

    def run(self, load, emit=None):
        vals = {}
        for n in self.order:
            k = self.net.nodes[n]
            if k[0] == 'in':
                vals[n] = load(k[1])
            elif k[0] == 'add':
                vals[n] = vals[k[1]] + vals[k[2]]
            elif k[0] == 'sub':
                vals[n] = vals[k[1]] - vals[k[2]]
            else:
                vals[n] = vals[k[1]] * k[2]
        return [None if o is None else vals[o[0]] for o in self.outputs]

    @property
    def signs(self):
        return [0 if o is None else o[1] for o in self.outputs]

    def matrix(self, n_in, signed=True):
        eye = np.eye(n_in)
        res = self.run(lambda i: eye[i])
        rows = []
        for r, s in zip(res, self.signs):
            rows.append(np.zeros(n_in) if r is None else (r * s if signed else r))
        return np.stack(rows)


def transpose(net, outputs, wanted_inputs):
    prog = Prog(net, outputs)
    live = set(prog.order)
    consumers = {n: [] for n in prog.order}
    for n in prog.order:
        k = net.nodes[n]
        if k[0] == 'add':
            consumers[k[1]].append((n, 1.0)); consumers[k[2]].append((n, 1.0))
        elif k[0] == 'sub':
            consumers[k[1]].append((n, 1.0)); consumers[k[2]].append((n, -1.0))
        elif k[0] == 'mul':
            consumers[k[1]].append((n, k[2]))
    outmap = {}
    for r, o in enumerate(outputs):
        if o is not None:
            outmap.setdefault(o[0], []).append((r, o[1]))
    tn = Net()
    memo = {}

    def adj(n):
        if n in memo:
            return memo[n]
        acc = None
        for r, s in outmap.get(n, []):
            v = tn.inp(r)
            acc = tn.add(acc, v if s > 0 else tn.neg(v))
        for c, coef in consumers[n]:
            acc = tn.add(acc, tn.mul(adj(c), coef))
        memo[n] = acc
        return acc
    outs = []
    for i in wanted_inputs:
        key = ('in', i)
        if key in net.cse and net.cse[key] in live:
            outs.append(adj(net.cse[key]))
        else:
            outs.append(None)
    return tn, outs


def build(N, taps, scale=True, variant=0):
    hop = N - taps + 1
    na = Net()
    U = rfft(na, [na.inp(t) for t in range(N)])
    a_out = [U[0][0], U[N // 2][0]]
    bins = list(range(1, N // 2))
    for k in bins:
        a, b = U[k]
        if variant == 0:
            a_out += [na.add(a, b), a, b]
        else:
            a_out += [a, na.sub(b, a), na.add(a, b)]
    nc = Net()
    V = rfft(nc, [nc.inp(t) for t in range(N)])
    c_out = [V[0][0], V[N // 2][0]]
    for k in bins:
        al, be = V[k]
        c_out += [nc.add(al, be), be, nc.neg(al)]
    tn, c_res = transpose(nc, c_out, list(range(hop)))
    def mkb(ntaps):
        nb = Net()
        Wf = rfft(nb, [nb.inp(t) if t < ntaps else None for t in range(N)])
        s0 = 1.0 / N if scale else 0.5
        b_out = [nb.mul(Wf[0][0], s0), nb.mul(Wf[N // 2][0], s0)]
        for k in bins:
            c = Wf[k][0]
            d = nb.neg(Wf[k][1])
            sc = 2.0 / N if scale else 1.0
            if variant == 0:
                b_out += [nb.mul(c, sc), nb.mul(nb.sub(d, c), sc), nb.mul(nb.add(c, d), sc)]
            else:
                b_out += [nb.mul(nb.add(c, d), sc), nb.mul(c, sc), nb.mul(d, sc)]
        return nb, b_out
    nb, b_out = mkb(taps)
    nb1, b1_out = mkb(taps - 1)
    return dict(N=N, hop=hop, taps=taps, na=na, a_out=a_out, nb=nb, b_out=b_out, nb1=nb1, b1_out=b1_out,
                tn=tn, c_res=c_res, bins=bins)


def max_live(net, order, outputs, out_at_once=True):
    uses = {n: 0 for n in order}
    for n in order:
        k = net.nodes[n]
        for a in ([k[1], k[2]] if k[0] in ('add', 'sub') else [k[1]] if k[0] == 'mul' else []):
            uses[a] += 1
    live = set(); peak = 0; tot = 0
    rem = dict(uses)
    for n in order:
        k = net.nodes[n]
        live.add(n)
        peak = max(peak, len(live))
        for a in set([k[1], k[2]] if k[0] in ('add', 'sub') else [k[1]] if k[0] == 'mul' else []):
            rem[a] -= (1 if k[0] == 'mul' or k[1] != k[2] else 2)
            if rem[a] == 0:
                live.discard(a)
        if rem[n] == 0:
            live.discard(n)
        tot += len(live)
    return peak, tot / len(order)


def min_live_order(net, outputs, seed=0, tries=200):
    base = Prog(net, outputs).order
    nodes = set(base)
    def operands(n):
        k = net.nodes[n]
        return [k[1], k[2]] if k[0] in ('add', 'sub') else [k[1]] if k[0] == 'mul' else []
    consumers = {n: [] for n in base}
    for n in base:
        for a in set(operands(n)):
            consumers[a].append(n)
    best = (max_live(net, base, outputs), base)
    rnd = random.Random(seed)
    pos = {n: i for i, n in enumerate(base)}
    for it in range(tries):
        done = set(); order = []
        live = set()
        remc = {n: len(consumers[n]) for n in base}
        isin = {n: net.nodes[n][0] == 'in' for n in base}
        def ready(n):
            return n not in done and not isin[n] and all((a in done) or isin[a] for a in operands(n))
        noise = rnd.random() * 1.5
        work = [n for n in base if not isin[n]]
        left = set(work)
        while left:
            cands = [n for n in left if ready(n)]
            def score(n):
                ops = set(operands(n))
                newloads = sum(1 for a in ops if a not in done)
                kills = sum(1 for a in ops if remc[a] == 1)
                born = 0 if remc[n] == 0 else 1
                return (newloads + born - kills) + noise * rnd.random() + 1e-4 * pos[n]
            n = min(cands, key=score)
            for a in sorted(set(operands(n)), key=lambda a: pos[a]):
                if a not in done:
                    done.add(a); order.append(a)
                remc[a] -= 1
            done.add(n); order.append(n); left.discard(n)
        ml = max_live(net, order, outputs)
        if ml < best[0]:
            best = (ml, order)
    return best


def solve_signs(G, iters=200000, seed=0):
    rnd = random.Random(seed)
    nets = {'A': (G['na'], G['a_out']), 'B': (G['nb'], G['b_out']), 'C': (G['tn'], G['c_res'])}
    order = {k: Prog(*v).order for k, v in nets.items()}
    R = len(G['a_out'])
    sig = {}
    for k in 'ABC':
        for n in order[k]:
            sig[(k, n)] = 1
    fixed = set()
    for k in 'AB':
        for n in order[k]:
            if nets[k][0].nodes[n][0] == 'in':
                fixed.add((k, n))
    for o in G['c_res']:
        sig[('C', o[0])] = o[1]; fixed.add(('C', o[0]))
    cin = {}
    for n in order['C']:
        nd = G['tn'].nodes[n]
        if nd[0] == 'in':
            cin[nd[1]] = n; fixed.add(('C', n))
    def cin_sign(r):
        a, b = G['a_out'][r], G['b_out'][r]
        return (sig[('A', a[0])] * a[1]) * (sig[('B', b[0])] * b[1])
    outmap = {}
    for r in range(R):
        outmap.setdefault(('A', G['a_out'][r][0]), []).append(r)
        outmap.setdefault(('B', G['b_out'][r][0]), []).append(r)
    def refresh():
        for r, n in cin.items():
            sig[('C', n)] = cin_sign(r)
    clauses = []
    for k in 'ABC':
        net = nets[k][0]
        for n in order[k]:
            nd = net.nodes[n]
            if nd[0] in ('add', 'sub'):
                clauses.append((k, n, nd[1], nd[2], 1 if nd[0] == 'add' else -1))
    occ = {}
    for ci, (k, n, a, b, cb) in enumerate(clauses):
        for v in (n, a, b):
            occ.setdefault((k, v), []).append(ci)
    def viol(ci):
        k, n, a, b, cb = clauses[ci]
        return sig[(k, n)] * sig[(k, a)] < 0 and sig[(k, n)] * cb * sig[(k, b)] < 0
    def flip(v):
        sig[v] = -sig[v]
        for r in outmap.get(v, []):
            if r in cin:
                sig[('C', cin[r])] = cin_sign(r)
    def affected(v):
        cs = set(occ.get(v, []))
        for r in outmap.get(v, []):
            if r in cin:
                cs.update(occ.get(('C', cin[r]), []))
        return cs
    flippers = {}
    for v, rs in outmap.items():
        for r in rs:
            if r in cin:
                flippers.setdefault(('C', cin[r]), []).append(v)
    refresh()
    bad = {ci for ci in range(len(clauses)) if viol(ci)}
    best = (len(bad), dict(sig))
    for it in range(iters):
        if not bad:
            break
        ci = rnd.choice(list(bad))
        k, n, a, b, cb = clauses[ci]
        cands = []
        for v in ((k, n), (k, a), (k, b)):
            if v in fixed:
                cands += flippers.get(v, [])
            else:
                cands.append(v)
        cands = [v for v in cands if v not in fixed]
        if not cands:
            continue
        def delta(v):
            cs = affected(v)
            before = sum(viol(c) for c in cs)
            flip(v)
            after = sum(viol(c) for c in cs)
            flip(v)
            return after - before
        if rnd.random() < 0.2:
            v = rnd.choice(cands)
        else:
            v = min(cands, key=lambda v: (delta(v), rnd.random()))
        cs = affected(v)
        flip(v)
        for c in cs:
            if viol(c): bad.add(c)
            else: bad.discard(c)
        if len(bad) < best[0]:
            best = (len(bad), dict(sig))
    nb, sg = best
    return ({n: s for (k, n), s in sg.items() if k == 'A'}, {n: s for (k, n), s in sg.items() if k == 'B'},
            {n: s for (k, n), s in sg.items() if k == 'C'}, nb)


class FixedProg:
    def __init__(self, net, outputs, sig, order=None):
        self.net, self.outputs, self.sig = net, outputs, sig
        self.order = order if order is not None else Prog(net, outputs).order
    def count(self):
        c = {'add': 0, 'sub': 0, 'mul': 0, 'in': 0}
        for n in self.order:
            c[self.net.nodes[n][0]] += 1
        return c


N, TAPS = 40, 16
G = build(N, TAPS, scale=False, variant=1)
HOP = G['hop']; R = len(G['a_out'])
T, D, K = 16000, 512, 31
L = (T - K) // 2 + 1
MB = 64; NCH = -(-L // (HOP * MB))
CH = HOP * MB
XM = CH + 16
LP = NCH * CH
TM = T // 2
LAST_M = TM - (NCH - 1) * CH
HS = 2.0 / N
T2 = 1; W3 = 1
U32, F32, BF16 = jnp.uint32, jnp.float32, jnp.bfloat16

bins = G['bins']
ev = [0, 1] + [2 + 3 * i + q for i, k in enumerate(bins) if k % 2 == 0 for q in range(3)]
od = [2 + 3 * i + q for i, k in enumerate(bins) if k % 2 == 1 for q in range(3)]
if (N // 2) % 2 == 1:
    ev.remove(1); od = [1] + od
IDX = (ev, od)
RH = (len(ev), len(od))
LOC = {}
for hf in range(2):
    for i, r in enumerate(IDX[hf]):
        LOC[r] = (hf, i)
SA, SB, SC, NBAD = solve_signs(G)
assert NBAD == 0
def mkprog(net, outs, sig):
    return FixedProg(net, outs, sig, order=min_live_order(net, outs, tries=100)[1])
PA = [mkprog(G['na'], [G['a_out'][r] for r in idx], SA) for idx in IDX]
PB = [mkprog(G['nb'], [G['b_out'][r] for r in idx], SB) for idx in IDX]
PC = mkprog(G['tn'], G['c_res'], SC)


def run_gen(prog, loads, sink):
    nsets = len(loads)
    vals = [dict() for _ in range(nsets)]
    sig = prog.sig
    outs = {}
    for r, o in enumerate(prog.outputs):
        outs.setdefault(o[0], []).append(r)
    for n in prog.order:
        k = prog.net.nodes[n]
        for s in range(nsets):
            v = vals[s]
            if k[0] == 'in':
                v[n] = loads[s](k[1])
            elif k[0] == 'mul':
                v[n] = v[k[1]] * (k[2] * sig[n] * sig[k[1]])
            else:
                a, b = k[1], k[2]
                cb = 1 if k[0] == 'add' else -1
                p, q = sig[n] * sig[a], sig[n] * cb * sig[b]
                if p > 0 and q > 0: v[n] = v[a] + v[b]
                elif p > 0: v[n] = v[a] - v[b]
                elif q > 0: v[n] = v[b] - v[a]
                else: v[n] = -(v[a] + v[b])
            yield 1
        for r in outs.get(n, []):
            yield from sink(r, [vals[s][n] for s in range(nsets)])


def drain(gen):
    for _ in gen:
        pass


def unpack(wd, hi):
    wd = (wd & jnp.uint32(0xffff0000)) if hi else (wd << 16)
    return lax.bitcast_convert_type(wd, F32)


def pack(lo, hi):
    return pltpu.pack_elementwise([lo, hi], packed_dtype=BF16)


def prog_weight(prog, nsets, per_out):
    return len(prog.order) * nsets + len(prog.outputs) * per_out


def interleave(mms, gens_weights):
    total = sum(w for _, w in gens_weights)
    def allops():
        for g, _ in gens_weights:
            yield from g
    gen = allops()
    e = 0; done = False
    for i, mm in enumerate(mms):
        mm()
        tgt = (i + 1) * total // len(mms)
        while not done and e < tgt:
            try:
                e += next(gen)
            except StopIteration:
                done = True
    for _ in gen:
        pass


def merge(lists):
    lists = [l for l in lists if l]
    out = []
    pos = [0] * len(lists)
    tot = sum(len(l) for l in lists)
    for _ in range(tot):
        i = min((i for i in range(len(lists)) if pos[i] < len(lists[i])), key=lambda i: (pos[i] + 0.5) / len(lists[i]))
        out.append(lists[i][pos[i]]); pos[i] += 1
    return out


C0 = math.sqrt(2.0 / math.pi)
def gelu_half(zh):
    u = zh * (zh * zh * (8.0 * C0 * 0.044715) + 2.0 * C0)
    return zh * jnp.tanh(u) + zh


def kernel(x_hbm, w_hbm, gam_ref, bet_ref, out_hbm,
           xb0, xb1, xb2, xb3, we, wo, xe, xo, ye, yo, h0, h1, h2, h3, st, nrm, gsm, xsem, wsem, osem):
    xb = (xb0, xb1, xb2, xb3)
    wh = (we, wo); xh = (xe, xo); yy = (ye, yo)
    hh = (h0, h1, h2, h3)
    x32 = x_hbm.bitcast(U32)
    w32 = w_hbm.bitcast(F32)
    o32 = out_hbm.bitcast(F32)
    LASTJ = 2 * NCH - 1

    def x_copy(j, c, full):
        b = j // NCH
        cj = j % NCH
        rows = XM if full else LAST_M
        return pltpu.make_async_copy(
            x32.at[b, pl.ds(pl.multiple_of(cj * CH, 8), rows), pl.ds(c * 128, 128)],
            xb[c].at[pl.ds(0, rows), :], xsem.at[c])

    def x_start(j):
        cj = j % NCH
        @pl.when(cj < NCH - 1)
        def _():
            for c in range(4):
                x_copy(j, c, True).start()
        @pl.when(cj == NCH - 1)
        def _():
            for c in range(4):
                x_copy(j, c, False).start()
                xb[c][pl.ds(LAST_M, XM - LAST_M), :] = jnp.zeros((XM - LAST_M, 128), U32)

    def x_wait(j, cs=range(4)):
        cj = j % NCH
        @pl.when(cj < NCH - 1)
        def _():
            for c in cs:
                x_copy(j, c, True).wait()
        @pl.when(cj == NCH - 1)
        def _():
            for c in cs:
                x_copy(j, c, False).wait()

    WQ = 4
    def w_copy(n, q):
        dst = hh[n].at[1, pl.ds(0, K * 256), :].reshape(K, 256, 128)
        r = 256 // WQ
        return pltpu.make_async_copy(w32.at[:, pl.ds(q * r, r), pl.ds(n * 128, 128)], dst.at[:, pl.ds(q * r, r), :], wsem.at[n, q])

    def o_copy(n, r0, rows, k):
        return pltpu.make_async_copy(hh[n].at[0, pl.ds(r0, rows), :], o32.at[pl.ds(r0, rows), n, 0, :], osem.at[n, k])

    def a_piece(g, c, p, half):
        dyn = not isinstance(g, int)
        base = pl.multiple_of(g * (16 * HOP), 8) if dyn else g * (16 * HOP)
        row = pl.multiple_of(g * 8, 8) if dyn else g * 8
        xw = xb[c].at[pl.ds(base, 16 * HOP + 16), :]
        def mkload(o):
            return lambda t: unpack(xw[pl.ds(t + o * HOP, 8, stride=2 * HOP), :], p)
        def sink(i, vs):
            xh[half][i, pl.ds(row, 8), p * 512 + c * 128:p * 512 + (c + 1) * 128] = pack(vs[0], vs[1])
            yield 1
        return run_gen(PA[half], [mkload(0), mkload(1)], sink), prog_weight(PA[half], 2, 1)

    def a_pieces(half):
        return [a_piece(g, c, p, half) for c in range(4) for g in range(MB // 16) for p in range(2)]

    def w_piece(n, g, p, half):
        dyn = not isinstance(g, int)
        row = pl.multiple_of(g * 8, 8) if dyn else g * 8
        cache = {}
        def word(j):
            if j not in cache:
                cache[j] = lax.bitcast_convert_type(hh[n][1, pl.ds((2 * j + p) * 256 + row, 8), :], U32)
            return cache[j]
        def mkload(hi):
            def load(j):
                if 2 * j + p >= K:
                    return jnp.zeros((8, 128), F32)
                return unpack(word(j), hi)
            return load
        def sink(i, vs):
            wh[half][n, i, pl.ds(p * 256 + row, 8), :] = pack(vs[0], vs[1])
            yield 1
        return run_gen(PB[half], [mkload(0), mkload(1)], sink), prog_weight(PB[half], 2, 1)

    def c_pieces(j, n):
        if isinstance(j, int):
            b, cj = j // NCH, j % NCH
            slot = b
        else:
            valid = j >= 0
            b = jnp.where(valid, j // NCH, 0)
            cj = jnp.where(valid, j % NCH, NCH - 1)
            slot = jnp.where(valid, b, 2)
        state = {}
        def col(g):
            if g == 0:
                state['c'] = st[slot, n, 2]; state['a1'] = st[slot, n, 0]; state['a2'] = st[slot, n, 1]
            base = cj * CH + g * (8 * HOP)
            if not isinstance(j, int):
                base = pl.multiple_of(base, 8)
            hs = hh[n].at[b, pl.ds(base, 8 * HOP), :]
            def sink(t, vs):
                hs[pl.ds(t, 8, stride=HOP), :] = vs[0]
                d = vs[0] - state['c']
                state['a1'] = state['a1'] + d
                state['a2'] = state['a2'] + d * d
                yield 4
            yield from run_gen(PC, [lambda r: yy[LOC[r][0]][n, LOC[r][1], g * 8:(g + 1) * 8, :]], sink)
            if g == MB // 8 - 1:
                st[slot, n, 0] = state['a1']; st[slot, n, 1] = state['a2']
        return [(col(g), prog_weight(PC, 1, 4)) for g in range(MB // 8)]

    def set_shift(j, n):
        @pl.when(jnp.logical_and(j >= 0, j % NCH == 0))
        def _():
            st[j // NCH, n, 2] = jnp.broadcast_to(ye[n, LOC[0][1], 0:1, :], (8, 128))

    def finalize_stats(n):
        sub = lax.broadcasted_iota(jnp.int32, (8, 128), 0)
        for b in range(2):
            c = st[b, n, 2]
            r0 = (L // 8) * 8
            c1 = jnp.zeros((8, 128), F32); c2 = jnp.zeros((8, 128), F32)
            for r in range(r0, LP, 8):
                d = hh[n][b, r:r + 8, :] - c
                if r < L:
                    d = jnp.where(sub >= L - r, d, 0.0)
                c1 = c1 + d; c2 = c2 + d * d
            s1 = jnp.sum(st[b, n, 0] - c1, axis=0, keepdims=True)
            s2 = jnp.sum(st[b, n, 1] - c2, axis=0, keepdims=True)
            md = s1 * (1.0 / L)
            var = (s2 * (1.0 / L) - md * md) * (HS * HS)
            mu = c[0:1] + md
            a = (HS * lax.rsqrt(var + 1e-5)) * gam_ref[...].astype(F32).reshape(1, D)[:, n * 128:(n + 1) * 128]
            bb = bet_ref[...].astype(F32).reshape(1, D)[:, n * 128:(n + 1) * 128] - mu * a
            nrm[n, b, 0] = jnp.broadcast_to(0.5 * a, (8, 128))
            nrm[n, b, 1] = jnp.broadcast_to(0.5 * bb, (8, 128))

    def d_vreg(n, r, cs):
        a0, b0, a1, b1 = cs
        z0 = gelu_half(hh[n][0, pl.ds(r, 8), :] * a0 + b0)
        z1 = gelu_half(hh[n][1, pl.ds(r, 8), :] * a1 + b1)
        hh[n][0, pl.ds(r, 8), :] = lax.bitcast_convert_type(pack(z0, z1), F32)

    def d_consts(n):
        return nrm[n, 0, 0], nrm[n, 0, 1], nrm[n, 1, 0], nrm[n, 1, 1]

    def d_pieces(n, ra=0, rb=LP):
        state = {}
        def piece(r0, r1):
            if 'cs' not in state:
                state['cs'] = d_consts(n)
            for r in range(r0, r1, 8):
                d_vreg(n, r, state['cs'])
                yield 19
        P = 200
        return [(piece(r, min(r + P, rb)), 19 * (min(r + P, rb) - r) // 8) for r in range(ra, rb, P)]

    def fin_piece(n):
        def gen():
            finalize_stats(n)
            yield 100
        return [(gen(), 100)]

    NPC = 4
    PR = -(-(-(-L // NPC)) // 8) * 8
    def d_loop(n):
        cs = d_consts(n)
        UN = 5
        for k in range(NPC):
            r0 = k * PR; r1 = min(r0 + PR, LP)
            nv = -(-(r1 - r0) // 8)
            assert nv % UN == 0, nv
            def body(i, carry):
                for u in range(UN):
                    d_vreg(n, pl.multiple_of(r0 + (i * UN + u) * 8, 8), cs)
                return carry
            lax.fori_loop(0, nv // UN, body, 0)
            o_copy(n, r0, min(r0 + PR, L) - r0, k).start()

    def o_start_all(n):
        for k in range(NPC):
            r0 = k * PR
            o_copy(n, r0, min(r0 + PR, L) - r0, k).start()

    def o_wait_all(n):
        for k in range(NPC):
            r0 = k * PR
            o_copy(n, r0, min(r0 + PR, L) - r0, k).wait()

    def mm(half, n, i):
        def f():
            lhs = pltpu.bitcast(xh[half][i], BF16)
            rhs = pltpu.bitcast(wh[half][n, i], BF16)
            yy[half][n, i] = jnp.dot(lhs, rhs, preferred_element_type=F32)
        return f

    def body(name, half, tiles, lists, sl=None):
        mms = [mm(half, n, i) for n in tiles for i in range(RH[half])]
        if sl is not None:
            mms = mms[sl]
        with jax.named_scope(name):
            interleave(mms, merge(lists))

    j0 = jnp.int32(0)
    gsm[0] = jnp.int32(0)
    x_start(j0)
    for q in range(WQ):
        w_copy(0, q).start()
    st[...] = jnp.zeros_like(st)

    with jax.named_scope("a0"):
        for c in range(4):
            x_wait(j0, [c])
            def a0(g, carry):
                for p in range(2):
                    drain(a_piece(g, c, p, 0)[0])
                return carry
            lax.fori_loop(0, MB // 16, a0, 0)
        for n in range(1, 4):
            for q in range(WQ):
                w_copy(n, q).start()

    with jax.named_scope("wstage"):
        GP = 32 // WQ
        for n in range(4):
            phases = (1,) if (n == 3 and W3) else (0, 1)
            def wl(g, carry):
                for p in phases:
                    for half in range(2):
                        drain(w_piece(n, g, p, half)[0])
                return carry
            def wq(q, carry):
                w_copy(n, q).wait()
                lax.fori_loop(q * GP, (q + 1) * GP, wl, 0)
                return carry
            lax.fori_loop(0, WQ, wq, 0)

    def main(j, carry):
        @pl.when(j >= 0)
        def _():
            body("E01", 0, (0, 1), [a_pieces(1)])
        @pl.when(j + 1 <= LASTJ)
        def _():
            x_start(j + 1)
        set_shift(j - 1, 2); set_shift(j - 1, 3)
        if W3:
            @pl.when(j == 0)
            def _():
                body("O01W", 1, (0, 1), [[w_piece(3, g, 0, half) for g in range(32) for half in range(2)]])
        @pl.when(j + 1 >= (2 if W3 else 1))
        def _():
            body("O01", 1, (0, 1), [c_pieces(j - 1, 2), c_pieces(j - 1, 3)])
        @pl.when(j < (LASTJ if T2 else LASTJ + 1))
        def _():
            set_shift(j, 0); set_shift(j, 1)
        @pl.when(j + 2 < (LASTJ if T2 else LASTJ + 1) + 2)
        def _():
            body("E23", 0, (2, 3), [c_pieces(j, 0), c_pieces(j, 1)])
        @pl.when(j + 1 <= LASTJ)
        def _():
            x_wait(j + 1)
        @pl.when(j < (LASTJ if T2 else LASTJ + 1))
        def _():
            body("O23", 1, (2, 3), [a_pieces(0)])
        return carry
    lax.fori_loop(0, LASTJ + 1, main, 0)

    jl = jnp.int32(LASTJ)
    if T2:
        gd = gsm[0]
        set_shift(jl, 0); set_shift(jl, 1)
        HR = 2 * PR
        def o_start(n, ks):
            for k in ks:
                r0 = k * PR
                o_copy(n, r0, min(r0 + PR, L) - r0, k).start()
        @pl.when(gd >= 0)
        def _():
            body("E2D", 0, (2,), [c_pieces(LASTJ, 0) + fin_piece(0) + d_pieces(0, 0, HR)])
        o_start(0, (0, 1))
        @pl.when(gd + 1 >= 1)
        def _():
            body("E3D", 0, (3,), [d_pieces(0, HR, LP) + c_pieces(LASTJ, 1) + fin_piece(1)])
        o_start(0, (2, 3))
        @pl.when(gd + 2 >= 2)
        def _():
            body("O2D", 1, (2,), [d_pieces(1, 0, HR)])
        o_start(1, (0, 1))
        @pl.when(gd + 3 >= 3)
        def _():
            body("O3D", 1, (3,), [d_pieces(1, HR, LP)])
        o_start(1, (2, 3))

    with jax.named_scope("tail"):
        set_shift(jl, 2); set_shift(jl, 3)
        for n in (2, 3):
            for g_, _ in c_pieces(jl, n):
                drain(g_)
        for n in range(2 if T2 else 0, 4):
            finalize_stats(n)
            d_loop(n)
        for n in range(4):
            o_wait_all(n)


@jax.jit
def pallas_standalone__self_sup_conv_stem_wavlm__speech_kernel(x, w, gn_gamma, gn_beta):
    out = pl.pallas_call(
        kernel,
        in_specs=[pl.BlockSpec(memory_space=pl.ANY), pl.BlockSpec(memory_space=pl.ANY),
                  pl.BlockSpec(memory_space=pltpu.VMEM), pl.BlockSpec(memory_space=pltpu.VMEM)],
        out_specs=pl.BlockSpec(memory_space=pl.ANY),
        out_shape=jax.ShapeDtypeStruct((L, 4, 2, 128), BF16),
        scratch_shapes=[pltpu.VMEM((XM, 128), U32)] * 4 + [
            pltpu.VMEM((4, RH[0], 512, 128), U32),
            pltpu.VMEM((4, RH[1], 512, 128), U32),
            pltpu.VMEM((RH[0], MB // 2, 1024), U32),
            pltpu.VMEM((RH[1], MB // 2, 1024), U32),
            pltpu.VMEM((4, RH[0], MB, 128), F32),
            pltpu.VMEM((4, RH[1], MB, 128), F32)] + [pltpu.VMEM((2, LP, 128), F32)] * 4 + [
            pltpu.VMEM((3, 4, 3, 8, 128), F32),
            pltpu.VMEM((4, 2, 2, 8, 128), F32),
            pltpu.SMEM((1,), jnp.int32),
            pltpu.SemaphoreType.DMA((4,)),
            pltpu.SemaphoreType.DMA((4, 4)),
            pltpu.SemaphoreType.DMA((4, 4)),
        ],
        compiler_params=pltpu.CompilerParams(vmem_limit_bytes=127 * 1024 * 1024),
    )(x, w, gn_gamma, gn_beta)
    return out.transpose(2, 0, 1, 3).reshape(2, L, D)
```

```python
import math
import random
import numpy as np
import jax, jax.numpy as jnp
from jax import lax
from jax.experimental import pallas as pl
from jax.experimental.pallas import tpu as pltpu


class Net:
    def __init__(self):
        self.nodes = []
        self.cse = {}

    def _mk(self, key):
        if key in self.cse:
            return self.cse[key]
        self.nodes.append(key)
        self.cse[key] = len(self.nodes) - 1
        return self.cse[key]

    def inp(self, i):
        return (self._mk(('in', i)), 1)

    def neg(self, x):
        return None if x is None else (x[0], -x[1])

    def add(self, x, y):
        if x is None:
            return y
        if y is None:
            return x
        (a, sa), (b, sb) = x, y
        if a == b:
            if sa == sb:
                return self.mul(x, 2.0)
            return None
        if sa == sb:
            if a > b:
                a, b = b, a
            return (self._mk(('add', a, b)), sa)
        if a > b:
            a, b, sa = b, a, sb
        return (self._mk(('sub', a, b)), sa)

    def sub(self, x, y):
        return self.add(x, self.neg(y))

    def mul(self, x, c):
        if x is None or abs(c) < 1e-12:
            return None
        a, s = x
        if c < 0:
            c, s = -c, -s
        if abs(c - 1.0) < 1e-12:
            return (a, s)
        c = float(np.float64(round(c, 14)))
        return (self._mk(('mul', a, c)), s)

    def cadd(self, x, y):
        return (self.add(x[0], y[0]), self.add(x[1], y[1]))

    def csub(self, x, y):
        return (self.sub(x[0], y[0]), self.sub(x[1], y[1]))

    def cmulc(self, x, c, s):
        a, b = x
        if abs(s) < 1e-12:
            return (self.mul(a, c), self.mul(b, c))
        if abs(c) < 1e-12:
            return (self.mul(b, -s), self.mul(a, s))
        if abs(abs(c) - abs(s)) < 1e-12:
            sg = 1.0 if s * c > 0 else -1.0
            re = self.sub(a, self.mul(b, sg))
            im = self.add(b, self.mul(a, sg))
            return (self.mul(re, c), self.mul(im, c))
        re = self.sub(self.mul(a, c), self.mul(b, s))
        im = self.add(self.mul(a, s), self.mul(b, c))
        return (re, im)


def w(k, n):
    ang = -2.0 * math.pi * (k % n) / n
    return math.cos(ang), math.sin(ang)


def cfft(net, z):
    n = len(z)
    if n == 1:
        return [z[0]]
    if n == 2:
        return [net.cadd(z[0], z[1]), net.csub(z[0], z[1])]
    if n % 4 == 0:
        h, q = n // 2, n // 4
        e = [net.cadd(z[t], z[t + h]) for t in range(h)]
        o = [net.csub(z[t], z[t + h]) for t in range(h)]
        z1, z3 = [], []
        for t in range(q):
            a, b = o[t], o[t + q]
            mib = (b[1], net.neg(b[0]))
            p = net.cadd(a, mib)
            m = net.csub(a, mib)
            z1.append(net.cmulc(p, *w(t, n)))
            z3.append(net.cmulc(m, *w(3 * t, n)))
        E = cfft(net, e)
        Z1 = cfft(net, z1)
        Z3 = cfft(net, z3)
        out = [None] * n
        for k in range(h):
            out[2 * k] = E[k]
        for k in range(q):
            out[4 * k + 1] = Z1[k]
            out[4 * k + 3] = Z3[k]
        return out
    if n % 2 == 0:
        m = n // 2
        out = [None] * n
        rows = []
        for t2 in range(m):
            a = z[(2 * t2) % n]
            b = z[(m + 2 * t2) % n]
            rows.append((net.cadd(a, b), net.csub(a, b)))
        for k1 in range(2):
            Z = cfft(net, [rows[t2][k1] for t2 in range(m)])
            for k2 in range(m):
                for k in range(n):
                    if k % 2 == k1 and k % m == k2:
                        out[k] = Z[k2]
        return out
    if n % 3 == 0 and n > 3:
        raise NotImplementedError
    out = []
    p = {t: net.cadd(z[t], z[n - t]) for t in range(1, (n + 1) // 2)}
    q = {t: net.csub(z[t], z[n - t]) for t in range(1, (n + 1) // 2)}
    s = z[0]
    for t in p:
        s = net.cadd(s, p[t])
    out = [None] * n
    out[0] = s
    for k in range(1, (n + 1) // 2):
        A = z[0]
        B = (None, None)
        for t in p:
            c, sn = w(k * t, n)
            A = net.cadd(A, (net.mul(p[t][0], c), net.mul(p[t][1], c)))
            B = net.cadd(B, (net.mul(q[t][1], -sn), net.mul(q[t][0], sn)))
        out[k] = net.cadd(A, B)
        out[n - k] = net.csub(A, B)
    return out


def cfft_pfa(net, z, n1, n2):
    n = n1 * n2
    out = [None] * n
    cols = [cfft_any(net, [z[(n2 * t1 + n1 * t2) % n] for t2 in range(n2)]) for t1 in range(n1)]
    for k2 in range(n2):
        Z = cfft_any(net, [cols[t1][k2] for t1 in range(n1)])
        for k1 in range(n1):
            for k in range(n):
                if k % n1 == k1 and k % n2 == k2:
                    out[k] = Z[k1]
    return out


def cfft5(net, z):
    c1, c2 = math.cos(2 * math.pi / 5), math.cos(4 * math.pi / 5)
    s1, s2 = math.sin(2 * math.pi / 5), math.sin(4 * math.pi / 5)
    t1 = net.cadd(z[1], z[4]); t2 = net.cadd(z[2], z[3])
    t3 = net.csub(z[1], z[4]); t4 = net.csub(z[2], z[3])
    t5 = net.cadd(t1, t2)
    def rm(x, c):
        return (net.mul(x[0], c), net.mul(x[1], c))
    m1 = rm(t5, (c1 + c2) / 2 - 1.0)
    m2 = rm(net.csub(t1, t2), (c1 - c2) / 2)
    y0 = net.cadd(z[0], t5)
    a = net.cadd(y0, m1)
    a1 = net.cadd(a, m2); a2 = net.csub(a, m2)
    m3 = rm(net.cadd(t3, t4), s2)
    m4 = rm(t3, s1 - s2)
    m5 = rm(t4, s1 + s2)
    b1 = net.cadd(m3, m4)
    b2 = net.csub(m3, m5)
    def mi(x):
        return (x[1], net.neg(x[0]))
    return [y0, net.cadd(a1, mi(b1)), net.cadd(a2, mi(b2)), net.csub(a2, mi(b2)), net.csub(a1, mi(b1))]


def rfft5(net, x):
    c1, c2 = math.cos(2 * math.pi / 5), math.cos(4 * math.pi / 5)
    s1, s2 = math.sin(2 * math.pi / 5), math.sin(4 * math.pi / 5)
    t1 = net.add(x[1], x[4]); t2 = net.add(x[2], x[3])
    t3 = net.sub(x[1], x[4]); t4 = net.sub(x[2], x[3])
    t5 = net.add(t1, t2)
    m1 = net.mul(t5, (c1 + c2) / 2 - 1.0)
    m2 = net.mul(net.sub(t1, t2), (c1 - c2) / 2)
    y0 = net.add(x[0], t5)
    a = net.add(y0, m1)
    a1 = net.add(a, m2); a2 = net.sub(a, m2)
    m3 = net.mul(net.add(t3, t4), s2)
    m4 = net.mul(t3, s1 - s2)
    m5 = net.mul(t4, s1 + s2)
    b1 = net.add(m3, m4); b2 = net.sub(m3, m5)
    return [(y0, None), (a1, net.neg(b1)), (a2, net.neg(b2))]


def cfft_any(net, z):
    n = len(z)
    if n == 5:
        return cfft5(net, z)
    if n == 12:
        return cfft_pfa(net, z, 3, 4)
    if n == 10:
        return cfft_pfa(net, z, 5, 2)
    if n == 20:
        return cfft_pfa(net, z, 5, 4)
    if n == 6:
        return cfft_pfa(net, z, 3, 2)
    if n == 14:
        return cfft_pfa(net, z, 7, 2)
    if n == 15:
        return cfft_pfa(net, z, 5, 3)
    return cfft(net, z)


def rfft_pfa(net, x, n1, n2):
    n = n1 * n2
    inner = [rfft(net, [x[(n2 * t1 + n1 * t2) % n] for t1 in range(n1)]) for t2 in range(n2)]
    out = [None] * (n // 2 + 1)
    for k1 in range(n1 // 2 + 1):
        col = [inner[t2][k1] for t2 in range(n2)]
        if all(c[1] is None for c in col):
            Z = rfft(net, [c[0] for c in col])
            Z = Z + [(Z[n2 - k2][0], net.neg(Z[n2 - k2][1])) for k2 in range(len(Z), n2)]
        else:
            Z = cfft_any(net, col)
        for k2 in range(n2):
            k = [k for k in range(n) if k % n1 == k1 and k % n2 == k2][0]
            if k <= n // 2:
                if out[k] is None:
                    out[k] = Z[k2]
            else:
                if out[n - k] is None:
                    out[n - k] = (Z[k2][0], net.neg(Z[k2][1]))
    return out


PFA = {40: (8, 5), 20: (4, 5), 24: (8, 3), 48: (16, 3), 12: (4, 3), 56: (8, 7), 10: (2, 5), 6: (2, 3), 60: (4, 15), 15: (3, 5), 44: (4, 11), 36: (4, 9)}
USE_PFA = True


def rfft(net, x):
    n = len(x)
    if USE_PFA and n in PFA:
        return rfft_pfa(net, x, *PFA[n])
    if n == 1:
        return [(x[0], None)]
    if n == 2:
        return [(net.add(x[0], x[1]), None), (net.sub(x[0], x[1]), None)]
    if n % 4 == 0:
        h, q = n // 2, n // 4
        e = [net.add(x[t], x[t + h]) for t in range(h)]
        o = [net.sub(x[t], x[t + h]) for t in range(h)]
        z = [net.cmulc((o[t], net.neg(o[t + q])), *w(t, n)) for t in range(q)]
        E = rfft(net, e)
        Z = cfft_any(net, z)
        out = [None] * (h + 1)
        for k in range(len(E)):
            out[2 * k] = E[k]
        for k in range(q):
            f = 4 * k + 1
            if f <= h:
                out[f] = Z[k]
            else:
                out[n - f] = (Z[k][0], net.neg(Z[k][1]))
        return out
    if n % 2 == 0:
        m = n // 2
        e = [net.add(x[t], x[t + m]) for t in range(m)]
        o = [net.sub(x[t], x[t + m]) for t in range(m)]
        E = rfft(net, e)
        op = [o[t] if t % 2 == 0 else net.neg(o[t]) for t in range(m)]
        O = rfft(net, op)
        out = [None] * (m + 1)
        for k in range(len(E)):
            out[2 * k] = E[k]
        for f in range(1, m + 1, 2):
            j = ((f - m) // 2) % m
            if j <= m // 2:
                out[f] = O[j]
            else:
                out[f] = (O[m - j][0], net.neg(O[m - j][1]))
        return out
    if n == 5:
        return rfft5(net, x)
    p = {t: net.add(x[t], x[n - t]) for t in range(1, (n + 1) // 2)}
    q = {t: net.sub(x[t], x[n - t]) for t in range(1, (n + 1) // 2)}
    s = x[0]
    for t in p:
        s = net.add(s, p[t])
    out = [(s, None)]
    for k in range(1, (n + 1) // 2):
        A = x[0]
        B = None
        for t in p:
            c, sn = w(k * t, n)
            A = net.add(A, net.mul(p[t], c))
            B = net.add(B, net.mul(q[t], sn))
        out.append((A, B))
    return out


class Prog:
    def __init__(self, net, outputs):
        order = []
        seen = set()

        def visit(n):
            if n in seen:
                return
            seen.add(n)
            k = net.nodes[n]
            if k[0] in ('add', 'sub'):
                visit(k[1]); visit(k[2])
            elif k[0] == 'mul':
                visit(k[1])
            order.append(n)
        for o in outputs:
            if o is not None:
                visit(o[0])
        self.net = net
        self.order = order
        self.outputs = outputs

    def count(self):
        c = {'add': 0, 'sub': 0, 'mul': 0, 'in': 0}
        for n in self.order:
            c[self.net.nodes[n][0]] += 1
        return c

    def run(self, load, emit=None):
        vals = {}
        for n in self.order:
            k = self.net.nodes[n]
            if k[0] == 'in':
                vals[n] = load(k[1])
            elif k[0] == 'add':
                vals[n] = vals[k[1]] + vals[k[2]]
            elif k[0] == 'sub':
                vals[n] = vals[k[1]] - vals[k[2]]
            else:
                vals[n] = vals[k[1]] * k[2]
        return [None if o is None else vals[o[0]] for o in self.outputs]

    @property
    def signs(self):
        return [0 if o is None else o[1] for o in self.outputs]

    def matrix(self, n_in, signed=True):
        eye = np.eye(n_in)
        res = self.run(lambda i: eye[i])
        rows = []
        for r, s in zip(res, self.signs):
            rows.append(np.zeros(n_in) if r is None else (r * s if signed else r))
        return np.stack(rows)


def transpose(net, outputs, wanted_inputs):
    prog = Prog(net, outputs)
    live = set(prog.order)
    consumers = {n: [] for n in prog.order}
    for n in prog.order:
        k = net.nodes[n]
        if k[0] == 'add':
            consumers[k[1]].append((n, 1.0)); consumers[k[2]].append((n, 1.0))
        elif k[0] == 'sub':
            consumers[k[1]].append((n, 1.0)); consumers[k[2]].append((n, -1.0))
        elif k[0] == 'mul':
            consumers[k[1]].append((n, k[2]))
    outmap = {}
    for r, o in enumerate(outputs):
        if o is not None:
            outmap.setdefault(o[0], []).append((r, o[1]))
    tn = Net()
    memo = {}

    def adj(n):
        if n in memo:
            return memo[n]
        acc = None
        for r, s in outmap.get(n, []):
            v = tn.inp(r)
            acc = tn.add(acc, v if s > 0 else tn.neg(v))
        for c, coef in consumers[n]:
            acc = tn.add(acc, tn.mul(adj(c), coef))
        memo[n] = acc
        return acc
    outs = []
    for i in wanted_inputs:
        key = ('in', i)
        if key in net.cse and net.cse[key] in live:
            outs.append(adj(net.cse[key]))
        else:
            outs.append(None)
    return tn, outs


def build(N, taps, scale=True, variant=0):
    hop = N - taps + 1
    na = Net()
    U = rfft(na, [na.inp(t) for t in range(N)])
    a_out = [U[0][0], U[N // 2][0]]
    bins = list(range(1, N // 2))
    for k in bins:
        a, b = U[k]
        if variant == 0:
            a_out += [na.add(a, b), a, b]
        else:
            a_out += [a, na.sub(b, a), na.add(a, b)]
    nc = Net()
    V = rfft(nc, [nc.inp(t) for t in range(N)])
    c_out = [V[0][0], V[N // 2][0]]
    for k in bins:
        al, be = V[k]
        c_out += [nc.add(al, be), be, nc.neg(al)]
    tn, c_res = transpose(nc, c_out, list(range(hop)))
    def mkb(ntaps):
        nb = Net()
        Wf = rfft(nb, [nb.inp(t) if t < ntaps else None for t in range(N)])
        s0 = 1.0 / N if scale else 0.5
        b_out = [nb.mul(Wf[0][0], s0), nb.mul(Wf[N // 2][0], s0)]
        for k in bins:
            c = Wf[k][0]
            d = nb.neg(Wf[k][1])
            sc = 2.0 / N if scale else 1.0
            if variant == 0:
                b_out += [nb.mul(c, sc), nb.mul(nb.sub(d, c), sc), nb.mul(nb.add(c, d), sc)]
            else:
                b_out += [nb.mul(nb.add(c, d), sc), nb.mul(c, sc), nb.mul(d, sc)]
        return nb, b_out
    nb, b_out = mkb(taps)
    nb1, b1_out = mkb(taps - 1)
    return dict(N=N, hop=hop, taps=taps, na=na, a_out=a_out, nb=nb, b_out=b_out, nb1=nb1, b1_out=b1_out,
                tn=tn, c_res=c_res, bins=bins)


def max_live(net, order, outputs, out_at_once=True):
    uses = {n: 0 for n in order}
    for n in order:
        k = net.nodes[n]
        for a in ([k[1], k[2]] if k[0] in ('add', 'sub') else [k[1]] if k[0] == 'mul' else []):
            uses[a] += 1
    live = set(); peak = 0; tot = 0
    rem = dict(uses)
    for n in order:
        k = net.nodes[n]
        live.add(n)
        peak = max(peak, len(live))
        for a in set([k[1], k[2]] if k[0] in ('add', 'sub') else [k[1]] if k[0] == 'mul' else []):
            rem[a] -= (1 if k[0] == 'mul' or k[1] != k[2] else 2)
            if rem[a] == 0:
                live.discard(a)
        if rem[n] == 0:
            live.discard(n)
        tot += len(live)
    return peak, tot / len(order)


def min_live_order(net, outputs, seed=0, tries=200):
    base = Prog(net, outputs).order
    nodes = set(base)
    def operands(n):
        k = net.nodes[n]
        return [k[1], k[2]] if k[0] in ('add', 'sub') else [k[1]] if k[0] == 'mul' else []
    consumers = {n: [] for n in base}
    for n in base:
        for a in set(operands(n)):
            consumers[a].append(n)
    best = (max_live(net, base, outputs), base)
    rnd = random.Random(seed)
    pos = {n: i for i, n in enumerate(base)}
    for it in range(tries):
        done = set(); order = []
        live = set()
        remc = {n: len(consumers[n]) for n in base}
        isin = {n: net.nodes[n][0] == 'in' for n in base}
        def ready(n):
            return n not in done and not isin[n] and all((a in done) or isin[a] for a in operands(n))
        noise = rnd.random() * 1.5
        work = [n for n in base if not isin[n]]
        left = set(work)
        while left:
            cands = [n for n in left if ready(n)]
            def score(n):
                ops = set(operands(n))
                newloads = sum(1 for a in ops if a not in done)
                kills = sum(1 for a in ops if remc[a] == 1)
                born = 0 if remc[n] == 0 else 1
                return (newloads + born - kills) + noise * rnd.random() + 1e-4 * pos[n]
            n = min(cands, key=score)
            for a in sorted(set(operands(n)), key=lambda a: pos[a]):
                if a not in done:
                    done.add(a); order.append(a)
                remc[a] -= 1
            done.add(n); order.append(n); left.discard(n)
        ml = max_live(net, order, outputs)
        if ml < best[0]:
            best = (ml, order)
    return best


def solve_signs(G, iters=200000, seed=0):
    rnd = random.Random(seed)
    nets = {'A': (G['na'], G['a_out']), 'B': (G['nb'], G['b_out']), 'C': (G['tn'], G['c_res'])}
    order = {k: Prog(*v).order for k, v in nets.items()}
    R = len(G['a_out'])
    sig = {}
    for k in 'ABC':
        for n in order[k]:
            sig[(k, n)] = 1
    fixed = set()
    for k in 'AB':
        for n in order[k]:
            if nets[k][0].nodes[n][0] == 'in':
                fixed.add((k, n))
    for o in G['c_res']:
        sig[('C', o[0])] = o[1]; fixed.add(('C', o[0]))
    cin = {}
    for n in order['C']:
        nd = G['tn'].nodes[n]
        if nd[0] == 'in':
            cin[nd[1]] = n; fixed.add(('C', n))
    def cin_sign(r):
        a, b = G['a_out'][r], G['b_out'][r]
        return (sig[('A', a[0])] * a[1]) * (sig[('B', b[0])] * b[1])
    outmap = {}
    for r in range(R):
        outmap.setdefault(('A', G['a_out'][r][0]), []).append(r)
        outmap.setdefault(('B', G['b_out'][r][0]), []).append(r)
    def refresh():
        for r, n in cin.items():
            sig[('C', n)] = cin_sign(r)
    clauses = []
    for k in 'ABC':
        net = nets[k][0]
        for n in order[k]:
            nd = net.nodes[n]
            if nd[0] in ('add', 'sub'):
                clauses.append((k, n, nd[1], nd[2], 1 if nd[0] == 'add' else -1))
    occ = {}
    for ci, (k, n, a, b, cb) in enumerate(clauses):
        for v in (n, a, b):
            occ.setdefault((k, v), []).append(ci)
    def viol(ci):
        k, n, a, b, cb = clauses[ci]
        return sig[(k, n)] * sig[(k, a)] < 0 and sig[(k, n)] * cb * sig[(k, b)] < 0
    def flip(v):
        sig[v] = -sig[v]
        for r in outmap.get(v, []):
            if r in cin:
                sig[('C', cin[r])] = cin_sign(r)
    def affected(v):
        cs = set(occ.get(v, []))
        for r in outmap.get(v, []):
            if r in cin:
                cs.update(occ.get(('C', cin[r]), []))
        return cs
    flippers = {}
    for v, rs in outmap.items():
        for r in rs:
            if r in cin:
                flippers.setdefault(('C', cin[r]), []).append(v)
    refresh()
    bad = {ci for ci in range(len(clauses)) if viol(ci)}
    best = (len(bad), dict(sig))
    for it in range(iters):
        if not bad:
            break
        ci = rnd.choice(list(bad))
        k, n, a, b, cb = clauses[ci]
        cands = []
        for v in ((k, n), (k, a), (k, b)):
            if v in fixed:
                cands += flippers.get(v, [])
            else:
                cands.append(v)
        cands = [v for v in cands if v not in fixed]
        if not cands:
            continue
        def delta(v):
            cs = affected(v)
            before = sum(viol(c) for c in cs)
            flip(v)
            after = sum(viol(c) for c in cs)
            flip(v)
            return after - before
        if rnd.random() < 0.2:
            v = rnd.choice(cands)
        else:
            v = min(cands, key=lambda v: (delta(v), rnd.random()))
        cs = affected(v)
        flip(v)
        for c in cs:
            if viol(c): bad.add(c)
            else: bad.discard(c)
        if len(bad) < best[0]:
            best = (len(bad), dict(sig))
    nb, sg = best
    return ({n: s for (k, n), s in sg.items() if k == 'A'}, {n: s for (k, n), s in sg.items() if k == 'B'},
            {n: s for (k, n), s in sg.items() if k == 'C'}, nb)


class FixedProg:
    def __init__(self, net, outputs, sig, order=None):
        self.net, self.outputs, self.sig = net, outputs, sig
        self.order = order if order is not None else Prog(net, outputs).order
    def count(self):
        c = {'add': 0, 'sub': 0, 'mul': 0, 'in': 0}
        for n in self.order:
            c[self.net.nodes[n][0]] += 1
        return c


N, TAPS = 40, 16
G = build(N, TAPS, scale=False, variant=1)
HOP = G['hop']; R = len(G['a_out'])
T, D, K = 16000, 512, 31
L = (T - K) // 2 + 1
MB = 64; NCH = -(-L // (HOP * MB))
CH = HOP * MB
XM = CH + 16
LP = NCH * CH
TM = T // 2
LAST_M = TM - (NCH - 1) * CH
HS = 2.0 / N
T2 = 1; W3 = 1
U32, F32, BF16 = jnp.uint32, jnp.float32, jnp.bfloat16

bins = G['bins']
ev = [0, 1] + [2 + 3 * i + q for i, k in enumerate(bins) if k % 2 == 0 for q in range(3)]
od = [2 + 3 * i + q for i, k in enumerate(bins) if k % 2 == 1 for q in range(3)]
if (N // 2) % 2 == 1:
    ev.remove(1); od = [1] + od
IDX = (ev, od)
RH = (len(ev), len(od))
LOC = {}
for hf in range(2):
    for i, r in enumerate(IDX[hf]):
        LOC[r] = (hf, i)
SA, SB, SC, NBAD = solve_signs(G)
assert NBAD == 0
def mkprog(net, outs, sig):
    return FixedProg(net, outs, sig, order=min_live_order(net, outs, tries=100)[1])
PA = [mkprog(G['na'], [G['a_out'][r] for r in idx], SA) for idx in IDX]
PB = [mkprog(G['nb'], [G['b_out'][r] for r in idx], SB) for idx in IDX]
PC = mkprog(G['tn'], G['c_res'], SC)


def run_gen(prog, loads, sink):
    nsets = len(loads)
    vals = [dict() for _ in range(nsets)]
    sig = prog.sig
    outs = {}
    for r, o in enumerate(prog.outputs):
        outs.setdefault(o[0], []).append(r)
    for n in prog.order:
        k = prog.net.nodes[n]
        for s in range(nsets):
            v = vals[s]
            if k[0] == 'in':
                v[n] = loads[s](k[1])
            elif k[0] == 'mul':
                v[n] = v[k[1]] * (k[2] * sig[n] * sig[k[1]])
            else:
                a, b = k[1], k[2]
                cb = 1 if k[0] == 'add' else -1
                p, q = sig[n] * sig[a], sig[n] * cb * sig[b]
                if p > 0 and q > 0: v[n] = v[a] + v[b]
                elif p > 0: v[n] = v[a] - v[b]
                elif q > 0: v[n] = v[b] - v[a]
                else: v[n] = -(v[a] + v[b])
            yield 1
        for r in outs.get(n, []):
            yield from sink(r, [vals[s][n] for s in range(nsets)])


def drain(gen):
    for _ in gen:
        pass


def unpack(wd, hi):
    wd = (wd & jnp.uint32(0xffff0000)) if hi else (wd << 16)
    return lax.bitcast_convert_type(wd, F32)


def pack(lo, hi):
    return pltpu.pack_elementwise([lo, hi], packed_dtype=BF16)


def prog_weight(prog, nsets, per_out):
    return len(prog.order) * nsets + len(prog.outputs) * per_out


def interleave(mms, gens_weights):
    total = sum(w for _, w in gens_weights)
    def allops():
        for g, _ in gens_weights:
            yield from g
    gen = allops()
    e = 0; done = False
    for i, mm in enumerate(mms):
        mm()
        tgt = (i + 1) * total // len(mms)
        while not done and e < tgt:
            try:
                e += next(gen)
            except StopIteration:
                done = True
    for _ in gen:
        pass


def merge(lists):
    lists = [l for l in lists if l]
    out = []
    pos = [0] * len(lists)
    tot = sum(len(l) for l in lists)
    for _ in range(tot):
        i = min((i for i in range(len(lists)) if pos[i] < len(lists[i])), key=lambda i: (pos[i] + 0.5) / len(lists[i]))
        out.append(lists[i][pos[i]]); pos[i] += 1
    return out


C0 = math.sqrt(2.0 / math.pi)
def gelu_half(zh):
    u = zh * (zh * zh * (8.0 * C0 * 0.044715) + 2.0 * C0)
    return zh * jnp.tanh(u) + zh


def kernel(x_hbm, w_hbm, gam_ref, bet_ref, out_hbm,
           xb0, xb1, xb2, xb3, we, wo, xe, xo, ye, yo, h0, h1, h2, h3, st, nrm, gsm, xsem, wsem, osem):
    xb = (xb0, xb1, xb2, xb3)
    wh = (we, wo); xh = (xe, xo); yy = (ye, yo)
    hh = (h0, h1, h2, h3)
    x32 = x_hbm.bitcast(U32)
    w32 = w_hbm.bitcast(F32)
    o32 = out_hbm.bitcast(F32)
    LASTJ = 2 * NCH - 1

    def x_copy(j, c, full):
        b = j // NCH
        cj = j % NCH
        rows = XM if full else LAST_M
        return pltpu.make_async_copy(
            x32.at[b, pl.ds(pl.multiple_of(cj * CH, 8), rows), pl.ds(c * 128, 128)],
            xb[c].at[pl.ds(0, rows), :], xsem.at[c])

    def x_start(j):
        cj = j % NCH
        @pl.when(cj < NCH - 1)
        def _():
            for c in range(4):
                x_copy(j, c, True).start()
        @pl.when(cj == NCH - 1)
        def _():
            for c in range(4):
                x_copy(j, c, False).start()
                xb[c][pl.ds(LAST_M, XM - LAST_M), :] = jnp.zeros((XM - LAST_M, 128), U32)

    def x_wait(j, cs=range(4)):
        cj = j % NCH
        @pl.when(cj < NCH - 1)
        def _():
            for c in cs:
                x_copy(j, c, True).wait()
        @pl.when(cj == NCH - 1)
        def _():
            for c in cs:
                x_copy(j, c, False).wait()

    WQ = 4
    def w_copy(n, q):
        dst = hh[n].at[1, pl.ds(0, K * 256), :].reshape(K, 256, 128)
        r = 256 // WQ
        return pltpu.make_async_copy(w32.at[:, pl.ds(q * r, r), pl.ds(n * 128, 128)], dst.at[:, pl.ds(q * r, r), :], wsem.at[n, q])

    def o_copy(n, r0, rows, k):
        return pltpu.make_async_copy(hh[n].at[0, pl.ds(r0, rows), :], o32.at[pl.ds(r0, rows), n, 0, :], osem.at[n, k])

    def a_piece(g, c, p, half):
        dyn = not isinstance(g, int)
        base = pl.multiple_of(g * (16 * HOP), 8) if dyn else g * (16 * HOP)
        row = pl.multiple_of(g * 8, 8) if dyn else g * 8
        xw = xb[c].at[pl.ds(base, 16 * HOP + 16), :]
        def mkload(o):
            return lambda t: unpack(xw[pl.ds(t + o * HOP, 8, stride=2 * HOP), :], p)
        def sink(i, vs):
            xh[half][i, pl.ds(row, 8), p * 512 + c * 128:p * 512 + (c + 1) * 128] = pack(vs[0], vs[1])
            yield 1
        return run_gen(PA[half], [mkload(0), mkload(1)], sink), prog_weight(PA[half], 2, 1)

    def a_pieces(half):
        return [a_piece(g, c, p, half) for c in range(4) for g in range(MB // 16) for p in range(2)]

    def w_piece(n, g, p, half):
        dyn = not isinstance(g, int)
        row = pl.multiple_of(g * 8, 8) if dyn else g * 8
        cache = {}
        def word(j):
            if j not in cache:
                cache[j] = lax.bitcast_convert_type(hh[n][1, pl.ds((2 * j + p) * 256 + row, 8), :], U32)
            return cache[j]
        def mkload(hi):
            def load(j):
                if 2 * j + p >= K:
                    return jnp.zeros((8, 128), F32)
                return unpack(word(j), hi)
            return load
        def sink(i, vs):
            wh[half][n, i, pl.ds(p * 256 + row, 8), :] = pack(vs[0], vs[1])
            yield 1
        return run_gen(PB[half], [mkload(0), mkload(1)], sink), prog_weight(PB[half], 2, 1)

    def c_pieces(j, n):
        if isinstance(j, int):
            b, cj = j // NCH, j % NCH
            slot = b
        else:
            valid = j >= 0
            b = jnp.where(valid, j // NCH, 0)
            cj = jnp.where(valid, j % NCH, NCH - 1)
            slot = jnp.where(valid, b, 2)
        state = {}
        def col(g):
            if g == 0:
                state['c'] = st[slot, n, 2]; state['a1'] = st[slot, n, 0]; state['a2'] = st[slot, n, 1]
            base = cj * CH + g * (8 * HOP)
            if not isinstance(j, int):
                base = pl.multiple_of(base, 8)
            hs = hh[n].at[b, pl.ds(base, 8 * HOP), :]
            def sink(t, vs):
                hs[pl.ds(t, 8, stride=HOP), :] = vs[0]
                d = vs[0] - state['c']
                state['a1'] = state['a1'] + d
                state['a2'] = state['a2'] + d * d
                yield 4
            yield from run_gen(PC, [lambda r: yy[LOC[r][0]][n, LOC[r][1], g * 8:(g + 1) * 8, :]], sink)
            if g == MB // 8 - 1:
                st[slot, n, 0] = state['a1']; st[slot, n, 1] = state['a2']
        return [(col(g), prog_weight(PC, 1, 4)) for g in range(MB // 8)]

    def set_shift(j, n):
        @pl.when(jnp.logical_and(j >= 0, j % NCH == 0))
        def _():
            st[j // NCH, n, 2] = jnp.broadcast_to(ye[n, LOC[0][1], 0:1, :], (8, 128))

    def finalize_stats(n):
        sub = lax.broadcasted_iota(jnp.int32, (8, 128), 0)
        for b in range(2):
            c = st[b, n, 2]
            r0 = (L // 8) * 8
            c1 = jnp.zeros((8, 128), F32); c2 = jnp.zeros((8, 128), F32)
            for r in range(r0, LP, 8):
                d = hh[n][b, r:r + 8, :] - c
                if r < L:
                    d = jnp.where(sub >= L - r, d, 0.0)
                c1 = c1 + d; c2 = c2 + d * d
            s1 = jnp.sum(st[b, n, 0] - c1, axis=0, keepdims=True)
            s2 = jnp.sum(st[b, n, 1] - c2, axis=0, keepdims=True)
            md = s1 * (1.0 / L)
            var = (s2 * (1.0 / L) - md * md) * (HS * HS)
            mu = c[0:1] + md
            a = (HS * lax.rsqrt(var + 1e-5)) * gam_ref[...].astype(F32).reshape(1, D)[:, n * 128:(n + 1) * 128]
            bb = bet_ref[...].astype(F32).reshape(1, D)[:, n * 128:(n + 1) * 128] - mu * a
            nrm[n, b, 0] = jnp.broadcast_to(0.5 * a, (8, 128))
            nrm[n, b, 1] = jnp.broadcast_to(0.5 * bb, (8, 128))

    def d_vreg(n, r, cs):
        a0, b0, a1, b1 = cs
        z0 = gelu_half(hh[n][0, pl.ds(r, 8), :] * a0 + b0)
        z1 = gelu_half(hh[n][1, pl.ds(r, 8), :] * a1 + b1)
        hh[n][0, pl.ds(r, 8), :] = lax.bitcast_convert_type(pack(z0, z1), F32)

    def d_consts(n):
        return nrm[n, 0, 0], nrm[n, 0, 1], nrm[n, 1, 0], nrm[n, 1, 1]

    def d_pieces(n, ra=0, rb=LP):
        state = {}
        def piece(r0, r1):
            if 'cs' not in state:
                state['cs'] = d_consts(n)
            for r in range(r0, r1, 8):
                d_vreg(n, r, state['cs'])
                yield 19
        P = 200
        return [(piece(r, min(r + P, rb)), 19 * (min(r + P, rb) - r) // 8) for r in range(ra, rb, P)]

    def fin_piece(n):
        def gen():
            finalize_stats(n)
            yield 100
        return [(gen(), 100)]

    NPC = 4
    PR = -(-(-(-L // NPC)) // 8) * 8
    def d_loop(n, k0):
        cs = d_consts(n)
        UN = 5
        for k in range(k0, NPC):
            r0 = k * PR; r1 = min(r0 + PR, LP)
            nv = -(-(r1 - r0) // 8)
            assert nv % UN == 0, nv
            def body(i, carry):
                for u in range(UN):
                    d_vreg(n, pl.multiple_of(r0 + (i * UN + u) * 8, 8), cs)
                return carry
            lax.fori_loop(0, nv // UN, body, 0)
            o_copy(n, r0, min(r0 + PR, L) - r0, k).start()

    def o_start_all(n):
        for k in range(NPC):
            r0 = k * PR
            o_copy(n, r0, min(r0 + PR, L) - r0, k).start()

    def o_wait_all(n):
        for k in range(NPC):
            r0 = k * PR
            o_copy(n, r0, min(r0 + PR, L) - r0, k).wait()

    def mm(half, n, i):
        def f():
            lhs = pltpu.bitcast(xh[half][i], BF16)
            rhs = pltpu.bitcast(wh[half][n, i], BF16)
            yy[half][n, i] = jnp.dot(lhs, rhs, preferred_element_type=F32)
        return f

    def body(name, half, tiles, lists, sl=None):
        mms = [mm(half, n, i) for n in tiles for i in range(RH[half])]
        if sl is not None:
            mms = mms[sl]
        with jax.named_scope(name):
            interleave(mms, merge(lists))

    j0 = jnp.int32(0)
    for k_ in range(32):
        gsm[k_] = jnp.int32(0)
    x_start(j0)
    for q in range(WQ):
        w_copy(0, q).start()
    st[...] = jnp.zeros_like(st)

    with jax.named_scope("a0"):
        for c in range(4):
            x_wait(j0, [c])
            def a0(g, carry):
                for p in range(2):
                    drain(a_piece(g, c, p, 0)[0])
                return carry
            lax.fori_loop(0, MB // 16, a0, 0)
        for n in range(1, 4):
            for q in range(WQ):
                w_copy(n, q).start()

    with jax.named_scope("wstage"):
        GP = 32 // WQ
        for n in range(4):
            phases = (1,) if (n == 3 and W3) else (0, 1)
            def wl(g, carry):
                for p in phases:
                    for half in range(2):
                        drain(w_piece(n, g, p, half)[0])
                return carry
            def wq(q, carry):
                w_copy(n, q).wait()
                lax.fori_loop(q * GP, (q + 1) * GP, wl, 0)
                return carry
            lax.fori_loop(0, WQ, wq, 0)

    def main(j, carry):
        @pl.when(j >= 0)
        def _():
            body("E01", 0, (0, 1), [a_pieces(1)])
        @pl.when(j + 1 <= LASTJ)
        def _():
            x_start(j + 1)
        set_shift(j - 1, 2); set_shift(j - 1, 3)
        if W3:
            @pl.when(j == 0)
            def _():
                body("O01W", 1, (0, 1), [[w_piece(3, g, 0, half) for g in range(32) for half in range(2)]])
        @pl.when(j + 1 >= (2 if W3 else 1))
        def _():
            body("O01", 1, (0, 1), [c_pieces(j - 1, 2), c_pieces(j - 1, 3)])
        @pl.when(j < (LASTJ if T2 else LASTJ + 1))
        def _():
            set_shift(j, 0); set_shift(j, 1)
        @pl.when(j + 2 < (LASTJ if T2 else LASTJ + 1) + 2)
        def _():
            body("E23", 0, (2, 3), [c_pieces(j, 0), c_pieces(j, 1)])
        @pl.when(j + 1 <= LASTJ)
        def _():
            x_wait(j + 1)
        @pl.when(j < (LASTJ if T2 else LASTJ + 1))
        def _():
            body("O23", 1, (2, 3), [a_pieces(0)])
        return carry
    lax.fori_loop(0, LASTJ + 1, main, 0)

    jl = jnp.int32(LASTJ)
    if T2:
        gd = gsm[0]
        set_shift(jl, 0); set_shift(jl, 1)
        def o_start(n, ks):
            for k in ks:
                r0 = k * PR
                o_copy(n, r0, min(r0 + PR, L) - r0, k).start()
        def dq(n, k):
            return d_pieces(n, k * PR, min((k + 1) * PR, LP))
        allmm = [(0, 2, i) for i in range(RH[0])] + [(0, 3, i) for i in range(RH[0])] + \
                [(1, 2, i) for i in range(RH[1])] + [(1, 3, i) for i in range(RH[1])]
        no3 = len(allmm) - RH[1]
        cuts = [0, 12, 29, 46, 65, no3, len(allmm)]
        plan = [
            (c_pieces(LASTJ, 0) + fin_piece(0) + dq(0, 0), [(0, 0)]),
            (dq(0, 1), [(0, 1)]),
            (dq(0, 2) + c_pieces(LASTJ, 1) + fin_piece(1), [(0, 2)]),
            (dq(0, 3) + dq(1, 0), [(0, 3), (1, 0)]),
            (dq(1, 1) + dq(1, 2), [(1, 1), (1, 2)]),
            (dq(1, 3) + c_pieces(LASTJ, 2) + fin_piece(2) + dq(2, 0), [(1, 3), (2, 0)]),
        ]
        set_shift(jl, 2)
        for bi, (pcs, starts) in enumerate(plan):
            @pl.when(gsm[16 + bi] >= 0)
            def _():
                with jax.named_scope("D%d" % bi):
                    interleave([mm(*t) for t in allmm[cuts[bi]:cuts[bi + 1]]], pcs)
            for n_, k_ in starts:
                o_start(n_, (k_,))

    with jax.named_scope("tail"):
        set_shift(jl, 3)
        d_loop(2, 1)
        for g_, _ in c_pieces(LASTJ, 3):
            drain(g_)
        finalize_stats(3)
        d_loop(3, 0)
        for n in range(4):
            o_wait_all(n)


@jax.jit
def pallas_standalone__self_sup_conv_stem_wavlm__speech_kernel(x, w, gn_gamma, gn_beta):
    out = pl.pallas_call(
        kernel,
        in_specs=[pl.BlockSpec(memory_space=pl.ANY), pl.BlockSpec(memory_space=pl.ANY),
                  pl.BlockSpec(memory_space=pltpu.VMEM), pl.BlockSpec(memory_space=pltpu.VMEM)],
        out_specs=pl.BlockSpec(memory_space=pl.ANY),
        out_shape=jax.ShapeDtypeStruct((L, 4, 2, 128), BF16),
        scratch_shapes=[pltpu.VMEM((XM, 128), U32)] * 4 + [
            pltpu.VMEM((4, RH[0], 512, 128), U32),
            pltpu.VMEM((4, RH[1], 512, 128), U32),
            pltpu.VMEM((RH[0], MB // 2, 1024), U32),
            pltpu.VMEM((RH[1], MB // 2, 1024), U32),
            pltpu.VMEM((4, RH[0], MB, 128), F32),
            pltpu.VMEM((4, RH[1], MB, 128), F32)] + [pltpu.VMEM((2, LP, 128), F32)] * 4 + [
            pltpu.VMEM((3, 4, 3, 8, 128), F32),
            pltpu.VMEM((4, 2, 2, 8, 128), F32),
            pltpu.SMEM((32,), jnp.int32),
            pltpu.SemaphoreType.DMA((4,)),
            pltpu.SemaphoreType.DMA((4, 4)),
            pltpu.SemaphoreType.DMA((4, 4)),
        ],
        compiler_params=pltpu.CompilerParams(vmem_limit_bytes=127 * 1024 * 1024),
    )(x, w, gn_gamma, gn_beta)
    return out.transpose(2, 0, 1, 3).reshape(2, L, D)
```

```python
import math
import random
import numpy as np
import jax, jax.numpy as jnp
from jax import lax
from jax.experimental import pallas as pl
from jax.experimental.pallas import tpu as pltpu


class Net:
    def __init__(self):
        self.nodes = []
        self.cse = {}

    def _mk(self, key):
        if key in self.cse:
            return self.cse[key]
        self.nodes.append(key)
        self.cse[key] = len(self.nodes) - 1
        return self.cse[key]

    def inp(self, i):
        return (self._mk(('in', i)), 1)

    def neg(self, x):
        return None if x is None else (x[0], -x[1])

    def add(self, x, y):
        if x is None:
            return y
        if y is None:
            return x
        (a, sa), (b, sb) = x, y
        if a == b:
            if sa == sb:
                return self.mul(x, 2.0)
            return None
        if sa == sb:
            if a > b:
                a, b = b, a
            return (self._mk(('add', a, b)), sa)
        if a > b:
            a, b, sa = b, a, sb
        return (self._mk(('sub', a, b)), sa)

    def sub(self, x, y):
        return self.add(x, self.neg(y))

    def mul(self, x, c):
        if x is None or abs(c) < 1e-12:
            return None
        a, s = x
        if c < 0:
            c, s = -c, -s
        if abs(c - 1.0) < 1e-12:
            return (a, s)
        c = float(np.float64(round(c, 14)))
        return (self._mk(('mul', a, c)), s)

    def cadd(self, x, y):
        return (self.add(x[0], y[0]), self.add(x[1], y[1]))

    def csub(self, x, y):
        return (self.sub(x[0], y[0]), self.sub(x[1], y[1]))

    def cmulc(self, x, c, s):
        a, b = x
        if abs(s) < 1e-12:
            return (self.mul(a, c), self.mul(b, c))
        if abs(c) < 1e-12:
            return (self.mul(b, -s), self.mul(a, s))
        if abs(abs(c) - abs(s)) < 1e-12:
            sg = 1.0 if s * c > 0 else -1.0
            re = self.sub(a, self.mul(b, sg))
            im = self.add(b, self.mul(a, sg))
            return (self.mul(re, c), self.mul(im, c))
        re = self.sub(self.mul(a, c), self.mul(b, s))
        im = self.add(self.mul(a, s), self.mul(b, c))
        return (re, im)


def w(k, n):
    ang = -2.0 * math.pi * (k % n) / n
    return math.cos(ang), math.sin(ang)


def cfft(net, z):
    n = len(z)
    if n == 1:
        return [z[0]]
    if n == 2:
        return [net.cadd(z[0], z[1]), net.csub(z[0], z[1])]
    if n % 4 == 0:
        h, q = n // 2, n // 4
        e = [net.cadd(z[t], z[t + h]) for t in range(h)]
        o = [net.csub(z[t], z[t + h]) for t in range(h)]
        z1, z3 = [], []
        for t in range(q):
            a, b = o[t], o[t + q]
            mib = (b[1], net.neg(b[0]))
            p = net.cadd(a, mib)
            m = net.csub(a, mib)
            z1.append(net.cmulc(p, *w(t, n)))
            z3.append(net.cmulc(m, *w(3 * t, n)))
        E = cfft(net, e)
        Z1 = cfft(net, z1)
        Z3 = cfft(net, z3)
        out = [None] * n
        for k in range(h):
            out[2 * k] = E[k]
        for k in range(q):
            out[4 * k + 1] = Z1[k]
            out[4 * k + 3] = Z3[k]
        return out
    if n % 2 == 0:
        m = n // 2
        out = [None] * n
        rows = []
        for t2 in range(m):
            a = z[(2 * t2) % n]
            b = z[(m + 2 * t2) % n]
            rows.append((net.cadd(a, b), net.csub(a, b)))
        for k1 in range(2):
            Z = cfft(net, [rows[t2][k1] for t2 in range(m)])
            for k2 in range(m):
                for k in range(n):
                    if k % 2 == k1 and k % m == k2:
                        out[k] = Z[k2]
        return out
    if n % 3 == 0 and n > 3:
        raise NotImplementedError
    out = []
    p = {t: net.cadd(z[t], z[n - t]) for t in range(1, (n + 1) // 2)}
    q = {t: net.csub(z[t], z[n - t]) for t in range(1, (n + 1) // 2)}
    s = z[0]
    for t in p:
        s = net.cadd(s, p[t])
    out = [None] * n
    out[0] = s
    for k in range(1, (n + 1) // 2):
        A = z[0]
        B = (None, None)
        for t in p:
            c, sn = w(k * t, n)
            A = net.cadd(A, (net.mul(p[t][0], c), net.mul(p[t][1], c)))
            B = net.cadd(B, (net.mul(q[t][1], -sn), net.mul(q[t][0], sn)))
        out[k] = net.cadd(A, B)
        out[n - k] = net.csub(A, B)
    return out


def cfft_pfa(net, z, n1, n2):
    n = n1 * n2
    out = [None] * n
    cols = [cfft_any(net, [z[(n2 * t1 + n1 * t2) % n] for t2 in range(n2)]) for t1 in range(n1)]
    for k2 in range(n2):
        Z = cfft_any(net, [cols[t1][k2] for t1 in range(n1)])
        for k1 in range(n1):
            for k in range(n):
                if k % n1 == k1 and k % n2 == k2:
                    out[k] = Z[k1]
    return out


def cfft5(net, z):
    c1, c2 = math.cos(2 * math.pi / 5), math.cos(4 * math.pi / 5)
    s1, s2 = math.sin(2 * math.pi / 5), math.sin(4 * math.pi / 5)
    t1 = net.cadd(z[1], z[4]); t2 = net.cadd(z[2], z[3])
    t3 = net.csub(z[1], z[4]); t4 = net.csub(z[2], z[3])
    t5 = net.cadd(t1, t2)
    def rm(x, c):
        return (net.mul(x[0], c), net.mul(x[1], c))
    m1 = rm(t5, (c1 + c2) / 2 - 1.0)
    m2 = rm(net.csub(t1, t2), (c1 - c2) / 2)
    y0 = net.cadd(z[0], t5)
    a = net.cadd(y0, m1)
    a1 = net.cadd(a, m2); a2 = net.csub(a, m2)
    m3 = rm(net.cadd(t3, t4), s2)
    m4 = rm(t3, s1 - s2)
    m5 = rm(t4, s1 + s2)
    b1 = net.cadd(m3, m4)
    b2 = net.csub(m3, m5)
    def mi(x):
        return (x[1], net.neg(x[0]))
    return [y0, net.cadd(a1, mi(b1)), net.cadd(a2, mi(b2)), net.csub(a2, mi(b2)), net.csub(a1, mi(b1))]


def rfft5(net, x):
    c1, c2 = math.cos(2 * math.pi / 5), math.cos(4 * math.pi / 5)
    s1, s2 = math.sin(2 * math.pi / 5), math.sin(4 * math.pi / 5)
    t1 = net.add(x[1], x[4]); t2 = net.add(x[2], x[3])
    t3 = net.sub(x[1], x[4]); t4 = net.sub(x[2], x[3])
    t5 = net.add(t1, t2)
    m1 = net.mul(t5, (c1 + c2) / 2 - 1.0)
    m2 = net.mul(net.sub(t1, t2), (c1 - c2) / 2)
    y0 = net.add(x[0], t5)
    a = net.add(y0, m1)
    a1 = net.add(a, m2); a2 = net.sub(a, m2)
    m3 = net.mul(net.add(t3, t4), s2)
    m4 = net.mul(t3, s1 - s2)
    m5 = net.mul(t4, s1 + s2)
    b1 = net.add(m3, m4); b2 = net.sub(m3, m5)
    return [(y0, None), (a1, net.neg(b1)), (a2, net.neg(b2))]


def cfft_any(net, z):
    n = len(z)
    if n == 5:
        return cfft5(net, z)
    if n == 12:
        return cfft_pfa(net, z, 3, 4)
    if n == 10:
        return cfft_pfa(net, z, 5, 2)
    if n == 20:
        return cfft_pfa(net, z, 5, 4)
    if n == 6:
        return cfft_pfa(net, z, 3, 2)
    if n == 14:
        return cfft_pfa(net, z, 7, 2)
    if n == 15:
        return cfft_pfa(net, z, 5, 3)
    return cfft(net, z)


def rfft_pfa(net, x, n1, n2):
    n = n1 * n2
    inner = [rfft(net, [x[(n2 * t1 + n1 * t2) % n] for t1 in range(n1)]) for t2 in range(n2)]
    out = [None] * (n // 2 + 1)
    for k1 in range(n1 // 2 + 1):
        col = [inner[t2][k1] for t2 in range(n2)]
        if all(c[1] is None for c in col):
            Z = rfft(net, [c[0] for c in col])
            Z = Z + [(Z[n2 - k2][0], net.neg(Z[n2 - k2][1])) for k2 in range(len(Z), n2)]
        else:
            Z = cfft_any(net, col)
        for k2 in range(n2):
            k = [k for k in range(n) if k % n1 == k1 and k % n2 == k2][0]
            if k <= n // 2:
                if out[k] is None:
                    out[k] = Z[k2]
            else:
                if out[n - k] is None:
                    out[n - k] = (Z[k2][0], net.neg(Z[k2][1]))
    return out


PFA = {40: (8, 5), 20: (4, 5), 24: (8, 3), 48: (16, 3), 12: (4, 3), 56: (8, 7), 10: (2, 5), 6: (2, 3), 60: (4, 15), 15: (3, 5), 44: (4, 11), 36: (4, 9)}
USE_PFA = True


def rfft(net, x):
    n = len(x)
    if USE_PFA and n in PFA:
        return rfft_pfa(net, x, *PFA[n])
    if n == 1:
        return [(x[0], None)]
    if n == 2:
        return [(net.add(x[0], x[1]), None), (net.sub(x[0], x[1]), None)]
    if n % 4 == 0:
        h, q = n // 2, n // 4
        e = [net.add(x[t], x[t + h]) for t in range(h)]
        o = [net.sub(x[t], x[t + h]) for t in range(h)]
        z = [net.cmulc((o[t], net.neg(o[t + q])), *w(t, n)) for t in range(q)]
        E = rfft(net, e)
        Z = cfft_any(net, z)
        out = [None] * (h + 1)
        for k in range(len(E)):
            out[2 * k] = E[k]
        for k in range(q):
            f = 4 * k + 1
            if f <= h:
                out[f] = Z[k]
            else:
                out[n - f] = (Z[k][0], net.neg(Z[k][1]))
        return out
    if n % 2 == 0:
        m = n // 2
        e = [net.add(x[t], x[t + m]) for t in range(m)]
        o = [net.sub(x[t], x[t + m]) for t in range(m)]
        E = rfft(net, e)
        op = [o[t] if t % 2 == 0 else net.neg(o[t]) for t in range(m)]
        O = rfft(net, op)
        out = [None] * (m + 1)
        for k in range(len(E)):
            out[2 * k] = E[k]
        for f in range(1, m + 1, 2):
            j = ((f - m) // 2) % m
            if j <= m // 2:
                out[f] = O[j]
            else:
                out[f] = (O[m - j][0], net.neg(O[m - j][1]))
        return out
    if n == 5:
        return rfft5(net, x)
    p = {t: net.add(x[t], x[n - t]) for t in range(1, (n + 1) // 2)}
    q = {t: net.sub(x[t], x[n - t]) for t in range(1, (n + 1) // 2)}
    s = x[0]
    for t in p:
        s = net.add(s, p[t])
    out = [(s, None)]
    for k in range(1, (n + 1) // 2):
        A = x[0]
        B = None
        for t in p:
            c, sn = w(k * t, n)
            A = net.add(A, net.mul(p[t], c))
            B = net.add(B, net.mul(q[t], sn))
        out.append((A, B))
    return out


class Prog:
    def __init__(self, net, outputs):
        order = []
        seen = set()

        def visit(n):
            if n in seen:
                return
            seen.add(n)
            k = net.nodes[n]
            if k[0] in ('add', 'sub'):
                visit(k[1]); visit(k[2])
            elif k[0] == 'mul':
                visit(k[1])
            order.append(n)
        for o in outputs:
            if o is not None:
                visit(o[0])
        self.net = net
        self.order = order
        self.outputs = outputs

    def count(self):
        c = {'add': 0, 'sub': 0, 'mul': 0, 'in': 0}
        for n in self.order:
            c[self.net.nodes[n][0]] += 1
        return c

    def run(self, load, emit=None):
        vals = {}
        for n in self.order:
            k = self.net.nodes[n]
            if k[0] == 'in':
                vals[n] = load(k[1])
            elif k[0] == 'add':
                vals[n] = vals[k[1]] + vals[k[2]]
            elif k[0] == 'sub':
                vals[n] = vals[k[1]] - vals[k[2]]
            else:
                vals[n] = vals[k[1]] * k[2]
        return [None if o is None else vals[o[0]] for o in self.outputs]

    @property
    def signs(self):
        return [0 if o is None else o[1] for o in self.outputs]

    def matrix(self, n_in, signed=True):
        eye = np.eye(n_in)
        res = self.run(lambda i: eye[i])
        rows = []
        for r, s in zip(res, self.signs):
            rows.append(np.zeros(n_in) if r is None else (r * s if signed else r))
        return np.stack(rows)


def transpose(net, outputs, wanted_inputs):
    prog = Prog(net, outputs)
    live = set(prog.order)
    consumers = {n: [] for n in prog.order}
    for n in prog.order:
        k = net.nodes[n]
        if k[0] == 'add':
            consumers[k[1]].append((n, 1.0)); consumers[k[2]].append((n, 1.0))
        elif k[0] == 'sub':
            consumers[k[1]].append((n, 1.0)); consumers[k[2]].append((n, -1.0))
        elif k[0] == 'mul':
            consumers[k[1]].append((n, k[2]))
    outmap = {}
    for r, o in enumerate(outputs):
        if o is not None:
            outmap.setdefault(o[0], []).append((r, o[1]))
    tn = Net()
    memo = {}

    def adj(n):
        if n in memo:
            return memo[n]
        acc = None
        for r, s in outmap.get(n, []):
            v = tn.inp(r)
            acc = tn.add(acc, v if s > 0 else tn.neg(v))
        for c, coef in consumers[n]:
            acc = tn.add(acc, tn.mul(adj(c), coef))
        memo[n] = acc
        return acc
    outs = []
    for i in wanted_inputs:
        key = ('in', i)
        if key in net.cse and net.cse[key] in live:
            outs.append(adj(net.cse[key]))
        else:
            outs.append(None)
    return tn, outs


def build(N, taps, scale=True, variant=0):
    hop = N - taps + 1
    na = Net()
    U = rfft(na, [na.inp(t) for t in range(N)])
    a_out = [U[0][0], U[N // 2][0]]
    bins = list(range(1, N // 2))
    for k in bins:
        a, b = U[k]
        if variant == 0:
            a_out += [na.add(a, b), a, b]
        else:
            a_out += [a, na.sub(b, a), na.add(a, b)]
    nc = Net()
    V = rfft(nc, [nc.inp(t) for t in range(N)])
    c_out = [V[0][0], V[N // 2][0]]
    for k in bins:
        al, be = V[k]
        c_out += [nc.add(al, be), be, nc.neg(al)]
    tn, c_res = transpose(nc, c_out, list(range(hop)))
    def mkb(ntaps):
        nb = Net()
        Wf = rfft(nb, [nb.inp(t) if t < ntaps else None for t in range(N)])
        s0 = 1.0 / N if scale else 0.5
        b_out = [nb.mul(Wf[0][0], s0), nb.mul(Wf[N // 2][0], s0)]
        for k in bins:
            c = Wf[k][0]
            d = nb.neg(Wf[k][1])
            sc = 2.0 / N if scale else 1.0
            if variant == 0:
                b_out += [nb.mul(c, sc), nb.mul(nb.sub(d, c), sc), nb.mul(nb.add(c, d), sc)]
            else:
                b_out += [nb.mul(nb.add(c, d), sc), nb.mul(c, sc), nb.mul(d, sc)]
        return nb, b_out
    nb, b_out = mkb(taps)
    nb1, b1_out = mkb(taps - 1)
    return dict(N=N, hop=hop, taps=taps, na=na, a_out=a_out, nb=nb, b_out=b_out, nb1=nb1, b1_out=b1_out,
                tn=tn, c_res=c_res, bins=bins)


def max_live(net, order, outputs, out_at_once=True):
    uses = {n: 0 for n in order}
    for n in order:
        k = net.nodes[n]
        for a in ([k[1], k[2]] if k[0] in ('add', 'sub') else [k[1]] if k[0] == 'mul' else []):
            uses[a] += 1
    live = set(); peak = 0; tot = 0
    rem = dict(uses)
    for n in order:
        k = net.nodes[n]
        live.add(n)
        peak = max(peak, len(live))
        for a in set([k[1], k[2]] if k[0] in ('add', 'sub') else [k[1]] if k[0] == 'mul' else []):
            rem[a] -= (1 if k[0] == 'mul' or k[1] != k[2] else 2)
            if rem[a] == 0:
                live.discard(a)
        if rem[n] == 0:
            live.discard(n)
        tot += len(live)
    return peak, tot / len(order)


def min_live_order(net, outputs, seed=0, tries=200):
    base = Prog(net, outputs).order
    nodes = set(base)
    def operands(n):
        k = net.nodes[n]
        return [k[1], k[2]] if k[0] in ('add', 'sub') else [k[1]] if k[0] == 'mul' else []
    consumers = {n: [] for n in base}
    for n in base:
        for a in set(operands(n)):
            consumers[a].append(n)
    best = (max_live(net, base, outputs), base)
    rnd = random.Random(seed)
    pos = {n: i for i, n in enumerate(base)}
    for it in range(tries):
        done = set(); order = []
        live = set()
        remc = {n: len(consumers[n]) for n in base}
        isin = {n: net.nodes[n][0] == 'in' for n in base}
        def ready(n):
            return n not in done and not isin[n] and all((a in done) or isin[a] for a in operands(n))
        noise = rnd.random() * 1.5
        work = [n for n in base if not isin[n]]
        left = set(work)
        while left:
            cands = [n for n in left if ready(n)]
            def score(n):
                ops = set(operands(n))
                newloads = sum(1 for a in ops if a not in done)
                kills = sum(1 for a in ops if remc[a] == 1)
                born = 0 if remc[n] == 0 else 1
                return (newloads + born - kills) + noise * rnd.random() + 1e-4 * pos[n]
            n = min(cands, key=score)
            for a in sorted(set(operands(n)), key=lambda a: pos[a]):
                if a not in done:
                    done.add(a); order.append(a)
                remc[a] -= 1
            done.add(n); order.append(n); left.discard(n)
        ml = max_live(net, order, outputs)
        if ml < best[0]:
            best = (ml, order)
    return best


def solve_signs(G, iters=200000, seed=0):
    rnd = random.Random(seed)
    nets = {'A': (G['na'], G['a_out']), 'B': (G['nb'], G['b_out']), 'C': (G['tn'], G['c_res'])}
    order = {k: Prog(*v).order for k, v in nets.items()}
    R = len(G['a_out'])
    sig = {}
    for k in 'ABC':
        for n in order[k]:
            sig[(k, n)] = 1
    fixed = set()
    for k in 'AB':
        for n in order[k]:
            if nets[k][0].nodes[n][0] == 'in':
                fixed.add((k, n))
    for o in G['c_res']:
        sig[('C', o[0])] = o[1]; fixed.add(('C', o[0]))
    cin = {}
    for n in order['C']:
        nd = G['tn'].nodes[n]
        if nd[0] == 'in':
            cin[nd[1]] = n; fixed.add(('C', n))
    def cin_sign(r):
        a, b = G['a_out'][r], G['b_out'][r]
        return (sig[('A', a[0])] * a[1]) * (sig[('B', b[0])] * b[1])
    outmap = {}
    for r in range(R):
        outmap.setdefault(('A', G['a_out'][r][0]), []).append(r)
        outmap.setdefault(('B', G['b_out'][r][0]), []).append(r)
    def refresh():
        for r, n in cin.items():
            sig[('C', n)] = cin_sign(r)
    clauses = []
    for k in 'ABC':
        net = nets[k][0]
        for n in order[k]:
            nd = net.nodes[n]
            if nd[0] in ('add', 'sub'):
                clauses.append((k, n, nd[1], nd[2], 1 if nd[0] == 'add' else -1))
    occ = {}
    for ci, (k, n, a, b, cb) in enumerate(clauses):
        for v in (n, a, b):
            occ.setdefault((k, v), []).append(ci)
    def viol(ci):
        k, n, a, b, cb = clauses[ci]
        return sig[(k, n)] * sig[(k, a)] < 0 and sig[(k, n)] * cb * sig[(k, b)] < 0
    def flip(v):
        sig[v] = -sig[v]
        for r in outmap.get(v, []):
            if r in cin:
                sig[('C', cin[r])] = cin_sign(r)
    def affected(v):
        cs = set(occ.get(v, []))
        for r in outmap.get(v, []):
            if r in cin:
                cs.update(occ.get(('C', cin[r]), []))
        return cs
    flippers = {}
    for v, rs in outmap.items():
        for r in rs:
            if r in cin:
                flippers.setdefault(('C', cin[r]), []).append(v)
    refresh()
    bad = {ci for ci in range(len(clauses)) if viol(ci)}
    best = (len(bad), dict(sig))
    for it in range(iters):
        if not bad:
            break
        ci = rnd.choice(list(bad))
        k, n, a, b, cb = clauses[ci]
        cands = []
        for v in ((k, n), (k, a), (k, b)):
            if v in fixed:
                cands += flippers.get(v, [])
            else:
                cands.append(v)
        cands = [v for v in cands if v not in fixed]
        if not cands:
            continue
        def delta(v):
            cs = affected(v)
            before = sum(viol(c) for c in cs)
            flip(v)
            after = sum(viol(c) for c in cs)
            flip(v)
            return after - before
        if rnd.random() < 0.2:
            v = rnd.choice(cands)
        else:
            v = min(cands, key=lambda v: (delta(v), rnd.random()))
        cs = affected(v)
        flip(v)
        for c in cs:
            if viol(c): bad.add(c)
            else: bad.discard(c)
        if len(bad) < best[0]:
            best = (len(bad), dict(sig))
    nb, sg = best
    return ({n: s for (k, n), s in sg.items() if k == 'A'}, {n: s for (k, n), s in sg.items() if k == 'B'},
            {n: s for (k, n), s in sg.items() if k == 'C'}, nb)


class FixedProg:
    def __init__(self, net, outputs, sig, order=None):
        self.net, self.outputs, self.sig = net, outputs, sig
        self.order = order if order is not None else Prog(net, outputs).order
    def count(self):
        c = {'add': 0, 'sub': 0, 'mul': 0, 'in': 0}
        for n in self.order:
            c[self.net.nodes[n][0]] += 1
        return c


N, TAPS = 40, 16
G = build(N, TAPS, scale=False, variant=1)
HOP = G['hop']; R = len(G['a_out'])
T, D, K = 16000, 512, 31
L = (T - K) // 2 + 1
MB = 64; NCH = -(-L // (HOP * MB))
CH = HOP * MB
XM = CH + 16
LP = NCH * CH
TM = T // 2
LAST_M = TM - (NCH - 1) * CH
HS = 2.0 / N
T2 = 1; W3 = 1
U32, F32, BF16 = jnp.uint32, jnp.float32, jnp.bfloat16

bins = G['bins']
ev = [0, 1] + [2 + 3 * i + q for i, k in enumerate(bins) if k % 2 == 0 for q in range(3)]
od = [2 + 3 * i + q for i, k in enumerate(bins) if k % 2 == 1 for q in range(3)]
if (N // 2) % 2 == 1:
    ev.remove(1); od = [1] + od
IDX = (ev, od)
RH = (len(ev), len(od))
LOC = {}
for hf in range(2):
    for i, r in enumerate(IDX[hf]):
        LOC[r] = (hf, i)
SA, SB, SC, NBAD = solve_signs(G)
assert NBAD == 0
def mkprog(net, outs, sig):
    return FixedProg(net, outs, sig, order=min_live_order(net, outs, tries=100)[1])
PA = [mkprog(G['na'], [G['a_out'][r] for r in idx], SA) for idx in IDX]
PB = [mkprog(G['nb'], [G['b_out'][r] for r in idx], SB) for idx in IDX]
PC = mkprog(G['tn'], G['c_res'], SC)


def run_gen(prog, loads, sink):
    nsets = len(loads)
    vals = [dict() for _ in range(nsets)]
    sig = prog.sig
    outs = {}
    for r, o in enumerate(prog.outputs):
        outs.setdefault(o[0], []).append(r)
    for n in prog.order:
        k = prog.net.nodes[n]
        for s in range(nsets):
            v = vals[s]
            if k[0] == 'in':
                v[n] = loads[s](k[1])
            elif k[0] == 'mul':
                v[n] = v[k[1]] * (k[2] * sig[n] * sig[k[1]])
            else:
                a, b = k[1], k[2]
                cb = 1 if k[0] == 'add' else -1
                p, q = sig[n] * sig[a], sig[n] * cb * sig[b]
                if p > 0 and q > 0: v[n] = v[a] + v[b]
                elif p > 0: v[n] = v[a] - v[b]
                elif q > 0: v[n] = v[b] - v[a]
                else: v[n] = -(v[a] + v[b])
            yield 1
        for r in outs.get(n, []):
            yield from sink(r, [vals[s][n] for s in range(nsets)])


def drain(gen):
    for _ in gen:
        pass


def unpack(wd, hi):
    wd = (wd & jnp.uint32(0xffff0000)) if hi else (wd << 16)
    return lax.bitcast_convert_type(wd, F32)


def pack(lo, hi):
    return pltpu.pack_elementwise([lo, hi], packed_dtype=BF16)


def prog_weight(prog, nsets, per_out):
    return len(prog.order) * nsets + len(prog.outputs) * per_out


def interleave(mms, gens_weights):
    total = sum(w for _, w in gens_weights)
    def allops():
        for g, _ in gens_weights:
            yield from g
    gen = allops()
    e = 0; done = False
    for i, mm in enumerate(mms):
        mm()
        tgt = (i + 1) * total // len(mms)
        while not done and e < tgt:
            try:
                e += next(gen)
            except StopIteration:
                done = True
    for _ in gen:
        pass


def merge(lists):
    lists = [l for l in lists if l]
    out = []
    pos = [0] * len(lists)
    tot = sum(len(l) for l in lists)
    for _ in range(tot):
        i = min((i for i in range(len(lists)) if pos[i] < len(lists[i])), key=lambda i: (pos[i] + 0.5) / len(lists[i]))
        out.append(lists[i][pos[i]]); pos[i] += 1
    return out


C0 = math.sqrt(2.0 / math.pi)
def gelu_half(zh):
    u = zh * (zh * zh * (8.0 * C0 * 0.044715) + 2.0 * C0)
    return zh * jnp.tanh(u) + zh


def kernel(x_hbm, w_hbm, gam_ref, bet_ref, out_hbm,
           xb0, xb1, xb2, xb3, we, wo, xe, xo, ye, yo, h0, h1, h2, h3, st, nrm, gsm, xsem, wsem, osem):
    xb = (xb0, xb1, xb2, xb3)
    wh = (we, wo); xh = (xe, xo); yy = (ye, yo)
    hh = (h0, h1, h2, h3)
    x32 = x_hbm.bitcast(U32)
    w32 = w_hbm.bitcast(F32)
    o32 = out_hbm.bitcast(F32)
    LASTJ = 2 * NCH - 1

    def x_copy(j, c, full):
        b = j // NCH
        cj = j % NCH
        rows = XM if full else LAST_M
        return pltpu.make_async_copy(
            x32.at[b, pl.ds(pl.multiple_of(cj * CH, 8), rows), pl.ds(c * 128, 128)],
            xb[c].at[pl.ds(0, rows), :], xsem.at[c])

    def x_start(j):
        cj = j % NCH
        @pl.when(cj < NCH - 1)
        def _():
            for c in range(4):
                x_copy(j, c, True).start()
        @pl.when(cj == NCH - 1)
        def _():
            for c in range(4):
                x_copy(j, c, False).start()
                xb[c][pl.ds(LAST_M, XM - LAST_M), :] = jnp.zeros((XM - LAST_M, 128), U32)

    def x_wait(j, cs=range(4)):
        cj = j % NCH
        @pl.when(cj < NCH - 1)
        def _():
            for c in cs:
                x_copy(j, c, True).wait()
        @pl.when(cj == NCH - 1)
        def _():
            for c in cs:
                x_copy(j, c, False).wait()

    WQ = 4
    def w_copy(n, q):
        dst = hh[n].at[1, pl.ds(0, K * 256), :].reshape(K, 256, 128)
        r = 256 // WQ
        return pltpu.make_async_copy(w32.at[:, pl.ds(q * r, r), pl.ds(n * 128, 128)], dst.at[:, pl.ds(q * r, r), :], wsem.at[n, q])

    def o_copy(n, r0, rows, k):
        return pltpu.make_async_copy(hh[n].at[0, pl.ds(r0, rows), :], o32.at[pl.ds(r0, rows), n, 0, :], osem.at[n, k])

    def a_piece(g, c, p, half):
        dyn = not isinstance(g, int)
        base = pl.multiple_of(g * (16 * HOP), 8) if dyn else g * (16 * HOP)
        row = pl.multiple_of(g * 8, 8) if dyn else g * 8
        xw = xb[c].at[pl.ds(base, 16 * HOP + 16), :]
        def mkload(o):
            return lambda t: unpack(xw[pl.ds(t + o * HOP, 8, stride=2 * HOP), :], p)
        def sink(i, vs):
            xh[half][i, pl.ds(row, 8), p * 512 + c * 128:p * 512 + (c + 1) * 128] = pack(vs[0], vs[1])
            yield 1
        return run_gen(PA[half], [mkload(0), mkload(1)], sink), prog_weight(PA[half], 2, 1)

    def a_pieces(half):
        return [a_piece(g, c, p, half) for c in range(4) for g in range(MB // 16) for p in range(2)]

    def w_piece(n, g, p, half):
        dyn = not isinstance(g, int)
        row = pl.multiple_of(g * 8, 8) if dyn else g * 8
        cache = {}
        def word(j):
            if j not in cache:
                cache[j] = lax.bitcast_convert_type(hh[n][1, pl.ds((2 * j + p) * 256 + row, 8), :], U32)
            return cache[j]
        def mkload(hi):
            def load(j):
                if 2 * j + p >= K:
                    return jnp.zeros((8, 128), F32)
                return unpack(word(j), hi)
            return load
        def sink(i, vs):
            wh[half][n, i, pl.ds(p * 256 + row, 8), :] = pack(vs[0], vs[1])
            yield 1
        return run_gen(PB[half], [mkload(0), mkload(1)], sink), prog_weight(PB[half], 2, 1)

    def c_pieces(j, n):
        if isinstance(j, int):
            b, cj = j // NCH, j % NCH
            slot = b
        else:
            valid = j >= 0
            b = jnp.where(valid, j // NCH, 0)
            cj = jnp.where(valid, j % NCH, NCH - 1)
            slot = jnp.where(valid, b, 2)
        state = {}
        def col(g):
            if g == 0:
                state['c'] = st[slot, n, 2]; state['a1'] = st[slot, n, 0]; state['a2'] = st[slot, n, 1]
            base = cj * CH + g * (8 * HOP)
            if not isinstance(j, int):
                base = pl.multiple_of(base, 8)
            hs = hh[n].at[b, pl.ds(base, 8 * HOP), :]
            def sink(t, vs):
                hs[pl.ds(t, 8, stride=HOP), :] = vs[0]
                d = vs[0] - state['c']
                state['a1'] = state['a1'] + d
                state['a2'] = state['a2'] + d * d
                yield 4
            yield from run_gen(PC, [lambda r: yy[LOC[r][0]][n, LOC[r][1], g * 8:(g + 1) * 8, :]], sink)
            if g == MB // 8 - 1:
                st[slot, n, 0] = state['a1']; st[slot, n, 1] = state['a2']
        return [(col(g), prog_weight(PC, 1, 4)) for g in range(MB // 8)]

    def set_shift(j, n):
        @pl.when(jnp.logical_and(j >= 0, j % NCH == 0))
        def _():
            st[j // NCH, n, 2] = jnp.broadcast_to(ye[n, LOC[0][1], 0:1, :], (8, 128))

    def finalize_stats(n):
        sub = lax.broadcasted_iota(jnp.int32, (8, 128), 0)
        for b in range(2):
            c = st[b, n, 2]
            r0 = (L // 8) * 8
            c1 = jnp.zeros((8, 128), F32); c2 = jnp.zeros((8, 128), F32)
            for r in range(r0, LP, 8):
                d = hh[n][b, r:r + 8, :] - c
                if r < L:
                    d = jnp.where(sub >= L - r, d, 0.0)
                c1 = c1 + d; c2 = c2 + d * d
            s1 = jnp.sum(st[b, n, 0] - c1, axis=0, keepdims=True)
            s2 = jnp.sum(st[b, n, 1] - c2, axis=0, keepdims=True)
            md = s1 * (1.0 / L)
            var = (s2 * (1.0 / L) - md * md) * (HS * HS)
            mu = c[0:1] + md
            a = (HS * lax.rsqrt(var + 1e-5)) * gam_ref[...].astype(F32).reshape(1, D)[:, n * 128:(n + 1) * 128]
            bb = bet_ref[...].astype(F32).reshape(1, D)[:, n * 128:(n + 1) * 128] - mu * a
            nrm[n, b, 0] = jnp.broadcast_to(0.5 * a, (8, 128))
            nrm[n, b, 1] = jnp.broadcast_to(0.5 * bb, (8, 128))

    def d_vreg(n, r, cs):
        a0, b0, a1, b1 = cs
        z0 = gelu_half(hh[n][0, pl.ds(r, 8), :] * a0 + b0)
        z1 = gelu_half(hh[n][1, pl.ds(r, 8), :] * a1 + b1)
        hh[n][0, pl.ds(r, 8), :] = lax.bitcast_convert_type(pack(z0, z1), F32)

    def d_consts(n):
        return nrm[n, 0, 0], nrm[n, 0, 1], nrm[n, 1, 0], nrm[n, 1, 1]

    def d_pieces(n, ra=0, rb=LP):
        state = {}
        def piece(r0, r1):
            if 'cs' not in state:
                state['cs'] = d_consts(n)
            for r in range(r0, r1, 8):
                d_vreg(n, r, state['cs'])
                yield 19
        P = 200
        return [(piece(r, min(r + P, rb)), 19 * (min(r + P, rb) - r) // 8) for r in range(ra, rb, P)]

    def fin_piece(n):
        def gen():
            finalize_stats(n)
            yield 100
        return [(gen(), 100)]

    NPC = 4
    PR = -(-(-(-L // NPC)) // 8) * 8
    def d_loop(n, k0):
        cs = d_consts(n)
        UN = 5
        for k in range(k0, NPC):
            r0 = k * PR; r1 = min(r0 + PR, LP)
            nv = -(-(r1 - r0) // 8)
            assert nv % UN == 0, nv
            def body(i, carry):
                for u in range(UN):
                    d_vreg(n, pl.multiple_of(r0 + (i * UN + u) * 8, 8), cs)
                return carry
            lax.fori_loop(0, nv // UN, body, 0)
            o_copy(n, r0, min(r0 + PR, L) - r0, k).start()

    def o_start_all(n):
        for k in range(NPC):
            r0 = k * PR
            o_copy(n, r0, min(r0 + PR, L) - r0, k).start()

    def o_wait_all(n):
        for k in range(NPC):
            r0 = k * PR
            o_copy(n, r0, min(r0 + PR, L) - r0, k).wait()

    def mm(half, n, i):
        def f():
            lhs = pltpu.bitcast(xh[half][i], BF16)
            rhs = pltpu.bitcast(wh[half][n, i], BF16)
            yy[half][n, i] = jnp.dot(lhs, rhs, preferred_element_type=F32)
        return f

    def body(name, half, tiles, lists, sl=None):
        mms = [mm(half, n, i) for n in tiles for i in range(RH[half])]
        if sl is not None:
            mms = mms[sl]
        with jax.named_scope(name):
            interleave(mms, merge(lists))

    j0 = jnp.int32(0)
    for k_ in range(32):
        gsm[k_] = jnp.int32(0)
    x_start(j0)
    for q in range(WQ):
        w_copy(0, q).start()
    st[...] = jnp.zeros_like(st)

    with jax.named_scope("a0"):
        for c in range(4):
            x_wait(j0, [c])
            def a0(g, carry):
                for p in range(2):
                    drain(a_piece(g, c, p, 0)[0])
                return carry
            lax.fori_loop(0, MB // 16, a0, 0)
        for n in range(1, 4):
            for q in range(WQ):
                w_copy(n, q).start()

    with jax.named_scope("wstage"):
        GP = 32 // WQ
        for n in range(4):
            phases = (1,) if (n == 3 and W3) else (0, 1)
            def wl(g, carry):
                for p in phases:
                    for half in range(2):
                        drain(w_piece(n, g, p, half)[0])
                return carry
            def wq(q, carry):
                w_copy(n, q).wait()
                lax.fori_loop(q * GP, (q + 1) * GP, wl, 0)
                return carry
            lax.fori_loop(0, WQ, wq, 0)

    def main(j, carry):
        @pl.when(j >= 0)
        def _():
            body("E01", 0, (0, 1), [a_pieces(1)])
        @pl.when(j + 1 <= LASTJ)
        def _():
            x_start(j + 1)
        set_shift(j - 1, 2); set_shift(j - 1, 3)
        if W3:
            @pl.when(j == 0)
            def _():
                body("O01W", 1, (0, 1), [[w_piece(3, g, 0, half) for g in range(32) for half in range(2)]])
        @pl.when(j + 1 >= (2 if W3 else 1))
        def _():
            body("O01", 1, (0, 1), [c_pieces(j - 1, 2), c_pieces(j - 1, 3)])
        @pl.when(j < (LASTJ if T2 else LASTJ + 1))
        def _():
            set_shift(j, 0); set_shift(j, 1)
        @pl.when(j + 2 < (LASTJ if T2 else LASTJ + 1) + 2)
        def _():
            body("E23", 0, (2, 3), [c_pieces(j, 0), c_pieces(j, 1)])
        @pl.when(j + 1 <= LASTJ)
        def _():
            x_wait(j + 1)
        @pl.when(j < (LASTJ if T2 else LASTJ + 1))
        def _():
            body("O23", 1, (2, 3), [a_pieces(0)])
        return carry
    lax.fori_loop(0, LASTJ + 1, main, 0)

    jl = jnp.int32(LASTJ)
    if T2:
        gd = gsm[0]
        set_shift(jl, 0); set_shift(jl, 1)
        def o_start(n, ks):
            for k in ks:
                r0 = k * PR
                o_copy(n, r0, min(r0 + PR, L) - r0, k).start()
        def dq(n, k):
            return d_pieces(n, k * PR, min((k + 1) * PR, LP))
        allmm = [(0, 2, i) for i in range(RH[0])] + [(0, 3, i) for i in range(RH[0])] + \
                [(1, 2, i) for i in range(RH[1])] + [(1, 3, i) for i in range(RH[1])]
        no3 = len(allmm) - RH[1]
        cuts = [0, 8, 18, 28, 38, 52, 64, 76, no3, len(allmm)]
        plan = [
            (c_pieces(LASTJ, 0) + fin_piece(0) + dq(0, 0), [(0, 0)]),
            (dq(0, 1), [(0, 1)]),
            (dq(0, 2), [(0, 2)]),
            (dq(0, 3), [(0, 3)]),
            (c_pieces(LASTJ, 1) + fin_piece(1) + dq(1, 0), [(1, 0)]),
            (dq(1, 1), [(1, 1)]),
            (dq(1, 2), [(1, 2)]),
            (dq(1, 3), [(1, 3)]),
            (c_pieces(LASTJ, 2) + fin_piece(2) + dq(2, 0) + dq(2, 1), [(2, 0), (2, 1)]),
        ]
        set_shift(jl, 2)
        for bi, (pcs, starts) in enumerate(plan):
            @pl.when(gsm[16 + bi] >= 0)
            def _():
                with jax.named_scope("D%d" % bi):
                    interleave([mm(*t) for t in allmm[cuts[bi]:cuts[bi + 1]]], pcs)
            for n_, k_ in starts:
                o_start(n_, (k_,))

    with jax.named_scope("tail"):
        set_shift(jl, 3)
        d_loop(2, 2)
        for g_, _ in c_pieces(LASTJ, 3):
            drain(g_)
        finalize_stats(3)
        d_loop(3, 0)
        for n in range(4):
            o_wait_all(n)


@jax.jit
def pallas_standalone__self_sup_conv_stem_wavlm__speech_kernel(x, w, gn_gamma, gn_beta):
    out = pl.pallas_call(
        kernel,
        in_specs=[pl.BlockSpec(memory_space=pl.ANY), pl.BlockSpec(memory_space=pl.ANY),
                  pl.BlockSpec(memory_space=pltpu.VMEM), pl.BlockSpec(memory_space=pltpu.VMEM)],
        out_specs=pl.BlockSpec(memory_space=pl.ANY),
        out_shape=jax.ShapeDtypeStruct((L, 4, 2, 128), BF16),
        scratch_shapes=[pltpu.VMEM((XM, 128), U32)] * 4 + [
            pltpu.VMEM((4, RH[0], 512, 128), U32),
            pltpu.VMEM((4, RH[1], 512, 128), U32),
            pltpu.VMEM((RH[0], MB // 2, 1024), U32),
            pltpu.VMEM((RH[1], MB // 2, 1024), U32),
            pltpu.VMEM((4, RH[0], MB, 128), F32),
            pltpu.VMEM((4, RH[1], MB, 128), F32)] + [pltpu.VMEM((2, LP, 128), F32)] * 4 + [
            pltpu.VMEM((3, 4, 3, 8, 128), F32),
            pltpu.VMEM((4, 2, 2, 8, 128), F32),
            pltpu.SMEM((32,), jnp.int32),
            pltpu.SemaphoreType.DMA((4,)),
            pltpu.SemaphoreType.DMA((4, 4)),
            pltpu.SemaphoreType.DMA((4, 4)),
        ],
        compiler_params=pltpu.CompilerParams(vmem_limit_bytes=127 * 1024 * 1024),
    )(x, w, gn_gamma, gn_beta)
    return out.transpose(2, 0, 1, 3).reshape(2, L, D)
```

```python
import math
import random
import numpy as np
import jax, jax.numpy as jnp
from jax import lax
from jax.experimental import pallas as pl
from jax.experimental.pallas import tpu as pltpu


class Net:
    def __init__(self):
        self.nodes = []
        self.cse = {}

    def _mk(self, key):
        if key in self.cse:
            return self.cse[key]
        self.nodes.append(key)
        self.cse[key] = len(self.nodes) - 1
        return self.cse[key]

    def inp(self, i):
        return (self._mk(('in', i)), 1)

    def neg(self, x):
        return None if x is None else (x[0], -x[1])

    def add(self, x, y):
        if x is None:
            return y
        if y is None:
            return x
        (a, sa), (b, sb) = x, y
        if a == b:
            if sa == sb:
                return self.mul(x, 2.0)
            return None
        if sa == sb:
            if a > b:
                a, b = b, a
            return (self._mk(('add', a, b)), sa)
        if a > b:
            a, b, sa = b, a, sb
        return (self._mk(('sub', a, b)), sa)

    def sub(self, x, y):
        return self.add(x, self.neg(y))

    def mul(self, x, c):
        if x is None or abs(c) < 1e-12:
            return None
        a, s = x
        if c < 0:
            c, s = -c, -s
        if abs(c - 1.0) < 1e-12:
            return (a, s)
        c = float(np.float64(round(c, 14)))
        return (self._mk(('mul', a, c)), s)

    def cadd(self, x, y):
        return (self.add(x[0], y[0]), self.add(x[1], y[1]))

    def csub(self, x, y):
        return (self.sub(x[0], y[0]), self.sub(x[1], y[1]))

    def cmulc(self, x, c, s):
        a, b = x
        if abs(s) < 1e-12:
            return (self.mul(a, c), self.mul(b, c))
        if abs(c) < 1e-12:
            return (self.mul(b, -s), self.mul(a, s))
        if abs(abs(c) - abs(s)) < 1e-12:
            sg = 1.0 if s * c > 0 else -1.0
            re = self.sub(a, self.mul(b, sg))
            im = self.add(b, self.mul(a, sg))
            return (self.mul(re, c), self.mul(im, c))
        re = self.sub(self.mul(a, c), self.mul(b, s))
        im = self.add(self.mul(a, s), self.mul(b, c))
        return (re, im)


def w(k, n):
    ang = -2.0 * math.pi * (k % n) / n
    return math.cos(ang), math.sin(ang)


def cfft(net, z):
    n = len(z)
    if n == 1:
        return [z[0]]
    if n == 2:
        return [net.cadd(z[0], z[1]), net.csub(z[0], z[1])]
    if n % 4 == 0:
        h, q = n // 2, n // 4
        e = [net.cadd(z[t], z[t + h]) for t in range(h)]
        o = [net.csub(z[t], z[t + h]) for t in range(h)]
        z1, z3 = [], []
        for t in range(q):
            a, b = o[t], o[t + q]
            mib = (b[1], net.neg(b[0]))
            p = net.cadd(a, mib)
            m = net.csub(a, mib)
            z1.append(net.cmulc(p, *w(t, n)))
            z3.append(net.cmulc(m, *w(3 * t, n)))
        E = cfft(net, e)
        Z1 = cfft(net, z1)
        Z3 = cfft(net, z3)
        out = [None] * n
        for k in range(h):
            out[2 * k] = E[k]
        for k in range(q):
            out[4 * k + 1] = Z1[k]
            out[4 * k + 3] = Z3[k]
        return out
    if n % 2 == 0:
        m = n // 2
        out = [None] * n
        rows = []
        for t2 in range(m):
            a = z[(2 * t2) % n]
            b = z[(m + 2 * t2) % n]
            rows.append((net.cadd(a, b), net.csub(a, b)))
        for k1 in range(2):
            Z = cfft(net, [rows[t2][k1] for t2 in range(m)])
            for k2 in range(m):
                for k in range(n):
                    if k % 2 == k1 and k % m == k2:
                        out[k] = Z[k2]
        return out
    if n % 3 == 0 and n > 3:
        raise NotImplementedError
    out = []
    p = {t: net.cadd(z[t], z[n - t]) for t in range(1, (n + 1) // 2)}
    q = {t: net.csub(z[t], z[n - t]) for t in range(1, (n + 1) // 2)}
    s = z[0]
    for t in p:
        s = net.cadd(s, p[t])
    out = [None] * n
    out[0] = s
    for k in range(1, (n + 1) // 2):
        A = z[0]
        B = (None, None)
        for t in p:
            c, sn = w(k * t, n)
            A = net.cadd(A, (net.mul(p[t][0], c), net.mul(p[t][1], c)))
            B = net.cadd(B, (net.mul(q[t][1], -sn), net.mul(q[t][0], sn)))
        out[k] = net.cadd(A, B)
        out[n - k] = net.csub(A, B)
    return out


def cfft_pfa(net, z, n1, n2):
    n = n1 * n2
    out = [None] * n
    cols = [cfft_any(net, [z[(n2 * t1 + n1 * t2) % n] for t2 in range(n2)]) for t1 in range(n1)]
    for k2 in range(n2):
        Z = cfft_any(net, [cols[t1][k2] for t1 in range(n1)])
        for k1 in range(n1):
            for k in range(n):
                if k % n1 == k1 and k % n2 == k2:
                    out[k] = Z[k1]
    return out


def cfft5(net, z):
    c1, c2 = math.cos(2 * math.pi / 5), math.cos(4 * math.pi / 5)
    s1, s2 = math.sin(2 * math.pi / 5), math.sin(4 * math.pi / 5)
    t1 = net.cadd(z[1], z[4]); t2 = net.cadd(z[2], z[3])
    t3 = net.csub(z[1], z[4]); t4 = net.csub(z[2], z[3])
    t5 = net.cadd(t1, t2)
    def rm(x, c):
        return (net.mul(x[0], c), net.mul(x[1], c))
    m1 = rm(t5, (c1 + c2) / 2 - 1.0)
    m2 = rm(net.csub(t1, t2), (c1 - c2) / 2)
    y0 = net.cadd(z[0], t5)
    a = net.cadd(y0, m1)
    a1 = net.cadd(a, m2); a2 = net.csub(a, m2)
    m3 = rm(net.cadd(t3, t4), s2)
    m4 = rm(t3, s1 - s2)
    m5 = rm(t4, s1 + s2)
    b1 = net.cadd(m3, m4)
    b2 = net.csub(m3, m5)
    def mi(x):
        return (x[1], net.neg(x[0]))
    return [y0, net.cadd(a1, mi(b1)), net.cadd(a2, mi(b2)), net.csub(a2, mi(b2)), net.csub(a1, mi(b1))]


def rfft5(net, x):
    c1, c2 = math.cos(2 * math.pi / 5), math.cos(4 * math.pi / 5)
    s1, s2 = math.sin(2 * math.pi / 5), math.sin(4 * math.pi / 5)
    t1 = net.add(x[1], x[4]); t2 = net.add(x[2], x[3])
    t3 = net.sub(x[1], x[4]); t4 = net.sub(x[2], x[3])
    t5 = net.add(t1, t2)
    m1 = net.mul(t5, (c1 + c2) / 2 - 1.0)
    m2 = net.mul(net.sub(t1, t2), (c1 - c2) / 2)
    y0 = net.add(x[0], t5)
    a = net.add(y0, m1)
    a1 = net.add(a, m2); a2 = net.sub(a, m2)
    m3 = net.mul(net.add(t3, t4), s2)
    m4 = net.mul(t3, s1 - s2)
    m5 = net.mul(t4, s1 + s2)
    b1 = net.add(m3, m4); b2 = net.sub(m3, m5)
    return [(y0, None), (a1, net.neg(b1)), (a2, net.neg(b2))]


def cfft_any(net, z):
    n = len(z)
    if n == 5:
        return cfft5(net, z)
    if n == 12:
        return cfft_pfa(net, z, 3, 4)
    if n == 10:
        return cfft_pfa(net, z, 5, 2)
    if n == 20:
        return cfft_pfa(net, z, 5, 4)
    if n == 6:
        return cfft_pfa(net, z, 3, 2)
    if n == 14:
        return cfft_pfa(net, z, 7, 2)
    if n == 15:
        return cfft_pfa(net, z, 5, 3)
    return cfft(net, z)


def rfft_pfa(net, x, n1, n2):
    n = n1 * n2
    inner = [rfft(net, [x[(n2 * t1 + n1 * t2) % n] for t1 in range(n1)]) for t2 in range(n2)]
    out = [None] * (n // 2 + 1)
    for k1 in range(n1 // 2 + 1):
        col = [inner[t2][k1] for t2 in range(n2)]
        if all(c[1] is None for c in col):
            Z = rfft(net, [c[0] for c in col])
            Z = Z + [(Z[n2 - k2][0], net.neg(Z[n2 - k2][1])) for k2 in range(len(Z), n2)]
        else:
            Z = cfft_any(net, col)
        for k2 in range(n2):
            k = [k for k in range(n) if k % n1 == k1 and k % n2 == k2][0]
            if k <= n // 2:
                if out[k] is None:
                    out[k] = Z[k2]
            else:
                if out[n - k] is None:
                    out[n - k] = (Z[k2][0], net.neg(Z[k2][1]))
    return out


PFA = {40: (8, 5), 20: (4, 5), 24: (8, 3), 48: (16, 3), 12: (4, 3), 56: (8, 7), 10: (2, 5), 6: (2, 3), 60: (4, 15), 15: (3, 5), 44: (4, 11), 36: (4, 9)}
USE_PFA = True


def rfft(net, x):
    n = len(x)
    if USE_PFA and n in PFA:
        return rfft_pfa(net, x, *PFA[n])
    if n == 1:
        return [(x[0], None)]
    if n == 2:
        return [(net.add(x[0], x[1]), None), (net.sub(x[0], x[1]), None)]
    if n % 4 == 0:
        h, q = n // 2, n // 4
        e = [net.add(x[t], x[t + h]) for t in range(h)]
        o = [net.sub(x[t], x[t + h]) for t in range(h)]
        z = [net.cmulc((o[t], net.neg(o[t + q])), *w(t, n)) for t in range(q)]
        E = rfft(net, e)
        Z = cfft_any(net, z)
        out = [None] * (h + 1)
        for k in range(len(E)):
            out[2 * k] = E[k]
        for k in range(q):
            f = 4 * k + 1
            if f <= h:
                out[f] = Z[k]
            else:
                out[n - f] = (Z[k][0], net.neg(Z[k][1]))
        return out
    if n % 2 == 0:
        m = n // 2
        e = [net.add(x[t], x[t + m]) for t in range(m)]
        o = [net.sub(x[t], x[t + m]) for t in range(m)]
        E = rfft(net, e)
        op = [o[t] if t % 2 == 0 else net.neg(o[t]) for t in range(m)]
        O = rfft(net, op)
        out = [None] * (m + 1)
        for k in range(len(E)):
            out[2 * k] = E[k]
        for f in range(1, m + 1, 2):
            j = ((f - m) // 2) % m
            if j <= m // 2:
                out[f] = O[j]
            else:
                out[f] = (O[m - j][0], net.neg(O[m - j][1]))
        return out
    if n == 5:
        return rfft5(net, x)
    p = {t: net.add(x[t], x[n - t]) for t in range(1, (n + 1) // 2)}
    q = {t: net.sub(x[t], x[n - t]) for t in range(1, (n + 1) // 2)}
    s = x[0]
    for t in p:
        s = net.add(s, p[t])
    out = [(s, None)]
    for k in range(1, (n + 1) // 2):
        A = x[0]
        B = None
        for t in p:
            c, sn = w(k * t, n)
            A = net.add(A, net.mul(p[t], c))
            B = net.add(B, net.mul(q[t], sn))
        out.append((A, B))
    return out


class Prog:
    def __init__(self, net, outputs):
        order = []
        seen = set()

        def visit(n):
            if n in seen:
                return
            seen.add(n)
            k = net.nodes[n]
            if k[0] in ('add', 'sub'):
                visit(k[1]); visit(k[2])
            elif k[0] == 'mul':
                visit(k[1])
            order.append(n)
        for o in outputs:
            if o is not None:
                visit(o[0])
        self.net = net
        self.order = order
        self.outputs = outputs

    def count(self):
        c = {'add': 0, 'sub': 0, 'mul': 0, 'in': 0}
        for n in self.order:
            c[self.net.nodes[n][0]] += 1
        return c

    def run(self, load, emit=None):
        vals = {}
        for n in self.order:
            k = self.net.nodes[n]
            if k[0] == 'in':
                vals[n] = load(k[1])
            elif k[0] == 'add':
                vals[n] = vals[k[1]] + vals[k[2]]
            elif k[0] == 'sub':
                vals[n] = vals[k[1]] - vals[k[2]]
            else:
                vals[n] = vals[k[1]] * k[2]
        return [None if o is None else vals[o[0]] for o in self.outputs]

    @property
    def signs(self):
        return [0 if o is None else o[1] for o in self.outputs]

    def matrix(self, n_in, signed=True):
        eye = np.eye(n_in)
        res = self.run(lambda i: eye[i])
        rows = []
        for r, s in zip(res, self.signs):
            rows.append(np.zeros(n_in) if r is None else (r * s if signed else r))
        return np.stack(rows)


def transpose(net, outputs, wanted_inputs):
    prog = Prog(net, outputs)
    live = set(prog.order)
    consumers = {n: [] for n in prog.order}
    for n in prog.order:
        k = net.nodes[n]
        if k[0] == 'add':
            consumers[k[1]].append((n, 1.0)); consumers[k[2]].append((n, 1.0))
        elif k[0] == 'sub':
            consumers[k[1]].append((n, 1.0)); consumers[k[2]].append((n, -1.0))
        elif k[0] == 'mul':
            consumers[k[1]].append((n, k[2]))
    outmap = {}
    for r, o in enumerate(outputs):
        if o is not None:
            outmap.setdefault(o[0], []).append((r, o[1]))
    tn = Net()
    memo = {}

    def adj(n):
        if n in memo:
            return memo[n]
        acc = None
        for r, s in outmap.get(n, []):
            v = tn.inp(r)
            acc = tn.add(acc, v if s > 0 else tn.neg(v))
        for c, coef in consumers[n]:
            acc = tn.add(acc, tn.mul(adj(c), coef))
        memo[n] = acc
        return acc
    outs = []
    for i in wanted_inputs:
        key = ('in', i)
        if key in net.cse and net.cse[key] in live:
            outs.append(adj(net.cse[key]))
        else:
            outs.append(None)
    return tn, outs


def build(N, taps, scale=True, variant=0):
    hop = N - taps + 1
    na = Net()
    U = rfft(na, [na.inp(t) for t in range(N)])
    a_out = [U[0][0], U[N // 2][0]]
    bins = list(range(1, N // 2))
    for k in bins:
        a, b = U[k]
        if variant == 0:
            a_out += [na.add(a, b), a, b]
        else:
            a_out += [a, na.sub(b, a), na.add(a, b)]
    nc = Net()
    V = rfft(nc, [nc.inp(t) for t in range(N)])
    c_out = [V[0][0], V[N // 2][0]]
    for k in bins:
        al, be = V[k]
        c_out += [nc.add(al, be), be, nc.neg(al)]
    tn, c_res = transpose(nc, c_out, list(range(hop)))
    def mkb(ntaps):
        nb = Net()
        Wf = rfft(nb, [nb.inp(t) if t < ntaps else None for t in range(N)])
        s0 = 1.0 / N if scale else 0.5
        b_out = [nb.mul(Wf[0][0], s0), nb.mul(Wf[N // 2][0], s0)]
        for k in bins:
            c = Wf[k][0]
            d = nb.neg(Wf[k][1])
            sc = 2.0 / N if scale else 1.0
            if variant == 0:
                b_out += [nb.mul(c, sc), nb.mul(nb.sub(d, c), sc), nb.mul(nb.add(c, d), sc)]
            else:
                b_out += [nb.mul(nb.add(c, d), sc), nb.mul(c, sc), nb.mul(d, sc)]
        return nb, b_out
    nb, b_out = mkb(taps)
    nb1, b1_out = mkb(taps - 1)
    return dict(N=N, hop=hop, taps=taps, na=na, a_out=a_out, nb=nb, b_out=b_out, nb1=nb1, b1_out=b1_out,
                tn=tn, c_res=c_res, bins=bins)


def max_live(net, order, outputs, out_at_once=True):
    uses = {n: 0 for n in order}
    for n in order:
        k = net.nodes[n]
        for a in ([k[1], k[2]] if k[0] in ('add', 'sub') else [k[1]] if k[0] == 'mul' else []):
            uses[a] += 1
    live = set(); peak = 0; tot = 0
    rem = dict(uses)
    for n in order:
        k = net.nodes[n]
        live.add(n)
        peak = max(peak, len(live))
        for a in set([k[1], k[2]] if k[0] in ('add', 'sub') else [k[1]] if k[0] == 'mul' else []):
            rem[a] -= (1 if k[0] == 'mul' or k[1] != k[2] else 2)
            if rem[a] == 0:
                live.discard(a)
        if rem[n] == 0:
            live.discard(n)
        tot += len(live)
    return peak, tot / len(order)


def min_live_order(net, outputs, seed=0, tries=200):
    base = Prog(net, outputs).order
    nodes = set(base)
    def operands(n):
        k = net.nodes[n]
        return [k[1], k[2]] if k[0] in ('add', 'sub') else [k[1]] if k[0] == 'mul' else []
    consumers = {n: [] for n in base}
    for n in base:
        for a in set(operands(n)):
            consumers[a].append(n)
    best = (max_live(net, base, outputs), base)
    rnd = random.Random(seed)
    pos = {n: i for i, n in enumerate(base)}
    for it in range(tries):
        done = set(); order = []
        live = set()
        remc = {n: len(consumers[n]) for n in base}
        isin = {n: net.nodes[n][0] == 'in' for n in base}
        def ready(n):
            return n not in done and not isin[n] and all((a in done) or isin[a] for a in operands(n))
        noise = rnd.random() * 1.5
        work = [n for n in base if not isin[n]]
        left = set(work)
        while left:
            cands = [n for n in left if ready(n)]
            def score(n):
                ops = set(operands(n))
                newloads = sum(1 for a in ops if a not in done)
                kills = sum(1 for a in ops if remc[a] == 1)
                born = 0 if remc[n] == 0 else 1
                return (newloads + born - kills) + noise * rnd.random() + 1e-4 * pos[n]
            n = min(cands, key=score)
            for a in sorted(set(operands(n)), key=lambda a: pos[a]):
                if a not in done:
                    done.add(a); order.append(a)
                remc[a] -= 1
            done.add(n); order.append(n); left.discard(n)
        ml = max_live(net, order, outputs)
        if ml < best[0]:
            best = (ml, order)
    return best


def solve_signs(G, iters=200000, seed=0):
    rnd = random.Random(seed)
    nets = {'A': (G['na'], G['a_out']), 'B': (G['nb'], G['b_out']), 'C': (G['tn'], G['c_res'])}
    order = {k: Prog(*v).order for k, v in nets.items()}
    R = len(G['a_out'])
    sig = {}
    for k in 'ABC':
        for n in order[k]:
            sig[(k, n)] = 1
    fixed = set()
    for k in 'AB':
        for n in order[k]:
            if nets[k][0].nodes[n][0] == 'in':
                fixed.add((k, n))
    for o in G['c_res']:
        sig[('C', o[0])] = o[1]; fixed.add(('C', o[0]))
    cin = {}
    for n in order['C']:
        nd = G['tn'].nodes[n]
        if nd[0] == 'in':
            cin[nd[1]] = n; fixed.add(('C', n))
    def cin_sign(r):
        a, b = G['a_out'][r], G['b_out'][r]
        return (sig[('A', a[0])] * a[1]) * (sig[('B', b[0])] * b[1])
    outmap = {}
    for r in range(R):
        outmap.setdefault(('A', G['a_out'][r][0]), []).append(r)
        outmap.setdefault(('B', G['b_out'][r][0]), []).append(r)
    def refresh():
        for r, n in cin.items():
            sig[('C', n)] = cin_sign(r)
    clauses = []
    for k in 'ABC':
        net = nets[k][0]
        for n in order[k]:
            nd = net.nodes[n]
            if nd[0] in ('add', 'sub'):
                clauses.append((k, n, nd[1], nd[2], 1 if nd[0] == 'add' else -1))
    occ = {}
    for ci, (k, n, a, b, cb) in enumerate(clauses):
        for v in (n, a, b):
            occ.setdefault((k, v), []).append(ci)
    def viol(ci):
        k, n, a, b, cb = clauses[ci]
        return sig[(k, n)] * sig[(k, a)] < 0 and sig[(k, n)] * cb * sig[(k, b)] < 0
    def flip(v):
        sig[v] = -sig[v]
        for r in outmap.get(v, []):
            if r in cin:
                sig[('C', cin[r])] = cin_sign(r)
    def affected(v):
        cs = set(occ.get(v, []))
        for r in outmap.get(v, []):
            if r in cin:
                cs.update(occ.get(('C', cin[r]), []))
        return cs
    flippers = {}
    for v, rs in outmap.items():
        for r in rs:
            if r in cin:
                flippers.setdefault(('C', cin[r]), []).append(v)
    refresh()
    bad = {ci for ci in range(len(clauses)) if viol(ci)}
    best = (len(bad), dict(sig))
    for it in range(iters):
        if not bad:
            break
        ci = rnd.choice(list(bad))
        k, n, a, b, cb = clauses[ci]
        cands = []
        for v in ((k, n), (k, a), (k, b)):
            if v in fixed:
                cands += flippers.get(v, [])
            else:
                cands.append(v)
        cands = [v for v in cands if v not in fixed]
        if not cands:
            continue
        def delta(v):
            cs = affected(v)
            before = sum(viol(c) for c in cs)
            flip(v)
            after = sum(viol(c) for c in cs)
            flip(v)
            return after - before
        if rnd.random() < 0.2:
            v = rnd.choice(cands)
        else:
            v = min(cands, key=lambda v: (delta(v), rnd.random()))
        cs = affected(v)
        flip(v)
        for c in cs:
            if viol(c): bad.add(c)
            else: bad.discard(c)
        if len(bad) < best[0]:
            best = (len(bad), dict(sig))
    nb, sg = best
    return ({n: s for (k, n), s in sg.items() if k == 'A'}, {n: s for (k, n), s in sg.items() if k == 'B'},
            {n: s for (k, n), s in sg.items() if k == 'C'}, nb)


class FixedProg:
    def __init__(self, net, outputs, sig, order=None):
        self.net, self.outputs, self.sig = net, outputs, sig
        self.order = order if order is not None else Prog(net, outputs).order
    def count(self):
        c = {'add': 0, 'sub': 0, 'mul': 0, 'in': 0}
        for n in self.order:
            c[self.net.nodes[n][0]] += 1
        return c


N, TAPS = 40, 16
G = build(N, TAPS, scale=False, variant=1)
HOP = G['hop']; R = len(G['a_out'])
T, D, K = 16000, 512, 31
L = (T - K) // 2 + 1
MB = 64; NCH = -(-L // (HOP * MB))
CH = HOP * MB
XM = CH + 16
LP = NCH * CH
TM = T // 2
LAST_M = TM - (NCH - 1) * CH
HS = 2.0 / N
T2 = 1; W3 = 1
U32, F32, BF16 = jnp.uint32, jnp.float32, jnp.bfloat16

bins = G['bins']
ev = [0, 1] + [2 + 3 * i + q for i, k in enumerate(bins) if k % 2 == 0 for q in range(3)]
od = [2 + 3 * i + q for i, k in enumerate(bins) if k % 2 == 1 for q in range(3)]
if (N // 2) % 2 == 1:
    ev.remove(1); od = [1] + od
IDX = (ev, od)
RH = (len(ev), len(od))
LOC = {}
for hf in range(2):
    for i, r in enumerate(IDX[hf]):
        LOC[r] = (hf, i)
SA, SB, SC, NBAD = solve_signs(G)
assert NBAD == 0
def mkprog(net, outs, sig):
    return FixedProg(net, outs, sig, order=min_live_order(net, outs, tries=100)[1])
PA = [mkprog(G['na'], [G['a_out'][r] for r in idx], SA) for idx in IDX]
PB = [mkprog(G['nb'], [G['b_out'][r] for r in idx], SB) for idx in IDX]
PC = mkprog(G['tn'], G['c_res'], SC)


def run_gen(prog, loads, sink):
    nsets = len(loads)
    vals = [dict() for _ in range(nsets)]
    sig = prog.sig
    outs = {}
    for r, o in enumerate(prog.outputs):
        outs.setdefault(o[0], []).append(r)
    for n in prog.order:
        k = prog.net.nodes[n]
        for s in range(nsets):
            v = vals[s]
            if k[0] == 'in':
                v[n] = loads[s](k[1])
            elif k[0] == 'mul':
                v[n] = v[k[1]] * (k[2] * sig[n] * sig[k[1]])
            else:
                a, b = k[1], k[2]
                cb = 1 if k[0] == 'add' else -1
                p, q = sig[n] * sig[a], sig[n] * cb * sig[b]
                if p > 0 and q > 0: v[n] = v[a] + v[b]
                elif p > 0: v[n] = v[a] - v[b]
                elif q > 0: v[n] = v[b] - v[a]
                else: v[n] = -(v[a] + v[b])
            yield 1
        for r in outs.get(n, []):
            yield from sink(r, [vals[s][n] for s in range(nsets)])


def drain(gen):
    for _ in gen:
        pass


def unpack(wd, hi):
    wd = (wd & jnp.uint32(0xffff0000)) if hi else (wd << 16)
    return lax.bitcast_convert_type(wd, F32)


def pack(lo, hi):
    return pltpu.pack_elementwise([lo, hi], packed_dtype=BF16)


def prog_weight(prog, nsets, per_out):
    return len(prog.order) * nsets + len(prog.outputs) * per_out


def interleave(mms, gens_weights):
    total = sum(w for _, w in gens_weights)
    def allops():
        for g, _ in gens_weights:
            yield from g
    gen = allops()
    e = 0; done = False
    for i, mm in enumerate(mms):
        mm()
        tgt = (i + 1) * total // len(mms)
        while not done and e < tgt:
            try:
                e += next(gen)
            except StopIteration:
                done = True
    for _ in gen:
        pass


def merge(lists):
    lists = [l for l in lists if l]
    out = []
    pos = [0] * len(lists)
    tot = sum(len(l) for l in lists)
    for _ in range(tot):
        i = min((i for i in range(len(lists)) if pos[i] < len(lists[i])), key=lambda i: (pos[i] + 0.5) / len(lists[i]))
        out.append(lists[i][pos[i]]); pos[i] += 1
    return out


C0 = math.sqrt(2.0 / math.pi)
def gelu_half(zh):
    u = zh * (zh * zh * (8.0 * C0 * 0.044715) + 2.0 * C0)
    return zh * jnp.tanh(u) + zh


def kernel(x_hbm, w_hbm, gam_ref, bet_ref, out_hbm,
           xb0, xb1, xb2, xb3, we, wo, xe, xo, ye, yo, h0, h1, h2, h3, st, nrm, gsm, xsem, wsem, osem):
    xb = (xb0, xb1, xb2, xb3)
    wh = (we, wo); xh = (xe, xo); yy = (ye, yo)
    hh = (h0, h1, h2, h3)
    x32 = x_hbm.bitcast(U32)
    w32 = w_hbm.bitcast(F32)
    o32 = out_hbm.bitcast(F32)
    LASTJ = 2 * NCH - 1

    def x_copy(j, c, full):
        b = j // NCH
        cj = j % NCH
        rows = XM if full else LAST_M
        return pltpu.make_async_copy(
            x32.at[b, pl.ds(pl.multiple_of(cj * CH, 8), rows), pl.ds(c * 128, 128)],
            xb[c].at[pl.ds(0, rows), :], xsem.at[c])

    def x_start(j):
        cj = j % NCH
        @pl.when(cj < NCH - 1)
        def _():
            for c in range(4):
                x_copy(j, c, True).start()
        @pl.when(cj == NCH - 1)
        def _():
            for c in range(4):
                x_copy(j, c, False).start()
                xb[c][pl.ds(LAST_M, XM - LAST_M), :] = jnp.zeros((XM - LAST_M, 128), U32)

    def x_wait(j, cs=range(4)):
        cj = j % NCH
        @pl.when(cj < NCH - 1)
        def _():
            for c in cs:
                x_copy(j, c, True).wait()
        @pl.when(cj == NCH - 1)
        def _():
            for c in cs:
                x_copy(j, c, False).wait()

    WQ = 8
    def w_copy(n, q):
        dst = hh[n].at[1, pl.ds(0, K * 256), :].reshape(K, 256, 128)
        r = 256 // WQ
        return pltpu.make_async_copy(w32.at[:, pl.ds(q * r, r), pl.ds(n * 128, 128)], dst.at[:, pl.ds(q * r, r), :], wsem.at[n, q])

    def o_copy(n, r0, rows, k):
        return pltpu.make_async_copy(hh[n].at[0, pl.ds(r0, rows), :], o32.at[pl.ds(r0, rows), n, 0, :], osem.at[n, k])

    def a_piece(g, c, p, half):
        dyn = not isinstance(g, int)
        base = pl.multiple_of(g * (16 * HOP), 8) if dyn else g * (16 * HOP)
        row = pl.multiple_of(g * 8, 8) if dyn else g * 8
        xw = xb[c].at[pl.ds(base, 16 * HOP + 16), :]
        def mkload(o):
            return lambda t: unpack(xw[pl.ds(t + o * HOP, 8, stride=2 * HOP), :], p)
        def sink(i, vs):
            xh[half][i, pl.ds(row, 8), p * 512 + c * 128:p * 512 + (c + 1) * 128] = pack(vs[0], vs[1])
            yield 1
        return run_gen(PA[half], [mkload(0), mkload(1)], sink), prog_weight(PA[half], 2, 1)

    def a_pieces(half):
        return [a_piece(g, c, p, half) for c in range(4) for g in range(MB // 16) for p in range(2)]

    def w_piece(n, g, p, half):
        dyn = not isinstance(g, int)
        row = pl.multiple_of(g * 8, 8) if dyn else g * 8
        cache = {}
        def word(j):
            if j not in cache:
                cache[j] = lax.bitcast_convert_type(hh[n][1, pl.ds((2 * j + p) * 256 + row, 8), :], U32)
            return cache[j]
        def mkload(hi):
            def load(j):
                if 2 * j + p >= K:
                    return jnp.zeros((8, 128), F32)
                return unpack(word(j), hi)
            return load
        def sink(i, vs):
            wh[half][n, i, pl.ds(p * 256 + row, 8), :] = pack(vs[0], vs[1])
            yield 1
        return run_gen(PB[half], [mkload(0), mkload(1)], sink), prog_weight(PB[half], 2, 1)

    def c_pieces(j, n):
        if isinstance(j, int):
            b, cj = j // NCH, j % NCH
            slot = b
        else:
            valid = j >= 0
            b = jnp.where(valid, j // NCH, 0)
            cj = jnp.where(valid, j % NCH, NCH - 1)
            slot = jnp.where(valid, b, 2)
        state = {}
        def col(g):
            if g == 0:
                state['c'] = st[slot, n, 2]; state['a1'] = st[slot, n, 0]; state['a2'] = st[slot, n, 1]
            base = cj * CH + g * (8 * HOP)
            if not isinstance(j, int):
                base = pl.multiple_of(base, 8)
            hs = hh[n].at[b, pl.ds(base, 8 * HOP), :]
            def sink(t, vs):
                hs[pl.ds(t, 8, stride=HOP), :] = vs[0]
                d = vs[0] - state['c']
                state['a1'] = state['a1'] + d
                state['a2'] = state['a2'] + d * d
                yield 4
            yield from run_gen(PC, [lambda r: yy[LOC[r][0]][n, LOC[r][1], g * 8:(g + 1) * 8, :]], sink)
            if g == MB // 8 - 1:
                st[slot, n, 0] = state['a1']; st[slot, n, 1] = state['a2']
        return [(col(g), prog_weight(PC, 1, 4)) for g in range(MB // 8)]

    def set_shift(j, n):
        @pl.when(jnp.logical_and(j >= 0, j % NCH == 0))
        def _():
            st[j // NCH, n, 2] = jnp.broadcast_to(ye[n, LOC[0][1], 0:1, :], (8, 128))

    def finalize_stats(n):
        sub = lax.broadcasted_iota(jnp.int32, (8, 128), 0)
        for b in range(2):
            c = st[b, n, 2]
            r0 = (L // 8) * 8
            c1 = jnp.zeros((8, 128), F32); c2 = jnp.zeros((8, 128), F32)
            for r in range(r0, LP, 8):
                d = hh[n][b, r:r + 8, :] - c
                if r < L:
                    d = jnp.where(sub >= L - r, d, 0.0)
                c1 = c1 + d; c2 = c2 + d * d
            s1 = jnp.sum(st[b, n, 0] - c1, axis=0, keepdims=True)
            s2 = jnp.sum(st[b, n, 1] - c2, axis=0, keepdims=True)
            md = s1 * (1.0 / L)
            var = (s2 * (1.0 / L) - md * md) * (HS * HS)
            mu = c[0:1] + md
            a = (HS * lax.rsqrt(var + 1e-5)) * gam_ref[...].astype(F32).reshape(1, D)[:, n * 128:(n + 1) * 128]
            bb = bet_ref[...].astype(F32).reshape(1, D)[:, n * 128:(n + 1) * 128] - mu * a
            nrm[n, b, 0] = jnp.broadcast_to(0.5 * a, (8, 128))
            nrm[n, b, 1] = jnp.broadcast_to(0.5 * bb, (8, 128))

    def d_vreg(n, r, cs):
        a0, b0, a1, b1 = cs
        z0 = gelu_half(hh[n][0, pl.ds(r, 8), :] * a0 + b0)
        z1 = gelu_half(hh[n][1, pl.ds(r, 8), :] * a1 + b1)
        hh[n][0, pl.ds(r, 8), :] = lax.bitcast_convert_type(pack(z0, z1), F32)

    def d_consts(n):
        return nrm[n, 0, 0], nrm[n, 0, 1], nrm[n, 1, 0], nrm[n, 1, 1]

    def d_pieces(n, ra=0, rb=LP):
        state = {}
        def piece(r0, r1):
            if 'cs' not in state:
                state['cs'] = d_consts(n)
            for r in range(r0, r1, 8):
                d_vreg(n, r, state['cs'])
                yield 19
        P = 200
        return [(piece(r, min(r + P, rb)), 19 * (min(r + P, rb) - r) // 8) for r in range(ra, rb, P)]

    def fin_piece(n):
        def gen():
            finalize_stats(n)
            yield 100
        return [(gen(), 100)]

    NPC = 4
    PR = -(-(-(-L // NPC)) // 8) * 8
    def d_loop(n, k0):
        cs = d_consts(n)
        UN = 5
        for k in range(k0, NPC):
            r0 = k * PR; r1 = min(r0 + PR, LP)
            nv = -(-(r1 - r0) // 8)
            assert nv % UN == 0, nv
            def body(i, carry):
                for u in range(UN):
                    d_vreg(n, pl.multiple_of(r0 + (i * UN + u) * 8, 8), cs)
                return carry
            lax.fori_loop(0, nv // UN, body, 0)
            o_copy(n, r0, min(r0 + PR, L) - r0, k).start()

    def o_start_all(n):
        for k in range(NPC):
            r0 = k * PR
            o_copy(n, r0, min(r0 + PR, L) - r0, k).start()

    def o_wait_all(n):
        for k in range(NPC):
            r0 = k * PR
            o_copy(n, r0, min(r0 + PR, L) - r0, k).wait()

    def mm(half, n, i):
        def f():
            lhs = pltpu.bitcast(xh[half][i], BF16)
            rhs = pltpu.bitcast(wh[half][n, i], BF16)
            yy[half][n, i] = jnp.dot(lhs, rhs, preferred_element_type=F32)
        return f

    def body(name, half, tiles, lists, sl=None):
        mms = [mm(half, n, i) for n in tiles for i in range(RH[half])]
        if sl is not None:
            mms = mms[sl]
        with jax.named_scope(name):
            interleave(mms, merge(lists))

    j0 = jnp.int32(0)
    for k_ in range(32):
        gsm[k_] = jnp.int32(0)
    x_start(j0)
    for q in range(WQ):
        w_copy(0, q).start()
    st[...] = jnp.zeros_like(st)

    with jax.named_scope("a0"):
        for c in range(4):
            x_wait(j0, [c])
            def a0(g, carry):
                for p in range(2):
                    drain(a_piece(g, c, p, 0)[0])
                return carry
            lax.fori_loop(0, MB // 16, a0, 0)
        for n in range(1, 4):
            for q in range(WQ):
                w_copy(n, q).start()

    with jax.named_scope("wstage"):
        GP = 32 // WQ
        for n in range(4):
            phases = (1,) if (n == 3 and W3) else (0, 1)
            def wl(g, carry):
                for p in phases:
                    for half in range(2):
                        drain(w_piece(n, g, p, half)[0])
                return carry
            def wq(q, carry):
                w_copy(n, q).wait()
                lax.fori_loop(q * GP, (q + 1) * GP, wl, 0)
                return carry
            lax.fori_loop(0, WQ, wq, 0)

    def main(j, carry):
        @pl.when(j >= 0)
        def _():
            body("E01", 0, (0, 1), [a_pieces(1)])
        @pl.when(j + 1 <= LASTJ)
        def _():
            x_start(j + 1)
        set_shift(j - 1, 2); set_shift(j - 1, 3)
        if W3:
            @pl.when(j == 0)
            def _():
                body("O01W", 1, (0, 1), [[w_piece(3, g, 0, half) for g in range(32) for half in range(2)]])
        @pl.when(j + 1 >= (2 if W3 else 1))
        def _():
            body("O01", 1, (0, 1), [c_pieces(j - 1, 2), c_pieces(j - 1, 3)])
        @pl.when(j < (LASTJ if T2 else LASTJ + 1))
        def _():
            set_shift(j, 0); set_shift(j, 1)
        @pl.when(j + 2 < (LASTJ if T2 else LASTJ + 1) + 2)
        def _():
            body("E23", 0, (2, 3), [c_pieces(j, 0), c_pieces(j, 1)])
        @pl.when(j + 1 <= LASTJ)
        def _():
            x_wait(j + 1)
        @pl.when(j < (LASTJ if T2 else LASTJ + 1))
        def _():
            body("O23", 1, (2, 3), [a_pieces(0)])
        return carry
    lax.fori_loop(0, LASTJ + 1, main, 0)

    jl = jnp.int32(LASTJ)
    if T2:
        gd = gsm[0]
        set_shift(jl, 0); set_shift(jl, 1)
        def o_start(n, ks):
            for k in ks:
                r0 = k * PR
                o_copy(n, r0, min(r0 + PR, L) - r0, k).start()
        def dq(n, k):
            return d_pieces(n, k * PR, min((k + 1) * PR, LP))
        allmm = [(0, 2, i) for i in range(RH[0])] + [(0, 3, i) for i in range(RH[0])] + \
                [(1, 2, i) for i in range(RH[1])] + [(1, 3, i) for i in range(RH[1])]
        no3 = len(allmm) - RH[1]
        cuts = [0, 8, 18, 28, 38, 52, 64, 76, no3, len(allmm)]
        plan = [
            (c_pieces(LASTJ, 0) + fin_piece(0) + dq(0, 0), [(0, 0)]),
            (dq(0, 1), [(0, 1)]),
            (dq(0, 2), [(0, 2)]),
            (dq(0, 3), [(0, 3)]),
            (c_pieces(LASTJ, 1) + fin_piece(1) + dq(1, 0), [(1, 0)]),
            (dq(1, 1), [(1, 1)]),
            (dq(1, 2), [(1, 2)]),
            (dq(1, 3), [(1, 3)]),
            (c_pieces(LASTJ, 2) + fin_piece(2) + dq(2, 0), [(2, 0)]),
        ]
        set_shift(jl, 2)
        for bi, (pcs, starts) in enumerate(plan):
            @pl.when(gsm[16 + bi] >= 0)
            def _():
                with jax.named_scope("D%d" % bi):
                    interleave([mm(*t) for t in allmm[cuts[bi]:cuts[bi + 1]]], pcs)
            for n_, k_ in starts:
                o_start(n_, (k_,))

    with jax.named_scope("tail"):
        set_shift(jl, 3)
        d_loop(2, 1)
        for g_, _ in c_pieces(LASTJ, 3):
            drain(g_)
        finalize_stats(3)
        d_loop(3, 0)
        for n in range(4):
            o_wait_all(n)


@jax.jit
def pallas_standalone__self_sup_conv_stem_wavlm__speech_kernel(x, w, gn_gamma, gn_beta):
    out = pl.pallas_call(
        kernel,
        in_specs=[pl.BlockSpec(memory_space=pl.ANY), pl.BlockSpec(memory_space=pl.ANY),
                  pl.BlockSpec(memory_space=pltpu.VMEM), pl.BlockSpec(memory_space=pltpu.VMEM)],
        out_specs=pl.BlockSpec(memory_space=pl.ANY),
        out_shape=jax.ShapeDtypeStruct((L, 4, 2, 128), BF16),
        scratch_shapes=[pltpu.VMEM((XM, 128), U32)] * 4 + [
            pltpu.VMEM((4, RH[0], 512, 128), U32),
            pltpu.VMEM((4, RH[1], 512, 128), U32),
            pltpu.VMEM((RH[0], MB // 2, 1024), U32),
            pltpu.VMEM((RH[1], MB // 2, 1024), U32),
            pltpu.VMEM((4, RH[0], MB, 128), F32),
            pltpu.VMEM((4, RH[1], MB, 128), F32)] + [pltpu.VMEM((2, LP, 128), F32)] * 4 + [
            pltpu.VMEM((3, 4, 3, 8, 128), F32),
            pltpu.VMEM((4, 2, 2, 8, 128), F32),
            pltpu.SMEM((32,), jnp.int32),
            pltpu.SemaphoreType.DMA((4,)),
            pltpu.SemaphoreType.DMA((4, 8)),
            pltpu.SemaphoreType.DMA((4, 4)),
        ],
        compiler_params=pltpu.CompilerParams(vmem_limit_bytes=127 * 1024 * 1024),
    )(x, w, gn_gamma, gn_beta)
    return out.transpose(2, 0, 1, 3).reshape(2, L, D)
```

```python
import math
import random
import numpy as np
import jax, jax.numpy as jnp
from jax import lax
from jax.experimental import pallas as pl
from jax.experimental.pallas import tpu as pltpu


class Net:
    def __init__(self):
        self.nodes = []
        self.cse = {}

    def _mk(self, key):
        if key in self.cse:
            return self.cse[key]
        self.nodes.append(key)
        self.cse[key] = len(self.nodes) - 1
        return self.cse[key]

    def inp(self, i):
        return (self._mk(('in', i)), 1)

    def neg(self, x):
        return None if x is None else (x[0], -x[1])

    def add(self, x, y):
        if x is None:
            return y
        if y is None:
            return x
        (a, sa), (b, sb) = x, y
        if a == b:
            if sa == sb:
                return self.mul(x, 2.0)
            return None
        if sa == sb:
            if a > b:
                a, b = b, a
            return (self._mk(('add', a, b)), sa)
        if a > b:
            a, b, sa = b, a, sb
        return (self._mk(('sub', a, b)), sa)

    def sub(self, x, y):
        return self.add(x, self.neg(y))

    def mul(self, x, c):
        if x is None or abs(c) < 1e-12:
            return None
        a, s = x
        if c < 0:
            c, s = -c, -s
        if abs(c - 1.0) < 1e-12:
            return (a, s)
        c = float(np.float64(round(c, 14)))
        return (self._mk(('mul', a, c)), s)

    def cadd(self, x, y):
        return (self.add(x[0], y[0]), self.add(x[1], y[1]))

    def csub(self, x, y):
        return (self.sub(x[0], y[0]), self.sub(x[1], y[1]))

    def cmulc(self, x, c, s):
        a, b = x
        if abs(s) < 1e-12:
            return (self.mul(a, c), self.mul(b, c))
        if abs(c) < 1e-12:
            return (self.mul(b, -s), self.mul(a, s))
        if abs(abs(c) - abs(s)) < 1e-12:
            sg = 1.0 if s * c > 0 else -1.0
            re = self.sub(a, self.mul(b, sg))
            im = self.add(b, self.mul(a, sg))
            return (self.mul(re, c), self.mul(im, c))
        re = self.sub(self.mul(a, c), self.mul(b, s))
        im = self.add(self.mul(a, s), self.mul(b, c))
        return (re, im)


def w(k, n):
    ang = -2.0 * math.pi * (k % n) / n
    return math.cos(ang), math.sin(ang)


def cfft(net, z):
    n = len(z)
    if n == 1:
        return [z[0]]
    if n == 2:
        return [net.cadd(z[0], z[1]), net.csub(z[0], z[1])]
    if n % 4 == 0:
        h, q = n // 2, n // 4
        e = [net.cadd(z[t], z[t + h]) for t in range(h)]
        o = [net.csub(z[t], z[t + h]) for t in range(h)]
        z1, z3 = [], []
        for t in range(q):
            a, b = o[t], o[t + q]
            mib = (b[1], net.neg(b[0]))
            p = net.cadd(a, mib)
            m = net.csub(a, mib)
            z1.append(net.cmulc(p, *w(t, n)))
            z3.append(net.cmulc(m, *w(3 * t, n)))
        E = cfft(net, e)
        Z1 = cfft(net, z1)
        Z3 = cfft(net, z3)
        out = [None] * n
        for k in range(h):
            out[2 * k] = E[k]
        for k in range(q):
            out[4 * k + 1] = Z1[k]
            out[4 * k + 3] = Z3[k]
        return out
    if n % 2 == 0:
        m = n // 2
        out = [None] * n
        rows = []
        for t2 in range(m):
            a = z[(2 * t2) % n]
            b = z[(m + 2 * t2) % n]
            rows.append((net.cadd(a, b), net.csub(a, b)))
        for k1 in range(2):
            Z = cfft(net, [rows[t2][k1] for t2 in range(m)])
            for k2 in range(m):
                for k in range(n):
                    if k % 2 == k1 and k % m == k2:
                        out[k] = Z[k2]
        return out
    if n % 3 == 0 and n > 3:
        raise NotImplementedError
    out = []
    p = {t: net.cadd(z[t], z[n - t]) for t in range(1, (n + 1) // 2)}
    q = {t: net.csub(z[t], z[n - t]) for t in range(1, (n + 1) // 2)}
    s = z[0]
    for t in p:
        s = net.cadd(s, p[t])
    out = [None] * n
    out[0] = s
    for k in range(1, (n + 1) // 2):
        A = z[0]
        B = (None, None)
        for t in p:
            c, sn = w(k * t, n)
            A = net.cadd(A, (net.mul(p[t][0], c), net.mul(p[t][1], c)))
            B = net.cadd(B, (net.mul(q[t][1], -sn), net.mul(q[t][0], sn)))
        out[k] = net.cadd(A, B)
        out[n - k] = net.csub(A, B)
    return out


def cfft_pfa(net, z, n1, n2):
    n = n1 * n2
    out = [None] * n
    cols = [cfft_any(net, [z[(n2 * t1 + n1 * t2) % n] for t2 in range(n2)]) for t1 in range(n1)]
    for k2 in range(n2):
        Z = cfft_any(net, [cols[t1][k2] for t1 in range(n1)])
        for k1 in range(n1):
            for k in range(n):
                if k % n1 == k1 and k % n2 == k2:
                    out[k] = Z[k1]
    return out


def cfft5(net, z):
    c1, c2 = math.cos(2 * math.pi / 5), math.cos(4 * math.pi / 5)
    s1, s2 = math.sin(2 * math.pi / 5), math.sin(4 * math.pi / 5)
    t1 = net.cadd(z[1], z[4]); t2 = net.cadd(z[2], z[3])
    t3 = net.csub(z[1], z[4]); t4 = net.csub(z[2], z[3])
    t5 = net.cadd(t1, t2)
    def rm(x, c):
        return (net.mul(x[0], c), net.mul(x[1], c))
    m1 = rm(t5, (c1 + c2) / 2 - 1.0)
    m2 = rm(net.csub(t1, t2), (c1 - c2) / 2)
    y0 = net.cadd(z[0], t5)
    a = net.cadd(y0, m1)
    a1 = net.cadd(a, m2); a2 = net.csub(a, m2)
    m3 = rm(net.cadd(t3, t4), s2)
    m4 = rm(t3, s1 - s2)
    m5 = rm(t4, s1 + s2)
    b1 = net.cadd(m3, m4)
    b2 = net.csub(m3, m5)
    def mi(x):
        return (x[1], net.neg(x[0]))
    return [y0, net.cadd(a1, mi(b1)), net.cadd(a2, mi(b2)), net.csub(a2, mi(b2)), net.csub(a1, mi(b1))]


def rfft5(net, x):
    c1, c2 = math.cos(2 * math.pi / 5), math.cos(4 * math.pi / 5)
    s1, s2 = math.sin(2 * math.pi / 5), math.sin(4 * math.pi / 5)
    t1 = net.add(x[1], x[4]); t2 = net.add(x[2], x[3])
    t3 = net.sub(x[1], x[4]); t4 = net.sub(x[2], x[3])
    t5 = net.add(t1, t2)
    m1 = net.mul(t5, (c1 + c2) / 2 - 1.0)
    m2 = net.mul(net.sub(t1, t2), (c1 - c2) / 2)
    y0 = net.add(x[0], t5)
    a = net.add(y0, m1)
    a1 = net.add(a, m2); a2 = net.sub(a, m2)
    m3 = net.mul(net.add(t3, t4), s2)
    m4 = net.mul(t3, s1 - s2)
    m5 = net.mul(t4, s1 + s2)
    b1 = net.add(m3, m4); b2 = net.sub(m3, m5)
    return [(y0, None), (a1, net.neg(b1)), (a2, net.neg(b2))]


def cfft_any(net, z):
    n = len(z)
    if n == 5:
        return cfft5(net, z)
    if n == 12:
        return cfft_pfa(net, z, 3, 4)
    if n == 10:
        return cfft_pfa(net, z, 5, 2)
    if n == 20:
        return cfft_pfa(net, z, 5, 4)
    if n == 6:
        return cfft_pfa(net, z, 3, 2)
    if n == 14:
        return cfft_pfa(net, z, 7, 2)
    if n == 15:
        return cfft_pfa(net, z, 5, 3)
    return cfft(net, z)


def rfft_pfa(net, x, n1, n2):
    n = n1 * n2
    inner = [rfft(net, [x[(n2 * t1 + n1 * t2) % n] for t1 in range(n1)]) for t2 in range(n2)]
    out = [None] * (n // 2 + 1)
    for k1 in range(n1 // 2 + 1):
        col = [inner[t2][k1] for t2 in range(n2)]
        if all(c[1] is None for c in col):
            Z = rfft(net, [c[0] for c in col])
            Z = Z + [(Z[n2 - k2][0], net.neg(Z[n2 - k2][1])) for k2 in range(len(Z), n2)]
        else:
            Z = cfft_any(net, col)
        for k2 in range(n2):
            k = [k for k in range(n) if k % n1 == k1 and k % n2 == k2][0]
            if k <= n // 2:
                if out[k] is None:
                    out[k] = Z[k2]
            else:
                if out[n - k] is None:
                    out[n - k] = (Z[k2][0], net.neg(Z[k2][1]))
    return out


PFA = {40: (8, 5), 20: (4, 5), 24: (8, 3), 48: (16, 3), 12: (4, 3), 56: (8, 7), 10: (2, 5), 6: (2, 3), 60: (4, 15), 15: (3, 5), 44: (4, 11), 36: (4, 9)}
USE_PFA = True


def rfft(net, x):
    n = len(x)
    if USE_PFA and n in PFA:
        return rfft_pfa(net, x, *PFA[n])
    if n == 1:
        return [(x[0], None)]
    if n == 2:
        return [(net.add(x[0], x[1]), None), (net.sub(x[0], x[1]), None)]
    if n % 4 == 0:
        h, q = n // 2, n // 4
        e = [net.add(x[t], x[t + h]) for t in range(h)]
        o = [net.sub(x[t], x[t + h]) for t in range(h)]
        z = [net.cmulc((o[t], net.neg(o[t + q])), *w(t, n)) for t in range(q)]
        E = rfft(net, e)
        Z = cfft_any(net, z)
        out = [None] * (h + 1)
        for k in range(len(E)):
            out[2 * k] = E[k]
        for k in range(q):
            f = 4 * k + 1
            if f <= h:
                out[f] = Z[k]
            else:
                out[n - f] = (Z[k][0], net.neg(Z[k][1]))
        return out
    if n % 2 == 0:
        m = n // 2
        e = [net.add(x[t], x[t + m]) for t in range(m)]
        o = [net.sub(x[t], x[t + m]) for t in range(m)]
        E = rfft(net, e)
        op = [o[t] if t % 2 == 0 else net.neg(o[t]) for t in range(m)]
        O = rfft(net, op)
        out = [None] * (m + 1)
        for k in range(len(E)):
            out[2 * k] = E[k]
        for f in range(1, m + 1, 2):
            j = ((f - m) // 2) % m
            if j <= m // 2:
                out[f] = O[j]
            else:
                out[f] = (O[m - j][0], net.neg(O[m - j][1]))
        return out
    if n == 5:
        return rfft5(net, x)
    p = {t: net.add(x[t], x[n - t]) for t in range(1, (n + 1) // 2)}
    q = {t: net.sub(x[t], x[n - t]) for t in range(1, (n + 1) // 2)}
    s = x[0]
    for t in p:
        s = net.add(s, p[t])
    out = [(s, None)]
    for k in range(1, (n + 1) // 2):
        A = x[0]
        B = None
        for t in p:
            c, sn = w(k * t, n)
            A = net.add(A, net.mul(p[t], c))
            B = net.add(B, net.mul(q[t], sn))
        out.append((A, B))
    return out


class Prog:
    def __init__(self, net, outputs):
        order = []
        seen = set()

        def visit(n):
            if n in seen:
                return
            seen.add(n)
            k = net.nodes[n]
            if k[0] in ('add', 'sub'):
                visit(k[1]); visit(k[2])
            elif k[0] == 'mul':
                visit(k[1])
            order.append(n)
        for o in outputs:
            if o is not None:
                visit(o[0])
        self.net = net
        self.order = order
        self.outputs = outputs

    def count(self):
        c = {'add': 0, 'sub': 0, 'mul': 0, 'in': 0}
        for n in self.order:
            c[self.net.nodes[n][0]] += 1
        return c

    def run(self, load, emit=None):
        vals = {}
        for n in self.order:
            k = self.net.nodes[n]
            if k[0] == 'in':
                vals[n] = load(k[1])
            elif k[0] == 'add':
                vals[n] = vals[k[1]] + vals[k[2]]
            elif k[0] == 'sub':
                vals[n] = vals[k[1]] - vals[k[2]]
            else:
                vals[n] = vals[k[1]] * k[2]
        return [None if o is None else vals[o[0]] for o in self.outputs]

    @property
    def signs(self):
        return [0 if o is None else o[1] for o in self.outputs]

    def matrix(self, n_in, signed=True):
        eye = np.eye(n_in)
        res = self.run(lambda i: eye[i])
        rows = []
        for r, s in zip(res, self.signs):
            rows.append(np.zeros(n_in) if r is None else (r * s if signed else r))
        return np.stack(rows)


def transpose(net, outputs, wanted_inputs):
    prog = Prog(net, outputs)
    live = set(prog.order)
    consumers = {n: [] for n in prog.order}
    for n in prog.order:
        k = net.nodes[n]
        if k[0] == 'add':
            consumers[k[1]].append((n, 1.0)); consumers[k[2]].append((n, 1.0))
        elif k[0] == 'sub':
            consumers[k[1]].append((n, 1.0)); consumers[k[2]].append((n, -1.0))
        elif k[0] == 'mul':
            consumers[k[1]].append((n, k[2]))
    outmap = {}
    for r, o in enumerate(outputs):
        if o is not None:
            outmap.setdefault(o[0], []).append((r, o[1]))
    tn = Net()
    memo = {}

    def adj(n):
        if n in memo:
            return memo[n]
        acc = None
        for r, s in outmap.get(n, []):
            v = tn.inp(r)
            acc = tn.add(acc, v if s > 0 else tn.neg(v))
        for c, coef in consumers[n]:
            acc = tn.add(acc, tn.mul(adj(c), coef))
        memo[n] = acc
        return acc
    outs = []
    for i in wanted_inputs:
        key = ('in', i)
        if key in net.cse and net.cse[key] in live:
            outs.append(adj(net.cse[key]))
        else:
            outs.append(None)
    return tn, outs


def build(N, taps, scale=True, variant=0):
    hop = N - taps + 1
    na = Net()
    U = rfft(na, [na.inp(t) for t in range(N)])
    a_out = [U[0][0], U[N // 2][0]]
    bins = list(range(1, N // 2))
    for k in bins:
        a, b = U[k]
        if variant == 0:
            a_out += [na.add(a, b), a, b]
        else:
            a_out += [a, na.sub(b, a), na.add(a, b)]
    nc = Net()
    V = rfft(nc, [nc.inp(t) for t in range(N)])
    c_out = [V[0][0], V[N // 2][0]]
    for k in bins:
        al, be = V[k]
        c_out += [nc.add(al, be), be, nc.neg(al)]
    tn, c_res = transpose(nc, c_out, list(range(hop)))
    def mkb(ntaps):
        nb = Net()
        Wf = rfft(nb, [nb.inp(t) if t < ntaps else None for t in range(N)])
        s0 = 1.0 / N if scale else 0.5
        b_out = [nb.mul(Wf[0][0], s0), nb.mul(Wf[N // 2][0], s0)]
        for k in bins:
            c = Wf[k][0]
            d = nb.neg(Wf[k][1])
            sc = 2.0 / N if scale else 1.0
            if variant == 0:
                b_out += [nb.mul(c, sc), nb.mul(nb.sub(d, c), sc), nb.mul(nb.add(c, d), sc)]
            else:
                b_out += [nb.mul(nb.add(c, d), sc), nb.mul(c, sc), nb.mul(d, sc)]
        return nb, b_out
    nb, b_out = mkb(taps)
    nb1, b1_out = mkb(taps - 1)
    return dict(N=N, hop=hop, taps=taps, na=na, a_out=a_out, nb=nb, b_out=b_out, nb1=nb1, b1_out=b1_out,
                tn=tn, c_res=c_res, bins=bins)


def max_live(net, order, outputs, out_at_once=True):
    uses = {n: 0 for n in order}
    for n in order:
        k = net.nodes[n]
        for a in ([k[1], k[2]] if k[0] in ('add', 'sub') else [k[1]] if k[0] == 'mul' else []):
            uses[a] += 1
    live = set(); peak = 0; tot = 0
    rem = dict(uses)
    for n in order:
        k = net.nodes[n]
        live.add(n)
        peak = max(peak, len(live))
        for a in set([k[1], k[2]] if k[0] in ('add', 'sub') else [k[1]] if k[0] == 'mul' else []):
            rem[a] -= (1 if k[0] == 'mul' or k[1] != k[2] else 2)
            if rem[a] == 0:
                live.discard(a)
        if rem[n] == 0:
            live.discard(n)
        tot += len(live)
    return peak, tot / len(order)


def min_live_order(net, outputs, seed=0, tries=200):
    base = Prog(net, outputs).order
    nodes = set(base)
    def operands(n):
        k = net.nodes[n]
        return [k[1], k[2]] if k[0] in ('add', 'sub') else [k[1]] if k[0] == 'mul' else []
    consumers = {n: [] for n in base}
    for n in base:
        for a in set(operands(n)):
            consumers[a].append(n)
    best = (max_live(net, base, outputs), base)
    rnd = random.Random(seed)
    pos = {n: i for i, n in enumerate(base)}
    for it in range(tries):
        done = set(); order = []
        live = set()
        remc = {n: len(consumers[n]) for n in base}
        isin = {n: net.nodes[n][0] == 'in' for n in base}
        def ready(n):
            return n not in done and not isin[n] and all((a in done) or isin[a] for a in operands(n))
        noise = rnd.random() * 1.5
        work = [n for n in base if not isin[n]]
        left = set(work)
        while left:
            cands = [n for n in left if ready(n)]
            def score(n):
                ops = set(operands(n))
                newloads = sum(1 for a in ops if a not in done)
                kills = sum(1 for a in ops if remc[a] == 1)
                born = 0 if remc[n] == 0 else 1
                return (newloads + born - kills) + noise * rnd.random() + 1e-4 * pos[n]
            n = min(cands, key=score)
            for a in sorted(set(operands(n)), key=lambda a: pos[a]):
                if a not in done:
                    done.add(a); order.append(a)
                remc[a] -= 1
            done.add(n); order.append(n); left.discard(n)
        ml = max_live(net, order, outputs)
        if ml < best[0]:
            best = (ml, order)
    return best


def solve_signs(G, iters=200000, seed=0):
    rnd = random.Random(seed)
    nets = {'A': (G['na'], G['a_out']), 'B': (G['nb'], G['b_out']), 'C': (G['tn'], G['c_res'])}
    order = {k: Prog(*v).order for k, v in nets.items()}
    R = len(G['a_out'])
    sig = {}
    for k in 'ABC':
        for n in order[k]:
            sig[(k, n)] = 1
    fixed = set()
    for k in 'AB':
        for n in order[k]:
            if nets[k][0].nodes[n][0] == 'in':
                fixed.add((k, n))
    for o in G['c_res']:
        sig[('C', o[0])] = o[1]; fixed.add(('C', o[0]))
    cin = {}
    for n in order['C']:
        nd = G['tn'].nodes[n]
        if nd[0] == 'in':
            cin[nd[1]] = n; fixed.add(('C', n))
    def cin_sign(r):
        a, b = G['a_out'][r], G['b_out'][r]
        return (sig[('A', a[0])] * a[1]) * (sig[('B', b[0])] * b[1])
    outmap = {}
    for r in range(R):
        outmap.setdefault(('A', G['a_out'][r][0]), []).append(r)
        outmap.setdefault(('B', G['b_out'][r][0]), []).append(r)
    def refresh():
        for r, n in cin.items():
            sig[('C', n)] = cin_sign(r)
    clauses = []
    for k in 'ABC':
        net = nets[k][0]
        for n in order[k]:
            nd = net.nodes[n]
            if nd[0] in ('add', 'sub'):
                clauses.append((k, n, nd[1], nd[2], 1 if nd[0] == 'add' else -1))
    occ = {}
    for ci, (k, n, a, b, cb) in enumerate(clauses):
        for v in (n, a, b):
            occ.setdefault((k, v), []).append(ci)
    def viol(ci):
        k, n, a, b, cb = clauses[ci]
        return sig[(k, n)] * sig[(k, a)] < 0 and sig[(k, n)] * cb * sig[(k, b)] < 0
    def flip(v):
        sig[v] = -sig[v]
        for r in outmap.get(v, []):
            if r in cin:
                sig[('C', cin[r])] = cin_sign(r)
    def affected(v):
        cs = set(occ.get(v, []))
        for r in outmap.get(v, []):
            if r in cin:
                cs.update(occ.get(('C', cin[r]), []))
        return cs
    flippers = {}
    for v, rs in outmap.items():
        for r in rs:
            if r in cin:
                flippers.setdefault(('C', cin[r]), []).append(v)
    refresh()
    bad = {ci for ci in range(len(clauses)) if viol(ci)}
    best = (len(bad), dict(sig))
    for it in range(iters):
        if not bad:
            break
        ci = rnd.choice(list(bad))
        k, n, a, b, cb = clauses[ci]
        cands = []
        for v in ((k, n), (k, a), (k, b)):
            if v in fixed:
                cands += flippers.get(v, [])
            else:
                cands.append(v)
        cands = [v for v in cands if v not in fixed]
        if not cands:
            continue
        def delta(v):
            cs = affected(v)
            before = sum(viol(c) for c in cs)
            flip(v)
            after = sum(viol(c) for c in cs)
            flip(v)
            return after - before
        if rnd.random() < 0.2:
            v = rnd.choice(cands)
        else:
            v = min(cands, key=lambda v: (delta(v), rnd.random()))
        cs = affected(v)
        flip(v)
        for c in cs:
            if viol(c): bad.add(c)
            else: bad.discard(c)
        if len(bad) < best[0]:
            best = (len(bad), dict(sig))
    nb, sg = best
    return ({n: s for (k, n), s in sg.items() if k == 'A'}, {n: s for (k, n), s in sg.items() if k == 'B'},
            {n: s for (k, n), s in sg.items() if k == 'C'}, nb)


class FixedProg:
    def __init__(self, net, outputs, sig, order=None):
        self.net, self.outputs, self.sig = net, outputs, sig
        self.order = order if order is not None else Prog(net, outputs).order
    def count(self):
        c = {'add': 0, 'sub': 0, 'mul': 0, 'in': 0}
        for n in self.order:
            c[self.net.nodes[n][0]] += 1
        return c


N, TAPS = 40, 16
G = build(N, TAPS, scale=False, variant=1)
HOP = G['hop']; R = len(G['a_out'])
T, D, K = 16000, 512, 31
L = (T - K) // 2 + 1
MB = 64; NCH = -(-L // (HOP * MB))
CH = HOP * MB
XM = CH + 16
LP = NCH * CH
TM = T // 2
LAST_M = TM - (NCH - 1) * CH
HS = 2.0 / N
T2 = 1; W3 = 1
U32, F32, BF16 = jnp.uint32, jnp.float32, jnp.bfloat16

bins = G['bins']
ev = [0, 1] + [2 + 3 * i + q for i, k in enumerate(bins) if k % 2 == 0 for q in range(3)]
od = [2 + 3 * i + q for i, k in enumerate(bins) if k % 2 == 1 for q in range(3)]
if (N // 2) % 2 == 1:
    ev.remove(1); od = [1] + od
IDX = (ev, od)
RH = (len(ev), len(od))
LOC = {}
for hf in range(2):
    for i, r in enumerate(IDX[hf]):
        LOC[r] = (hf, i)
SA, SB, SC, NBAD = solve_signs(G)
assert NBAD == 0
def mkprog(net, outs, sig):
    return FixedProg(net, outs, sig, order=min_live_order(net, outs, tries=100)[1])
PA = [mkprog(G['na'], [G['a_out'][r] for r in idx], SA) for idx in IDX]
PB = [mkprog(G['nb'], [G['b_out'][r] for r in idx], SB) for idx in IDX]
PC = mkprog(G['tn'], G['c_res'], SC)


def run_gen(prog, loads, sink):
    nsets = len(loads)
    vals = [dict() for _ in range(nsets)]
    sig = prog.sig
    outs = {}
    for r, o in enumerate(prog.outputs):
        outs.setdefault(o[0], []).append(r)
    for n in prog.order:
        k = prog.net.nodes[n]
        for s in range(nsets):
            v = vals[s]
            if k[0] == 'in':
                v[n] = loads[s](k[1])
            elif k[0] == 'mul':
                v[n] = v[k[1]] * (k[2] * sig[n] * sig[k[1]])
            else:
                a, b = k[1], k[2]
                cb = 1 if k[0] == 'add' else -1
                p, q = sig[n] * sig[a], sig[n] * cb * sig[b]
                if p > 0 and q > 0: v[n] = v[a] + v[b]
                elif p > 0: v[n] = v[a] - v[b]
                elif q > 0: v[n] = v[b] - v[a]
                else: v[n] = -(v[a] + v[b])
            yield 1
        for r in outs.get(n, []):
            yield from sink(r, [vals[s][n] for s in range(nsets)])


def drain(gen):
    for _ in gen:
        pass


def unpack(wd, hi):
    wd = (wd & jnp.uint32(0xffff0000)) if hi else (wd << 16)
    return lax.bitcast_convert_type(wd, F32)


def pack(lo, hi):
    return pltpu.pack_elementwise([lo, hi], packed_dtype=BF16)


def prog_weight(prog, nsets, per_out):
    return len(prog.order) * nsets + len(prog.outputs) * per_out


def interleave(mms, gens_weights):
    total = sum(w for _, w in gens_weights)
    def allops():
        for g, _ in gens_weights:
            yield from g
    gen = allops()
    e = 0; done = False
    for i, mm in enumerate(mms):
        mm()
        tgt = (i + 1) * total // len(mms)
        while not done and e < tgt:
            try:
                e += next(gen)
            except StopIteration:
                done = True
    for _ in gen:
        pass


def merge(lists):
    lists = [l for l in lists if l]
    out = []
    pos = [0] * len(lists)
    tot = sum(len(l) for l in lists)
    for _ in range(tot):
        i = min((i for i in range(len(lists)) if pos[i] < len(lists[i])), key=lambda i: (pos[i] + 0.5) / len(lists[i]))
        out.append(lists[i][pos[i]]); pos[i] += 1
    return out


C0 = math.sqrt(2.0 / math.pi)
def gelu_half(zh):
    u = zh * (zh * zh * (8.0 * C0 * 0.044715) + 2.0 * C0)
    return zh * jnp.tanh(u) + zh


def kernel(x_hbm, w_hbm, gam_ref, bet_ref, out_hbm,
           xb0, xb1, xb2, xb3, we, wo, xe, xo, ye, yo, h0, h1, h2, h3, st, nrm, gsm, xsem, wsem, osem):
    xb = (xb0, xb1, xb2, xb3)
    wh = (we, wo); xh = (xe, xo); yy = (ye, yo)
    hh = (h0, h1, h2, h3)
    x32 = x_hbm.bitcast(U32)
    w32 = w_hbm.bitcast(F32)
    o32 = out_hbm.bitcast(F32)
    LASTJ = 2 * NCH - 1

    def x_copy(j, c, full):
        b = j // NCH
        cj = j % NCH
        rows = XM if full else LAST_M
        return pltpu.make_async_copy(
            x32.at[b, pl.ds(pl.multiple_of(cj * CH, 8), rows), pl.ds(c * 128, 128)],
            xb[c].at[pl.ds(0, rows), :], xsem.at[c])

    def x_start(j):
        cj = j % NCH
        @pl.when(cj < NCH - 1)
        def _():
            for c in range(4):
                x_copy(j, c, True).start()
        @pl.when(cj == NCH - 1)
        def _():
            for c in range(4):
                x_copy(j, c, False).start()
                xb[c][pl.ds(LAST_M, XM - LAST_M), :] = jnp.zeros((XM - LAST_M, 128), U32)

    def x_wait(j, cs=range(4)):
        cj = j % NCH
        @pl.when(cj < NCH - 1)
        def _():
            for c in cs:
                x_copy(j, c, True).wait()
        @pl.when(cj == NCH - 1)
        def _():
            for c in cs:
                x_copy(j, c, False).wait()

    WQ = 8
    def w_copy(n, q):
        dst = hh[n].at[1, pl.ds(0, K * 256), :].reshape(K, 256, 128)
        r = 256 // WQ
        return pltpu.make_async_copy(w32.at[:, pl.ds(q * r, r), pl.ds(n * 128, 128)], dst.at[:, pl.ds(q * r, r), :], wsem.at[n, q])

    def o_copy(n, r0, rows, k):
        return pltpu.make_async_copy(hh[n].at[0, pl.ds(r0, rows), :], o32.at[pl.ds(r0, rows), n, 0, :], osem.at[n, k])

    def a_piece(g, c, p, half):
        dyn = not isinstance(g, int)
        base = pl.multiple_of(g * (16 * HOP), 8) if dyn else g * (16 * HOP)
        row = pl.multiple_of(g * 8, 8) if dyn else g * 8
        xw = xb[c].at[pl.ds(base, 16 * HOP + 16), :]
        def mkload(o):
            return lambda t: unpack(xw[pl.ds(t + o * HOP, 8, stride=2 * HOP), :], p)
        def sink(i, vs):
            xh[half][i, pl.ds(row, 8), p * 512 + c * 128:p * 512 + (c + 1) * 128] = pack(vs[0], vs[1])
            yield 1
        return run_gen(PA[half], [mkload(0), mkload(1)], sink), prog_weight(PA[half], 2, 1)

    def a_pieces(half):
        return [a_piece(g, c, p, half) for c in range(4) for g in range(MB // 16) for p in range(2)]

    def w_piece(n, g, p, half):
        dyn = not isinstance(g, int)
        row = pl.multiple_of(g * 8, 8) if dyn else g * 8
        cache = {}
        def word(j):
            if j not in cache:
                cache[j] = lax.bitcast_convert_type(hh[n][1, pl.ds((2 * j + p) * 256 + row, 8), :], U32)
            return cache[j]
        def mkload(hi):
            def load(j):
                if 2 * j + p >= K:
                    return jnp.zeros((8, 128), F32)
                return unpack(word(j), hi)
            return load
        def sink(i, vs):
            wh[half][n, i, pl.ds(p * 256 + row, 8), :] = pack(vs[0], vs[1])
            yield 1
        return run_gen(PB[half], [mkload(0), mkload(1)], sink), prog_weight(PB[half], 2, 1)

    def c_pieces(j, n):
        if isinstance(j, int):
            b, cj = j // NCH, j % NCH
            slot = b
        else:
            valid = j >= 0
            b = jnp.where(valid, j // NCH, 0)
            cj = jnp.where(valid, j % NCH, NCH - 1)
            slot = jnp.where(valid, b, 2)
        state = {}
        def col(g):
            if g == 0:
                state['c'] = st[slot, n, 2]; state['a1'] = st[slot, n, 0]; state['a2'] = st[slot, n, 1]
            base = cj * CH + g * (8 * HOP)
            if not isinstance(j, int):
                base = pl.multiple_of(base, 8)
            hs = hh[n].at[b, pl.ds(base, 8 * HOP), :]
            def sink(t, vs):
                hs[pl.ds(t, 8, stride=HOP), :] = vs[0]
                d = vs[0] - state['c']
                state['a1'] = state['a1'] + d
                state['a2'] = state['a2'] + d * d
                yield 4
            yield from run_gen(PC, [lambda r: yy[LOC[r][0]][n, LOC[r][1], g * 8:(g + 1) * 8, :]], sink)
            if g == MB // 8 - 1:
                st[slot, n, 0] = state['a1']; st[slot, n, 1] = state['a2']
        return [(col(g), prog_weight(PC, 1, 4)) for g in range(MB // 8)]

    def set_shift(j, n):
        @pl.when(jnp.logical_and(j >= 0, j % NCH == 0))
        def _():
            st[j // NCH, n, 2] = jnp.broadcast_to(ye[n, LOC[0][1], 0:1, :], (8, 128))

    def finalize_stats(n):
        sub = lax.broadcasted_iota(jnp.int32, (8, 128), 0)
        for b in range(2):
            c = st[b, n, 2]
            r0 = (L // 8) * 8
            c1 = jnp.zeros((8, 128), F32); c2 = jnp.zeros((8, 128), F32)
            for r in range(r0, LP, 8):
                d = hh[n][b, r:r + 8, :] - c
                if r < L:
                    d = jnp.where(sub >= L - r, d, 0.0)
                c1 = c1 + d; c2 = c2 + d * d
            s1 = jnp.sum(st[b, n, 0] - c1, axis=0, keepdims=True)
            s2 = jnp.sum(st[b, n, 1] - c2, axis=0, keepdims=True)
            md = s1 * (1.0 / L)
            var = (s2 * (1.0 / L) - md * md) * (HS * HS)
            mu = c[0:1] + md
            a = (HS * lax.rsqrt(var + 1e-5)) * gam_ref[...].astype(F32).reshape(1, D)[:, n * 128:(n + 1) * 128]
            bb = bet_ref[...].astype(F32).reshape(1, D)[:, n * 128:(n + 1) * 128] - mu * a
            nrm[n, b, 0] = jnp.broadcast_to(0.5 * a, (8, 128))
            nrm[n, b, 1] = jnp.broadcast_to(0.5 * bb, (8, 128))

    def d_vreg(n, r, cs):
        a0, b0, a1, b1 = cs
        z0 = gelu_half(hh[n][0, pl.ds(r, 8), :] * a0 + b0)
        z1 = gelu_half(hh[n][1, pl.ds(r, 8), :] * a1 + b1)
        hh[n][0, pl.ds(r, 8), :] = lax.bitcast_convert_type(pack(z0, z1), F32)

    def d_consts(n):
        return nrm[n, 0, 0], nrm[n, 0, 1], nrm[n, 1, 0], nrm[n, 1, 1]

    def d_pieces(n, ra=0, rb=LP):
        state = {}
        def piece(r0, r1):
            if 'cs' not in state:
                state['cs'] = d_consts(n)
            for r in range(r0, r1, 8):
                d_vreg(n, r, state['cs'])
                yield 19
        P = 200
        return [(piece(r, min(r + P, rb)), 19 * (min(r + P, rb) - r) // 8) for r in range(ra, rb, P)]

    def fin_piece(n):
        def gen():
            finalize_stats(n)
            yield 100
        return [(gen(), 100)]

    NPC = 4
    PR = -(-(-(-L // NPC)) // 8) * 8
    def d_loop(n, k0):
        cs = d_consts(n)
        UN = 5
        for k in range(k0, NPC):
            r0 = k * PR; r1 = min(r0 + PR, LP)
            nv = -(-(r1 - r0) // 8)
            assert nv % UN == 0, nv
            def body(i, carry):
                for u in range(UN):
                    d_vreg(n, pl.multiple_of(r0 + (i * UN + u) * 8, 8), cs)
                return carry
            lax.fori_loop(0, nv // UN, body, 0)
            o_copy(n, r0, min(r0 + PR, L) - r0, k).start()

    def o_start_all(n):
        for k in range(NPC):
            r0 = k * PR
            o_copy(n, r0, min(r0 + PR, L) - r0, k).start()

    def o_wait_all(n):
        for k in range(NPC):
            r0 = k * PR
            o_copy(n, r0, min(r0 + PR, L) - r0, k).wait()

    def mm(half, n, i):
        def f():
            lhs = pltpu.bitcast(xh[half][i], BF16)
            rhs = pltpu.bitcast(wh[half][n, i], BF16)
            yy[half][n, i] = jnp.dot(lhs, rhs, preferred_element_type=F32)
        return f

    def body(name, half, tiles, lists, sl=None):
        mms = [mm(half, n, i) for n in tiles for i in range(RH[half])]
        if sl is not None:
            mms = mms[sl]
        with jax.named_scope(name):
            interleave(mms, merge(lists))

    j0 = jnp.int32(0)
    for k_ in range(32):
        gsm[k_] = jnp.int32(0)
    x_start(j0)
    for q in range(WQ):
        w_copy(0, q).start()
    st[...] = jnp.zeros_like(st)

    with jax.named_scope("a0"):
        for c in range(4):
            x_wait(j0, [c])
            def a0(g, carry):
                for p in range(2):
                    drain(a_piece(g, c, p, 0)[0])
                return carry
            lax.fori_loop(0, MB // 16, a0, 0)
        for n in range(1, 4):
            for q in range(WQ):
                w_copy(n, q).start()

    GP = 32 // WQ
    QX = 2
    with jax.named_scope("wstage"):
        for n in range(4):
            def wl(g, carry):
                for p in range(2):
                    for half in range(2):
                        drain(w_piece(n, g, p, half)[0])
                return carry
            def wq(q, carry):
                w_copy(n, q).wait()
                lax.fori_loop(q * GP, (q + 1) * GP, wl, 0)
                return carry
            lax.fori_loop(0, QX if n == 3 else WQ, wq, 0)

    def main(j, carry):
        @pl.when(j >= 0)
        def _():
            body("E01", 0, (0, 1), [a_pieces(1)])
        @pl.when(j + 1 <= LASTJ)
        def _():
            x_start(j + 1)
        set_shift(j - 1, 2); set_shift(j - 1, 3)
        if W3:
            @pl.when(j <= 0)
            def _():
                for q in range(QX, WQ):
                    w_copy(3, q).wait()
            @pl.when(j == 0)
            def _():
                body("O01W", 1, (0, 1), [[w_piece(3, g, p, half) for g in range(QX * GP, 32) for p in range(2) for half in range(2)]])
        @pl.when(j + 1 >= (2 if W3 else 1))
        def _():
            body("O01", 1, (0, 1), [c_pieces(j - 1, 2), c_pieces(j - 1, 3)])
        @pl.when(j < (LASTJ if T2 else LASTJ + 1))
        def _():
            set_shift(j, 0); set_shift(j, 1)
        @pl.when(j + 2 < (LASTJ if T2 else LASTJ + 1) + 2)
        def _():
            body("E23", 0, (2, 3), [c_pieces(j, 0), c_pieces(j, 1)])
        @pl.when(j + 1 <= LASTJ)
        def _():
            x_wait(j + 1)
        @pl.when(j < (LASTJ if T2 else LASTJ + 1))
        def _():
            body("O23", 1, (2, 3), [a_pieces(0)])
        return carry
    lax.fori_loop(0, LASTJ + 1, main, 0)

    jl = jnp.int32(LASTJ)
    if T2:
        gd = gsm[0]
        set_shift(jl, 0); set_shift(jl, 1)
        def o_start(n, ks):
            for k in ks:
                r0 = k * PR
                o_copy(n, r0, min(r0 + PR, L) - r0, k).start()
        def dq(n, k):
            return d_pieces(n, k * PR, min((k + 1) * PR, LP))
        allmm = [(0, 2, i) for i in range(RH[0])] + [(0, 3, i) for i in range(RH[0])] + \
                [(1, 2, i) for i in range(RH[1])] + [(1, 3, i) for i in range(RH[1])]
        no3 = len(allmm) - RH[1]
        cuts = [0, 8, 18, 28, 38, 52, 64, 76, no3, len(allmm)]
        plan = [
            (c_pieces(LASTJ, 0) + fin_piece(0) + dq(0, 0), [(0, 0)]),
            (dq(0, 1), [(0, 1)]),
            (dq(0, 2), [(0, 2)]),
            (dq(0, 3), [(0, 3)]),
            (c_pieces(LASTJ, 1) + fin_piece(1) + dq(1, 0), [(1, 0)]),
            (dq(1, 1), [(1, 1)]),
            (dq(1, 2), [(1, 2)]),
            (dq(1, 3), [(1, 3)]),
            (c_pieces(LASTJ, 2) + fin_piece(2) + dq(2, 0), [(2, 0)]),
        ]
        set_shift(jl, 2)
        for bi, (pcs, starts) in enumerate(plan):
            @pl.when(gsm[16 + bi] >= 0)
            def _():
                with jax.named_scope("D%d" % bi):
                    interleave([mm(*t) for t in allmm[cuts[bi]:cuts[bi + 1]]], pcs)
            for n_, k_ in starts:
                o_start(n_, (k_,))

    with jax.named_scope("tail"):
        set_shift(jl, 3)
        d_loop(2, 1)
        for g_, _ in c_pieces(LASTJ, 3):
            drain(g_)
        finalize_stats(3)
        d_loop(3, 0)
        for n in range(4):
            o_wait_all(n)


@jax.jit
def pallas_standalone__self_sup_conv_stem_wavlm__speech_kernel(x, w, gn_gamma, gn_beta):
    out = pl.pallas_call(
        kernel,
        in_specs=[pl.BlockSpec(memory_space=pl.ANY), pl.BlockSpec(memory_space=pl.ANY),
                  pl.BlockSpec(memory_space=pltpu.VMEM), pl.BlockSpec(memory_space=pltpu.VMEM)],
        out_specs=pl.BlockSpec(memory_space=pl.ANY),
        out_shape=jax.ShapeDtypeStruct((L, 4, 2, 128), BF16),
        scratch_shapes=[pltpu.VMEM((XM, 128), U32)] * 4 + [
            pltpu.VMEM((4, RH[0], 512, 128), U32),
            pltpu.VMEM((4, RH[1], 512, 128), U32),
            pltpu.VMEM((RH[0], MB // 2, 1024), U32),
            pltpu.VMEM((RH[1], MB // 2, 1024), U32),
            pltpu.VMEM((4, RH[0], MB, 128), F32),
            pltpu.VMEM((4, RH[1], MB, 128), F32)] + [pltpu.VMEM((2, LP, 128), F32)] * 4 + [
            pltpu.VMEM((3, 4, 3, 8, 128), F32),
            pltpu.VMEM((4, 2, 2, 8, 128), F32),
            pltpu.SMEM((32,), jnp.int32),
            pltpu.SemaphoreType.DMA((4,)),
            pltpu.SemaphoreType.DMA((4, 8)),
            pltpu.SemaphoreType.DMA((4, 4)),
        ],
        compiler_params=pltpu.CompilerParams(vmem_limit_bytes=127 * 1024 * 1024),
    )(x, w, gn_gamma, gn_beta)
    return out.transpose(2, 0, 1, 3).reshape(2, L, D)
```

```python
import math
import random
import numpy as np
import jax, jax.numpy as jnp
from jax import lax
from jax.experimental import pallas as pl
from jax.experimental.pallas import tpu as pltpu


class Net:
    def __init__(self):
        self.nodes = []
        self.cse = {}

    def _mk(self, key):
        if key in self.cse:
            return self.cse[key]
        self.nodes.append(key)
        self.cse[key] = len(self.nodes) - 1
        return self.cse[key]

    def inp(self, i):
        return (self._mk(('in', i)), 1)

    def neg(self, x):
        return None if x is None else (x[0], -x[1])

    def add(self, x, y):
        if x is None:
            return y
        if y is None:
            return x
        (a, sa), (b, sb) = x, y
        if a == b:
            if sa == sb:
                return self.mul(x, 2.0)
            return None
        if sa == sb:
            if a > b:
                a, b = b, a
            return (self._mk(('add', a, b)), sa)
        if a > b:
            a, b, sa = b, a, sb
        return (self._mk(('sub', a, b)), sa)

    def sub(self, x, y):
        return self.add(x, self.neg(y))

    def mul(self, x, c):
        if x is None or abs(c) < 1e-12:
            return None
        a, s = x
        if c < 0:
            c, s = -c, -s
        if abs(c - 1.0) < 1e-12:
            return (a, s)
        c = float(np.float64(round(c, 14)))
        return (self._mk(('mul', a, c)), s)

    def cadd(self, x, y):
        return (self.add(x[0], y[0]), self.add(x[1], y[1]))

    def csub(self, x, y):
        return (self.sub(x[0], y[0]), self.sub(x[1], y[1]))

    def cmulc(self, x, c, s):
        a, b = x
        if abs(s) < 1e-12:
            return (self.mul(a, c), self.mul(b, c))
        if abs(c) < 1e-12:
            return (self.mul(b, -s), self.mul(a, s))
        if abs(abs(c) - abs(s)) < 1e-12:
            sg = 1.0 if s * c > 0 else -1.0
            re = self.sub(a, self.mul(b, sg))
            im = self.add(b, self.mul(a, sg))
            return (self.mul(re, c), self.mul(im, c))
        re = self.sub(self.mul(a, c), self.mul(b, s))
        im = self.add(self.mul(a, s), self.mul(b, c))
        return (re, im)


def w(k, n):
    ang = -2.0 * math.pi * (k % n) / n
    return math.cos(ang), math.sin(ang)


def cfft(net, z):
    n = len(z)
    if n == 1:
        return [z[0]]
    if n == 2:
        return [net.cadd(z[0], z[1]), net.csub(z[0], z[1])]
    if n % 4 == 0:
        h, q = n // 2, n // 4
        e = [net.cadd(z[t], z[t + h]) for t in range(h)]
        o = [net.csub(z[t], z[t + h]) for t in range(h)]
        z1, z3 = [], []
        for t in range(q):
            a, b = o[t], o[t + q]
            mib = (b[1], net.neg(b[0]))
            p = net.cadd(a, mib)
            m = net.csub(a, mib)
            z1.append(net.cmulc(p, *w(t, n)))
            z3.append(net.cmulc(m, *w(3 * t, n)))
        E = cfft(net, e)
        Z1 = cfft(net, z1)
        Z3 = cfft(net, z3)
        out = [None] * n
        for k in range(h):
            out[2 * k] = E[k]
        for k in range(q):
            out[4 * k + 1] = Z1[k]
            out[4 * k + 3] = Z3[k]
        return out
    if n % 2 == 0:
        m = n // 2
        out = [None] * n
        rows = []
        for t2 in range(m):
            a = z[(2 * t2) % n]
            b = z[(m + 2 * t2) % n]
            rows.append((net.cadd(a, b), net.csub(a, b)))
        for k1 in range(2):
            Z = cfft(net, [rows[t2][k1] for t2 in range(m)])
            for k2 in range(m):
                for k in range(n):
                    if k % 2 == k1 and k % m == k2:
                        out[k] = Z[k2]
        return out
    if n % 3 == 0 and n > 3:
        raise NotImplementedError
    out = []
    p = {t: net.cadd(z[t], z[n - t]) for t in range(1, (n + 1) // 2)}
    q = {t: net.csub(z[t], z[n - t]) for t in range(1, (n + 1) // 2)}
    s = z[0]
    for t in p:
        s = net.cadd(s, p[t])
    out = [None] * n
    out[0] = s
    for k in range(1, (n + 1) // 2):
        A = z[0]
        B = (None, None)
        for t in p:
            c, sn = w(k * t, n)
            A = net.cadd(A, (net.mul(p[t][0], c), net.mul(p[t][1], c)))
            B = net.cadd(B, (net.mul(q[t][1], -sn), net.mul(q[t][0], sn)))
        out[k] = net.cadd(A, B)
        out[n - k] = net.csub(A, B)
    return out


def cfft_pfa(net, z, n1, n2):
    n = n1 * n2
    out = [None] * n
    cols = [cfft_any(net, [z[(n2 * t1 + n1 * t2) % n] for t2 in range(n2)]) for t1 in range(n1)]
    for k2 in range(n2):
        Z = cfft_any(net, [cols[t1][k2] for t1 in range(n1)])
        for k1 in range(n1):
            for k in range(n):
                if k % n1 == k1 and k % n2 == k2:
                    out[k] = Z[k1]
    return out


def cfft5(net, z):
    c1, c2 = math.cos(2 * math.pi / 5), math.cos(4 * math.pi / 5)
    s1, s2 = math.sin(2 * math.pi / 5), math.sin(4 * math.pi / 5)
    t1 = net.cadd(z[1], z[4]); t2 = net.cadd(z[2], z[3])
    t3 = net.csub(z[1], z[4]); t4 = net.csub(z[2], z[3])
    t5 = net.cadd(t1, t2)
    def rm(x, c):
        return (net.mul(x[0], c), net.mul(x[1], c))
    m1 = rm(t5, (c1 + c2) / 2 - 1.0)
    m2 = rm(net.csub(t1, t2), (c1 - c2) / 2)
    y0 = net.cadd(z[0], t5)
    a = net.cadd(y0, m1)
    a1 = net.cadd(a, m2); a2 = net.csub(a, m2)
    m3 = rm(net.cadd(t3, t4), s2)
    m4 = rm(t3, s1 - s2)
    m5 = rm(t4, s1 + s2)
    b1 = net.cadd(m3, m4)
    b2 = net.csub(m3, m5)
    def mi(x):
        return (x[1], net.neg(x[0]))
    return [y0, net.cadd(a1, mi(b1)), net.cadd(a2, mi(b2)), net.csub(a2, mi(b2)), net.csub(a1, mi(b1))]


def rfft5(net, x):
    c1, c2 = math.cos(2 * math.pi / 5), math.cos(4 * math.pi / 5)
    s1, s2 = math.sin(2 * math.pi / 5), math.sin(4 * math.pi / 5)
    t1 = net.add(x[1], x[4]); t2 = net.add(x[2], x[3])
    t3 = net.sub(x[1], x[4]); t4 = net.sub(x[2], x[3])
    t5 = net.add(t1, t2)
    m1 = net.mul(t5, (c1 + c2) / 2 - 1.0)
    m2 = net.mul(net.sub(t1, t2), (c1 - c2) / 2)
    y0 = net.add(x[0], t5)
    a = net.add(y0, m1)
    a1 = net.add(a, m2); a2 = net.sub(a, m2)
    m3 = net.mul(net.add(t3, t4), s2)
    m4 = net.mul(t3, s1 - s2)
    m5 = net.mul(t4, s1 + s2)
    b1 = net.add(m3, m4); b2 = net.sub(m3, m5)
    return [(y0, None), (a1, net.neg(b1)), (a2, net.neg(b2))]


def cfft_any(net, z):
    n = len(z)
    if n == 5:
        return cfft5(net, z)
    if n == 12:
        return cfft_pfa(net, z, 3, 4)
    if n == 10:
        return cfft_pfa(net, z, 5, 2)
    if n == 20:
        return cfft_pfa(net, z, 5, 4)
    if n == 6:
        return cfft_pfa(net, z, 3, 2)
    if n == 14:
        return cfft_pfa(net, z, 7, 2)
    if n == 15:
        return cfft_pfa(net, z, 5, 3)
    return cfft(net, z)


def rfft_pfa(net, x, n1, n2):
    n = n1 * n2
    inner = [rfft(net, [x[(n2 * t1 + n1 * t2) % n] for t1 in range(n1)]) for t2 in range(n2)]
    out = [None] * (n // 2 + 1)
    for k1 in range(n1 // 2 + 1):
        col = [inner[t2][k1] for t2 in range(n2)]
        if all(c[1] is None for c in col):
            Z = rfft(net, [c[0] for c in col])
            Z = Z + [(Z[n2 - k2][0], net.neg(Z[n2 - k2][1])) for k2 in range(len(Z), n2)]
        else:
            Z = cfft_any(net, col)
        for k2 in range(n2):
            k = [k for k in range(n) if k % n1 == k1 and k % n2 == k2][0]
            if k <= n // 2:
                if out[k] is None:
                    out[k] = Z[k2]
            else:
                if out[n - k] is None:
                    out[n - k] = (Z[k2][0], net.neg(Z[k2][1]))
    return out


PFA = {40: (8, 5), 20: (4, 5), 24: (8, 3), 48: (16, 3), 12: (4, 3), 56: (8, 7), 10: (2, 5), 6: (2, 3), 60: (4, 15), 15: (3, 5), 44: (4, 11), 36: (4, 9)}
USE_PFA = True


def rfft(net, x):
    n = len(x)
    if USE_PFA and n in PFA:
        return rfft_pfa(net, x, *PFA[n])
    if n == 1:
        return [(x[0], None)]
    if n == 2:
        return [(net.add(x[0], x[1]), None), (net.sub(x[0], x[1]), None)]
    if n % 4 == 0:
        h, q = n // 2, n // 4
        e = [net.add(x[t], x[t + h]) for t in range(h)]
        o = [net.sub(x[t], x[t + h]) for t in range(h)]
        z = [net.cmulc((o[t], net.neg(o[t + q])), *w(t, n)) for t in range(q)]
        E = rfft(net, e)
        Z = cfft_any(net, z)
        out = [None] * (h + 1)
        for k in range(len(E)):
            out[2 * k] = E[k]
        for k in range(q):
            f = 4 * k + 1
            if f <= h:
                out[f] = Z[k]
            else:
                out[n - f] = (Z[k][0], net.neg(Z[k][1]))
        return out
    if n % 2 == 0:
        m = n // 2
        e = [net.add(x[t], x[t + m]) for t in range(m)]
        o = [net.sub(x[t], x[t + m]) for t in range(m)]
        E = rfft(net, e)
        op = [o[t] if t % 2 == 0 else net.neg(o[t]) for t in range(m)]
        O = rfft(net, op)
        out = [None] * (m + 1)
        for k in range(len(E)):
            out[2 * k] = E[k]
        for f in range(1, m + 1, 2):
            j = ((f - m) // 2) % m
            if j <= m // 2:
                out[f] = O[j]
            else:
                out[f] = (O[m - j][0], net.neg(O[m - j][1]))
        return out
    if n == 5:
        return rfft5(net, x)
    p = {t: net.add(x[t], x[n - t]) for t in range(1, (n + 1) // 2)}
    q = {t: net.sub(x[t], x[n - t]) for t in range(1, (n + 1) // 2)}
    s = x[0]
    for t in p:
        s = net.add(s, p[t])
    out = [(s, None)]
    for k in range(1, (n + 1) // 2):
        A = x[0]
        B = None
        for t in p:
            c, sn = w(k * t, n)
            A = net.add(A, net.mul(p[t], c))
            B = net.add(B, net.mul(q[t], sn))
        out.append((A, B))
    return out


class Prog:
    def __init__(self, net, outputs):
        order = []
        seen = set()

        def visit(n):
            if n in seen:
                return
            seen.add(n)
            k = net.nodes[n]
            if k[0] in ('add', 'sub'):
                visit(k[1]); visit(k[2])
            elif k[0] == 'mul':
                visit(k[1])
            order.append(n)
        for o in outputs:
            if o is not None:
                visit(o[0])
        self.net = net
        self.order = order
        self.outputs = outputs

    def count(self):
        c = {'add': 0, 'sub': 0, 'mul': 0, 'in': 0}
        for n in self.order:
            c[self.net.nodes[n][0]] += 1
        return c

    def run(self, load, emit=None):
        vals = {}
        for n in self.order:
            k = self.net.nodes[n]
            if k[0] == 'in':
                vals[n] = load(k[1])
            elif k[0] == 'add':
                vals[n] = vals[k[1]] + vals[k[2]]
            elif k[0] == 'sub':
                vals[n] = vals[k[1]] - vals[k[2]]
            else:
                vals[n] = vals[k[1]] * k[2]
        return [None if o is None else vals[o[0]] for o in self.outputs]

    @property
    def signs(self):
        return [0 if o is None else o[1] for o in self.outputs]

    def matrix(self, n_in, signed=True):
        eye = np.eye(n_in)
        res = self.run(lambda i: eye[i])
        rows = []
        for r, s in zip(res, self.signs):
            rows.append(np.zeros(n_in) if r is None else (r * s if signed else r))
        return np.stack(rows)


def transpose(net, outputs, wanted_inputs):
    prog = Prog(net, outputs)
    live = set(prog.order)
    consumers = {n: [] for n in prog.order}
    for n in prog.order:
        k = net.nodes[n]
        if k[0] == 'add':
            consumers[k[1]].append((n, 1.0)); consumers[k[2]].append((n, 1.0))
        elif k[0] == 'sub':
            consumers[k[1]].append((n, 1.0)); consumers[k[2]].append((n, -1.0))
        elif k[0] == 'mul':
            consumers[k[1]].append((n, k[2]))
    outmap = {}
    for r, o in enumerate(outputs):
        if o is not None:
            outmap.setdefault(o[0], []).append((r, o[1]))
    tn = Net()
    memo = {}

    def adj(n):
        if n in memo:
            return memo[n]
        acc = None
        for r, s in outmap.get(n, []):
            v = tn.inp(r)
            acc = tn.add(acc, v if s > 0 else tn.neg(v))
        for c, coef in consumers[n]:
            acc = tn.add(acc, tn.mul(adj(c), coef))
        memo[n] = acc
        return acc
    outs = []
    for i in wanted_inputs:
        key = ('in', i)
        if key in net.cse and net.cse[key] in live:
            outs.append(adj(net.cse[key]))
        else:
            outs.append(None)
    return tn, outs


def build(N, taps, scale=True, variant=0):
    hop = N - taps + 1
    na = Net()
    U = rfft(na, [na.inp(t) for t in range(N)])
    a_out = [U[0][0], U[N // 2][0]]
    bins = list(range(1, N // 2))
    for k in bins:
        a, b = U[k]
        if variant == 0:
            a_out += [na.add(a, b), a, b]
        else:
            a_out += [a, na.sub(b, a), na.add(a, b)]
    nc = Net()
    V = rfft(nc, [nc.inp(t) for t in range(N)])
    c_out = [V[0][0], V[N // 2][0]]
    for k in bins:
        al, be = V[k]
        c_out += [nc.add(al, be), be, nc.neg(al)]
    tn, c_res = transpose(nc, c_out, list(range(hop)))
    def mkb(ntaps):
        nb = Net()
        Wf = rfft(nb, [nb.inp(t) if t < ntaps else None for t in range(N)])
        s0 = 1.0 / N if scale else 0.5
        b_out = [nb.mul(Wf[0][0], s0), nb.mul(Wf[N // 2][0], s0)]
        for k in bins:
            c = Wf[k][0]
            d = nb.neg(Wf[k][1])
            sc = 2.0 / N if scale else 1.0
            if variant == 0:
                b_out += [nb.mul(c, sc), nb.mul(nb.sub(d, c), sc), nb.mul(nb.add(c, d), sc)]
            else:
                b_out += [nb.mul(nb.add(c, d), sc), nb.mul(c, sc), nb.mul(d, sc)]
        return nb, b_out
    nb, b_out = mkb(taps)
    nb1, b1_out = mkb(taps - 1)
    return dict(N=N, hop=hop, taps=taps, na=na, a_out=a_out, nb=nb, b_out=b_out, nb1=nb1, b1_out=b1_out,
                tn=tn, c_res=c_res, bins=bins)


def max_live(net, order, outputs, out_at_once=True):
    uses = {n: 0 for n in order}
    for n in order:
        k = net.nodes[n]
        for a in ([k[1], k[2]] if k[0] in ('add', 'sub') else [k[1]] if k[0] == 'mul' else []):
            uses[a] += 1
    live = set(); peak = 0; tot = 0
    rem = dict(uses)
    for n in order:
        k = net.nodes[n]
        live.add(n)
        peak = max(peak, len(live))
        for a in set([k[1], k[2]] if k[0] in ('add', 'sub') else [k[1]] if k[0] == 'mul' else []):
            rem[a] -= (1 if k[0] == 'mul' or k[1] != k[2] else 2)
            if rem[a] == 0:
                live.discard(a)
        if rem[n] == 0:
            live.discard(n)
        tot += len(live)
    return peak, tot / len(order)


def min_live_order(net, outputs, seed=0, tries=200):
    base = Prog(net, outputs).order
    nodes = set(base)
    def operands(n):
        k = net.nodes[n]
        return [k[1], k[2]] if k[0] in ('add', 'sub') else [k[1]] if k[0] == 'mul' else []
    consumers = {n: [] for n in base}
    for n in base:
        for a in set(operands(n)):
            consumers[a].append(n)
    best = (max_live(net, base, outputs), base)
    rnd = random.Random(seed)
    pos = {n: i for i, n in enumerate(base)}
    for it in range(tries):
        done = set(); order = []
        live = set()
        remc = {n: len(consumers[n]) for n in base}
        isin = {n: net.nodes[n][0] == 'in' for n in base}
        def ready(n):
            return n not in done and not isin[n] and all((a in done) or isin[a] for a in operands(n))
        noise = rnd.random() * 1.5
        work = [n for n in base if not isin[n]]
        left = set(work)
        while left:
            cands = [n for n in left if ready(n)]
            def score(n):
                ops = set(operands(n))
                newloads = sum(1 for a in ops if a not in done)
                kills = sum(1 for a in ops if remc[a] == 1)
                born = 0 if remc[n] == 0 else 1
                return (newloads + born - kills) + noise * rnd.random() + 1e-4 * pos[n]
            n = min(cands, key=score)
            for a in sorted(set(operands(n)), key=lambda a: pos[a]):
                if a not in done:
                    done.add(a); order.append(a)
                remc[a] -= 1
            done.add(n); order.append(n); left.discard(n)
        ml = max_live(net, order, outputs)
        if ml < best[0]:
            best = (ml, order)
    return best


def solve_signs(G, iters=200000, seed=0):
    rnd = random.Random(seed)
    nets = {'A': (G['na'], G['a_out']), 'B': (G['nb'], G['b_out']), 'C': (G['tn'], G['c_res'])}
    order = {k: Prog(*v).order for k, v in nets.items()}
    R = len(G['a_out'])
    sig = {}
    for k in 'ABC':
        for n in order[k]:
            sig[(k, n)] = 1
    fixed = set()
    for k in 'AB':
        for n in order[k]:
            if nets[k][0].nodes[n][0] == 'in':
                fixed.add((k, n))
    for o in G['c_res']:
        sig[('C', o[0])] = o[1]; fixed.add(('C', o[0]))
    cin = {}
    for n in order['C']:
        nd = G['tn'].nodes[n]
        if nd[0] == 'in':
            cin[nd[1]] = n; fixed.add(('C', n))
    def cin_sign(r):
        a, b = G['a_out'][r], G['b_out'][r]
        return (sig[('A', a[0])] * a[1]) * (sig[('B', b[0])] * b[1])
    outmap = {}
    for r in range(R):
        outmap.setdefault(('A', G['a_out'][r][0]), []).append(r)
        outmap.setdefault(('B', G['b_out'][r][0]), []).append(r)
    def refresh():
        for r, n in cin.items():
            sig[('C', n)] = cin_sign(r)
    clauses = []
    for k in 'ABC':
        net = nets[k][0]
        for n in order[k]:
            nd = net.nodes[n]
            if nd[0] in ('add', 'sub'):
                clauses.append((k, n, nd[1], nd[2], 1 if nd[0] == 'add' else -1))
    occ = {}
    for ci, (k, n, a, b, cb) in enumerate(clauses):
        for v in (n, a, b):
            occ.setdefault((k, v), []).append(ci)
    def viol(ci):
        k, n, a, b, cb = clauses[ci]
        return sig[(k, n)] * sig[(k, a)] < 0 and sig[(k, n)] * cb * sig[(k, b)] < 0
    def flip(v):
        sig[v] = -sig[v]
        for r in outmap.get(v, []):
            if r in cin:
                sig[('C', cin[r])] = cin_sign(r)
    def affected(v):
        cs = set(occ.get(v, []))
        for r in outmap.get(v, []):
            if r in cin:
                cs.update(occ.get(('C', cin[r]), []))
        return cs
    flippers = {}
    for v, rs in outmap.items():
        for r in rs:
            if r in cin:
                flippers.setdefault(('C', cin[r]), []).append(v)
    refresh()
    bad = {ci for ci in range(len(clauses)) if viol(ci)}
    best = (len(bad), dict(sig))
    for it in range(iters):
        if not bad:
            break
        ci = rnd.choice(list(bad))
        k, n, a, b, cb = clauses[ci]
        cands = []
        for v in ((k, n), (k, a), (k, b)):
            if v in fixed:
                cands += flippers.get(v, [])
            else:
                cands.append(v)
        cands = [v for v in cands if v not in fixed]
        if not cands:
            continue
        def delta(v):
            cs = affected(v)
            before = sum(viol(c) for c in cs)
            flip(v)
            after = sum(viol(c) for c in cs)
            flip(v)
            return after - before
        if rnd.random() < 0.2:
            v = rnd.choice(cands)
        else:
            v = min(cands, key=lambda v: (delta(v), rnd.random()))
        cs = affected(v)
        flip(v)
        for c in cs:
            if viol(c): bad.add(c)
            else: bad.discard(c)
        if len(bad) < best[0]:
            best = (len(bad), dict(sig))
    nb, sg = best
    return ({n: s for (k, n), s in sg.items() if k == 'A'}, {n: s for (k, n), s in sg.items() if k == 'B'},
            {n: s for (k, n), s in sg.items() if k == 'C'}, nb)


class FixedProg:
    def __init__(self, net, outputs, sig, order=None):
        self.net, self.outputs, self.sig = net, outputs, sig
        self.order = order if order is not None else Prog(net, outputs).order
    def count(self):
        c = {'add': 0, 'sub': 0, 'mul': 0, 'in': 0}
        for n in self.order:
            c[self.net.nodes[n][0]] += 1
        return c


N, TAPS = 40, 16
G = build(N, TAPS, scale=False, variant=1)
HOP = G['hop']; R = len(G['a_out'])
T, D, K = 16000, 512, 31
L = (T - K) // 2 + 1
MB = 64; NCH = -(-L // (HOP * MB))
CH = HOP * MB
XM = CH + 16
LP = NCH * CH
TM = T // 2
LAST_M = TM - (NCH - 1) * CH
HS = 2.0 / N
T2 = 1; W3 = 1
U32, F32, BF16 = jnp.uint32, jnp.float32, jnp.bfloat16

bins = G['bins']
ev = [0, 1] + [2 + 3 * i + q for i, k in enumerate(bins) if k % 2 == 0 for q in range(3)]
od = [2 + 3 * i + q for i, k in enumerate(bins) if k % 2 == 1 for q in range(3)]
if (N // 2) % 2 == 1:
    ev.remove(1); od = [1] + od
IDX = (ev, od)
RH = (len(ev), len(od))
LOC = {}
for hf in range(2):
    for i, r in enumerate(IDX[hf]):
        LOC[r] = (hf, i)
SA, SB, SC, NBAD = solve_signs(G)
assert NBAD == 0
def mkprog(net, outs, sig):
    return FixedProg(net, outs, sig, order=min_live_order(net, outs, tries=100)[1])
PA = [mkprog(G['na'], [G['a_out'][r] for r in idx], SA) for idx in IDX]
PB = [mkprog(G['nb'], [G['b_out'][r] for r in idx], SB) for idx in IDX]
PC = mkprog(G['tn'], G['c_res'], SC)


def run_gen(prog, loads, sink):
    nsets = len(loads)
    vals = [dict() for _ in range(nsets)]
    sig = prog.sig
    outs = {}
    for r, o in enumerate(prog.outputs):
        outs.setdefault(o[0], []).append(r)
    for n in prog.order:
        k = prog.net.nodes[n]
        for s in range(nsets):
            v = vals[s]
            if k[0] == 'in':
                v[n] = loads[s](k[1])
            elif k[0] == 'mul':
                v[n] = v[k[1]] * (k[2] * sig[n] * sig[k[1]])
            else:
                a, b = k[1], k[2]
                cb = 1 if k[0] == 'add' else -1
                p, q = sig[n] * sig[a], sig[n] * cb * sig[b]
                if p > 0 and q > 0: v[n] = v[a] + v[b]
                elif p > 0: v[n] = v[a] - v[b]
                elif q > 0: v[n] = v[b] - v[a]
                else: v[n] = -(v[a] + v[b])
            yield 1
        for r in outs.get(n, []):
            yield from sink(r, [vals[s][n] for s in range(nsets)])


def drain(gen):
    for _ in gen:
        pass


def unpack(wd, hi):
    wd = (wd & jnp.uint32(0xffff0000)) if hi else (wd << 16)
    return lax.bitcast_convert_type(wd, F32)


def pack(lo, hi):
    return pltpu.pack_elementwise([lo, hi], packed_dtype=BF16)


def prog_weight(prog, nsets, per_out):
    return len(prog.order) * nsets + len(prog.outputs) * per_out


def interleave(mms, gens_weights):
    total = sum(w for _, w in gens_weights)
    def allops():
        for g, _ in gens_weights:
            yield from g
    gen = allops()
    e = 0; done = False
    for i, mm in enumerate(mms):
        mm()
        tgt = (i + 1) * total // len(mms)
        while not done and e < tgt:
            try:
                e += next(gen)
            except StopIteration:
                done = True
    for _ in gen:
        pass


def merge(lists):
    lists = [l for l in lists if l]
    out = []
    pos = [0] * len(lists)
    tot = sum(len(l) for l in lists)
    for _ in range(tot):
        i = min((i for i in range(len(lists)) if pos[i] < len(lists[i])), key=lambda i: (pos[i] + 0.5) / len(lists[i]))
        out.append(lists[i][pos[i]]); pos[i] += 1
    return out


C0 = math.sqrt(2.0 / math.pi)
def gelu_half(zh):
    u = zh * (zh * zh * (8.0 * C0 * 0.044715) + 2.0 * C0)
    return zh * jnp.tanh(u) + zh


def kernel(x_hbm, w_hbm, gam_ref, bet_ref, out_hbm,
           xb0, xb1, xb2, xb3, we, wo, xe, xo, ye, yo, h0, h1, h2, h3, st, nrm, gsm, xsem, wsem, osem):
    xb = (xb0, xb1, xb2, xb3)
    wh = (we, wo); xh = (xe, xo); yy = (ye, yo)
    hh = (h0, h1, h2, h3)
    x32 = x_hbm.bitcast(U32)
    w32 = w_hbm.bitcast(F32)
    o32 = out_hbm.bitcast(F32)
    LASTJ = 2 * NCH - 1

    def x_copy(j, c, full):
        b = j // NCH
        cj = j % NCH
        rows = XM if full else LAST_M
        return pltpu.make_async_copy(
            x32.at[b, pl.ds(pl.multiple_of(cj * CH, 8), rows), pl.ds(c * 128, 128)],
            xb[c].at[pl.ds(0, rows), :], xsem.at[c])

    def x_start(j):
        cj = j % NCH
        @pl.when(cj < NCH - 1)
        def _():
            for c in range(4):
                x_copy(j, c, True).start()
        @pl.when(cj == NCH - 1)
        def _():
            for c in range(4):
                x_copy(j, c, False).start()
                xb[c][pl.ds(LAST_M, XM - LAST_M), :] = jnp.zeros((XM - LAST_M, 128), U32)

    def x_wait(j, cs=range(4)):
        cj = j % NCH
        @pl.when(cj < NCH - 1)
        def _():
            for c in cs:
                x_copy(j, c, True).wait()
        @pl.when(cj == NCH - 1)
        def _():
            for c in cs:
                x_copy(j, c, False).wait()

    WQ = 8
    def w_copy(n, q):
        dst = hh[n].at[1, pl.ds(0, K * 256), :].reshape(K, 256, 128)
        r = 256 // WQ
        return pltpu.make_async_copy(w32.at[:, pl.ds(q * r, r), pl.ds(n * 128, 128)], dst.at[:, pl.ds(q * r, r), :], wsem.at[n, q])

    def o_copy(n, r0, rows, k):
        return pltpu.make_async_copy(hh[n].at[0, pl.ds(r0, rows), :], o32.at[pl.ds(r0, rows), n, 0, :], osem.at[n, k])

    def a_piece(g, c, p, half):
        dyn = not isinstance(g, int)
        base = pl.multiple_of(g * (16 * HOP), 8) if dyn else g * (16 * HOP)
        row = pl.multiple_of(g * 8, 8) if dyn else g * 8
        xw = xb[c].at[pl.ds(base, 16 * HOP + 16), :]
        def mkload(o):
            return lambda t: unpack(xw[pl.ds(t + o * HOP, 8, stride=2 * HOP), :], p)
        def sink(i, vs):
            xh[half][i, pl.ds(row, 8), p * 512 + c * 128:p * 512 + (c + 1) * 128] = pack(vs[0], vs[1])
            yield 1
        return run_gen(PA[half], [mkload(0), mkload(1)], sink), prog_weight(PA[half], 2, 1)

    def a_pieces(half):
        return [a_piece(g, c, p, half) for c in range(4) for g in range(MB // 16) for p in range(2)]

    def w_piece(n, g, p, half):
        dyn = not isinstance(g, int)
        row = pl.multiple_of(g * 8, 8) if dyn else g * 8
        cache = {}
        def word(j):
            if j not in cache:
                cache[j] = lax.bitcast_convert_type(hh[n][1, pl.ds((2 * j + p) * 256 + row, 8), :], U32)
            return cache[j]
        def mkload(hi):
            def load(j):
                if 2 * j + p >= K:
                    return jnp.zeros((8, 128), F32)
                return unpack(word(j), hi)
            return load
        def sink(i, vs):
            wh[half][n, i, pl.ds(p * 256 + row, 8), :] = pack(vs[0], vs[1])
            yield 1
        return run_gen(PB[half], [mkload(0), mkload(1)], sink), prog_weight(PB[half], 2, 1)

    def c_pieces(j, n):
        if isinstance(j, int):
            b, cj = j // NCH, j % NCH
            slot = b
        else:
            valid = j >= 0
            b = jnp.where(valid, j // NCH, 0)
            cj = jnp.where(valid, j % NCH, NCH - 1)
            slot = jnp.where(valid, b, 2)
        state = {}
        def col(g):
            if g == 0:
                state['c'] = st[slot, n, 2]; state['a1'] = st[slot, n, 0]; state['a2'] = st[slot, n, 1]
            base = cj * CH + g * (8 * HOP)
            if not isinstance(j, int):
                base = pl.multiple_of(base, 8)
            hs = hh[n].at[b, pl.ds(base, 8 * HOP), :]
            def sink(t, vs):
                hs[pl.ds(t, 8, stride=HOP), :] = vs[0]
                d = vs[0] - state['c']
                state['a1'] = state['a1'] + d
                state['a2'] = state['a2'] + d * d
                yield 4
            yield from run_gen(PC, [lambda r: yy[LOC[r][0]][n, LOC[r][1], g * 8:(g + 1) * 8, :]], sink)
            if g == MB // 8 - 1:
                st[slot, n, 0] = state['a1']; st[slot, n, 1] = state['a2']
        return [(col(g), prog_weight(PC, 1, 4)) for g in range(MB // 8)]

    def set_shift(j, n):
        @pl.when(jnp.logical_and(j >= 0, j % NCH == 0))
        def _():
            st[j // NCH, n, 2] = jnp.broadcast_to(ye[n, LOC[0][1], 0:1, :], (8, 128))

    def finalize_stats(n):
        sub = lax.broadcasted_iota(jnp.int32, (8, 128), 0)
        for b in range(2):
            c = st[b, n, 2]
            r0 = (L // 8) * 8
            c1 = jnp.zeros((8, 128), F32); c2 = jnp.zeros((8, 128), F32)
            for r in range(r0, LP, 8):
                d = hh[n][b, r:r + 8, :] - c
                if r < L:
                    d = jnp.where(sub >= L - r, d, 0.0)
                c1 = c1 + d; c2 = c2 + d * d
            s1 = jnp.sum(st[b, n, 0] - c1, axis=0, keepdims=True)
            s2 = jnp.sum(st[b, n, 1] - c2, axis=0, keepdims=True)
            md = s1 * (1.0 / L)
            var = (s2 * (1.0 / L) - md * md) * (HS * HS)
            mu = c[0:1] + md
            a = (HS * lax.rsqrt(var + 1e-5)) * gam_ref[...].astype(F32).reshape(1, D)[:, n * 128:(n + 1) * 128]
            bb = bet_ref[...].astype(F32).reshape(1, D)[:, n * 128:(n + 1) * 128] - mu * a
            nrm[n, b, 0] = jnp.broadcast_to(0.5 * a, (8, 128))
            nrm[n, b, 1] = jnp.broadcast_to(0.5 * bb, (8, 128))

    def d_vreg(n, r, cs):
        a0, b0, a1, b1 = cs
        z0 = gelu_half(hh[n][0, pl.ds(r, 8), :] * a0 + b0)
        z1 = gelu_half(hh[n][1, pl.ds(r, 8), :] * a1 + b1)
        hh[n][0, pl.ds(r, 8), :] = lax.bitcast_convert_type(pack(z0, z1), F32)

    def d_consts(n):
        return nrm[n, 0, 0], nrm[n, 0, 1], nrm[n, 1, 0], nrm[n, 1, 1]

    def d_pieces(n, ra=0, rb=LP):
        state = {}
        def piece(r0, r1):
            if 'cs' not in state:
                state['cs'] = d_consts(n)
            for r in range(r0, r1, 8):
                d_vreg(n, r, state['cs'])
                yield 19
        P = 200
        return [(piece(r, min(r + P, rb)), 19 * (min(r + P, rb) - r) // 8) for r in range(ra, rb, P)]

    def fin_piece(n):
        def gen():
            finalize_stats(n)
            yield 100
        return [(gen(), 100)]

    NPC = 4
    PR = -(-(-(-L // NPC)) // 8) * 8
    def d_loop(n, k0):
        cs = d_consts(n)
        UN = 5
        for k in range(k0, NPC):
            r0 = k * PR; r1 = min(r0 + PR, LP)
            nv = -(-(r1 - r0) // 8)
            assert nv % UN == 0, nv
            def body(i, carry):
                for u in range(UN):
                    d_vreg(n, pl.multiple_of(r0 + (i * UN + u) * 8, 8), cs)
                return carry
            lax.fori_loop(0, nv // UN, body, 0)
            o_copy(n, r0, min(r0 + PR, L) - r0, k).start()

    def o_start_all(n):
        for k in range(NPC):
            r0 = k * PR
            o_copy(n, r0, min(r0 + PR, L) - r0, k).start()

    def o_wait_all(n):
        for k in range(NPC):
            r0 = k * PR
            o_copy(n, r0, min(r0 + PR, L) - r0, k).wait()

    def mm(half, n, i):
        def f():
            lhs = pltpu.bitcast(xh[half][i], BF16)
            rhs = pltpu.bitcast(wh[half][n, i], BF16)
            yy[half][n, i] = jnp.dot(lhs, rhs, preferred_element_type=F32)
        return f

    def body(name, half, tiles, lists, sl=None):
        mms = [mm(half, n, i) for n in tiles for i in range(RH[half])]
        if sl is not None:
            mms = mms[sl]
        with jax.named_scope(name):
            interleave(mms, merge(lists))

    j0 = jnp.int32(0)
    for k_ in range(32):
        gsm[k_] = jnp.int32(0)
    for n in range(2):
        for q in range(WQ):
            w_copy(n, q).start()
    st[...] = jnp.zeros_like(st)

    GP = 32 // WQ
    QX = 2
    def w_stage(n, nq):
        def wl(g, carry):
            for p in range(2):
                for half in range(2):
                    drain(w_piece(n, g, p, half)[0])
            return carry
        def wq(q, carry):
            w_copy(n, q).wait()
            lax.fori_loop(q * GP, (q + 1) * GP, wl, 0)
            return carry
        lax.fori_loop(0, nq, wq, 0)

    with jax.named_scope("w0"):
        w_stage(0, WQ)
    for q in range(WQ):
        w_copy(2, q).start()
    x_start(j0)
    with jax.named_scope("w1"):
        w_stage(1, WQ)
    for q in range(WQ):
        w_copy(3, q).start()
    with jax.named_scope("w2"):
        w_stage(2, WQ)
    with jax.named_scope("a0"):
        for c in range(4):
            x_wait(j0, [c])
            def a0(g, carry):
                for p in range(2):
                    drain(a_piece(g, c, p, 0)[0])
                return carry
            lax.fori_loop(0, MB // 16, a0, 0)
    with jax.named_scope("w3"):
        w_stage(3, QX)

    def main(j, carry):
        @pl.when(j >= 0)
        def _():
            body("E01", 0, (0, 1), [a_pieces(1)])
        @pl.when(j + 1 <= LASTJ)
        def _():
            x_start(j + 1)
        set_shift(j - 1, 2); set_shift(j - 1, 3)
        if W3:
            @pl.when(j <= 0)
            def _():
                for q in range(QX, WQ):
                    w_copy(3, q).wait()
            @pl.when(j == 0)
            def _():
                body("O01W", 1, (0, 1), [[w_piece(3, g, p, half) for g in range(QX * GP, 32) for p in range(2) for half in range(2)]])
        @pl.when(j + 1 >= (2 if W3 else 1))
        def _():
            body("O01", 1, (0, 1), [c_pieces(j - 1, 2), c_pieces(j - 1, 3)])
        @pl.when(j < (LASTJ if T2 else LASTJ + 1))
        def _():
            set_shift(j, 0); set_shift(j, 1)
        @pl.when(j + 2 < (LASTJ if T2 else LASTJ + 1) + 2)
        def _():
            body("E23", 0, (2, 3), [c_pieces(j, 0), c_pieces(j, 1)])
        @pl.when(j + 1 <= LASTJ)
        def _():
            x_wait(j + 1)
        @pl.when(j < (LASTJ if T2 else LASTJ + 1))
        def _():
            body("O23", 1, (2, 3), [a_pieces(0)])
        return carry
    lax.fori_loop(0, LASTJ + 1, main, 0)

    jl = jnp.int32(LASTJ)
    if T2:
        gd = gsm[0]
        set_shift(jl, 0); set_shift(jl, 1)
        def o_start(n, ks):
            for k in ks:
                r0 = k * PR
                o_copy(n, r0, min(r0 + PR, L) - r0, k).start()
        def dq(n, k):
            return d_pieces(n, k * PR, min((k + 1) * PR, LP))
        allmm = [(0, 2, i) for i in range(RH[0])] + [(0, 3, i) for i in range(RH[0])] + \
                [(1, 2, i) for i in range(RH[1])] + [(1, 3, i) for i in range(RH[1])]
        no3 = len(allmm) - RH[1]
        cuts = [0, 8, 18, 28, 38, 52, 64, 76, no3, len(allmm)]
        plan = [
            (c_pieces(LASTJ, 0) + fin_piece(0) + dq(0, 0), [(0, 0)]),
            (dq(0, 1), [(0, 1)]),
            (dq(0, 2), [(0, 2)]),
            (dq(0, 3), [(0, 3)]),
            (c_pieces(LASTJ, 1) + fin_piece(1) + dq(1, 0), [(1, 0)]),
            (dq(1, 1), [(1, 1)]),
            (dq(1, 2), [(1, 2)]),
            (dq(1, 3), [(1, 3)]),
            (c_pieces(LASTJ, 2) + fin_piece(2) + dq(2, 0), [(2, 0)]),
        ]
        set_shift(jl, 2)
        for bi, (pcs, starts) in enumerate(plan):
            @pl.when(gsm[16 + bi] >= 0)
            def _():
                with jax.named_scope("D%d" % bi):
                    interleave([mm(*t) for t in allmm[cuts[bi]:cuts[bi + 1]]], pcs)
            for n_, k_ in starts:
                o_start(n_, (k_,))

    with jax.named_scope("tail"):
        set_shift(jl, 3)
        d_loop(2, 1)
        for g_, _ in c_pieces(LASTJ, 3):
            drain(g_)
        finalize_stats(3)
        d_loop(3, 0)
        for n in range(4):
            o_wait_all(n)


@jax.jit
def pallas_standalone__self_sup_conv_stem_wavlm__speech_kernel(x, w, gn_gamma, gn_beta):
    out = pl.pallas_call(
        kernel,
        in_specs=[pl.BlockSpec(memory_space=pl.ANY), pl.BlockSpec(memory_space=pl.ANY),
                  pl.BlockSpec(memory_space=pltpu.VMEM), pl.BlockSpec(memory_space=pltpu.VMEM)],
        out_specs=pl.BlockSpec(memory_space=pl.ANY),
        out_shape=jax.ShapeDtypeStruct((L, 4, 2, 128), BF16),
        scratch_shapes=[pltpu.VMEM((XM, 128), U32)] * 4 + [
            pltpu.VMEM((4, RH[0], 512, 128), U32),
            pltpu.VMEM((4, RH[1], 512, 128), U32),
            pltpu.VMEM((RH[0], MB // 2, 1024), U32),
            pltpu.VMEM((RH[1], MB // 2, 1024), U32),
            pltpu.VMEM((4, RH[0], MB, 128), F32),
            pltpu.VMEM((4, RH[1], MB, 128), F32)] + [pltpu.VMEM((2, LP, 128), F32)] * 4 + [
            pltpu.VMEM((3, 4, 3, 8, 128), F32),
            pltpu.VMEM((4, 2, 2, 8, 128), F32),
            pltpu.SMEM((32,), jnp.int32),
            pltpu.SemaphoreType.DMA((4,)),
            pltpu.SemaphoreType.DMA((4, 8)),
            pltpu.SemaphoreType.DMA((4, 4)),
        ],
        compiler_params=pltpu.CompilerParams(vmem_limit_bytes=127 * 1024 * 1024),
    )(x, w, gn_gamma, gn_beta)
    return out.transpose(2, 0, 1, 3).reshape(2, L, D)
```
